```python
import jax
import jax.numpy as jnp

def _softmax(x, axis=-1):
    return jax.nn.softmax(x, axis=axis)

def _gelu(x):
    return jax.nn.gelu(x, approximate=True)

def _silu(x):
    return jax.nn.silu(x)

def _sigmoid(x):
    return jax.nn.sigmoid(x)

def _layernorm(x, axis=-1, eps=1e-05):
    m = jnp.mean(x, axis=axis, keepdims=True)
    v = jnp.var(x, axis=axis, keepdims=True)
    return (x - m) / jnp.sqrt(v + eps)

def _scatter_add(tgt, idx, src, axis=0):
    return tgt.at[idx].add(src)

def _segment_sum(src, seg, n):
    return jax.ops.segment_sum(src, seg, n)

class _Rng:

    def __init__(self, key):
        self._k = key

    def _next(self):
        self._k, sub = jax.random.split(self._k)
        return sub

    def normal(self, shape):
        return jax.random.normal(self._next(), shape, dtype=jnp.bfloat16)

    def randint(self, lo, hi, shape):
        return jax.random.randint(self._next(), shape, lo, hi, dtype=jnp.int32)

    def uniform(self, shape, lo=0.0, hi=1.0):
        return jax.random.uniform(self._next(), shape, jnp.bfloat16, lo, hi)

    def permutation(self, n):
        return jax.random.permutation(self._next(), n)
kernel_name = 'adaLN_cond__compressed_kv_cla__mixer_s_mlp__decode'

def setup_inputs():
    _rng = _Rng(jax.random.key(int.from_bytes(__import__("os").urandom(4), "little")))
    _w = lambda a: (lambda t: t.astype(jnp.bfloat16) if jnp.issubdtype(t.dtype, jnp.floating) else t)(jnp.asarray(a))

    def _A_setup():
        B, H, Sq, Sk, D, M = (8, 32, 1, 4096, 128, 512)
        Dc = 4 * D
        return {'x': _w((lambda *s: _rng.normal(s) * 0.05)(B, Sq, M)), 'c_kv': _w((lambda *s: _rng.normal(s) * 0.05)(B, Sk, Dc)), 'w_q': _w((lambda *s: _rng.normal(s) * 0.05)(M, H, D) * M ** (-0.5)), 'w_uk': _w((lambda *s: _rng.normal(s) * 0.05)(Dc, H, D) * Dc ** (-0.5)), 'w_uv': _w((lambda *s: _rng.normal(s) * 0.05)(Dc, H, D) * Dc ** (-0.5)), 'w_o': _w((lambda *s: _rng.normal(s) * 0.05)(H, D, M) * (H * D) ** (-0.5))}
    _A_in = _A_setup()

    def _B_setup():
        B, S, D, F = (8, 1, 512, 1792)
        return {'x': _w((lambda *s: _rng.normal(s) * 0.05)(B, S, D)), 'w1': _w((lambda *s: _rng.normal(s) * 0.05)(D, D) * D ** (-0.5)), 'w2': _w((lambda *s: _rng.normal(s) * 0.05)(D, D) * D ** (-0.5)), 'w3': _w((lambda *s: _rng.normal(s) * 0.05)(D, F) * D ** (-0.5)), 'w4': _w((lambda *s: _rng.normal(s) * 0.05)(F, D) * F ** (-0.5))}
    _B_in = _B_setup()
    return {'A_x': _A_in['x'], 'A_c_kv': _A_in['c_kv'], 'A_w_q': _A_in['w_q'], 'A_w_uk': _A_in['w_uk'], 'A_w_uv': _A_in['w_uv'], 'A_w_o': _A_in['w_o'], 'B_x': _B_in['x'], 'B_w1': _B_in['w1'], 'B_w2': _B_in['w2'], 'B_w3': _B_in['w3'], 'B_w4': _B_in['w4'], 'c': _w((lambda *s: _rng.normal(s) * 0.05)(8, 512)), 'w_mod': _w((lambda *s: _rng.normal(s) * 0.05)(512, 6 * 512) * 512 ** (-0.5))}

def reference(A_x, A_c_kv, A_w_q, A_w_uk, A_w_uv, A_w_o, B_x, B_w1, B_w2, B_w3, B_w4, c, w_mod):

    def _A_ref(x, c_kv, w_q, w_uk, w_uv, w_o):
        B, Sq, M = (x.shape[0], x.shape[1], x.shape[2])
        Sk = c_kv.shape[1]
        H, D = (w_q.shape[1], w_q.shape[2])
        q = jnp.einsum('bqm,mhd->bhqd', x, w_q)
        k = jnp.einsum('bkc,chd->bhkd', c_kv, w_uk)
        v = jnp.einsum('bkc,chd->bhkd', c_kv, w_uv)
        scores = jnp.einsum('bhqd,bhkd->bhqk', q, k) * D ** (-0.5)
        off = Sk - Sq
        qi = jnp.arange(Sq)[:, None]
        kj = jnp.arange(Sk)[None, :]
        cmask = kj <= qi + off
        scores = jnp.where(cmask[None, None], scores, -1000000000.0)
        p = _softmax(scores, axis=-1)
        ctx = jnp.einsum('bhqk,bhkd->bhqd', p, v)
        return jnp.einsum('bhqd,hdm->bqm', ctx, w_o)

    def _B_ref(x, w1, w2, w3, w4):
        B, S, D = x.shape
        h = _gelu(_layernorm(x, axis=-1) @ w1)
        c = D // 4
        g0 = jnp.pad(h[:, :, 0 * c:1 * c], ((0, 0), (1, 0), (0, 0)))[:, :S, :]
        g1 = jnp.pad(h[:, :, 1 * c:2 * c], ((0, 0), (0, 1), (0, 0)))[:, 1:, :]
        g2 = jnp.pad(h[:, :, 2 * c:3 * c], ((0, 0), (2, 0), (0, 0)))[:, :S, :]
        g3 = jnp.pad(h[:, :, 3 * c:], ((0, 0), (0, 2), (0, 0)))[:, 2:, :]
        hs = jnp.concatenate([g0, g1, g2, g3], axis=-1) @ w2
        x1 = x + hs
        h2 = _gelu(_layernorm(x1, axis=-1) @ w3) @ w4
        return x1 + h2
    x = A_x
    mod = (_silu(c) @ w_mod).reshape(c.shape[0], 6, 1, -1)
    sa, ca, ga, sb, cb, gb = (mod[:, 0].copy(), mod[:, 1].copy(), mod[:, 2].copy(), mod[:, 3].copy(), mod[:, 4].copy(), mod[:, 5].copy())
    h = _layernorm(x, axis=-1) * (1 + ca) + sa
    x = x + ga * _A_ref(h, A_c_kv, A_w_q, A_w_uk, A_w_uv, A_w_o)
    h = _layernorm(x, axis=-1) * (1 + cb) + sb
    x = x + gb * _B_ref(h, B_w1, B_w2, B_w3, B_w4)
    return x
```

```python
import functools
import math

import jax
import jax.numpy as jnp
from jax import lax
import jax.experimental.pallas as pl
import jax.experimental.pallas.tpu as pltpu

_F32 = jnp.float32
_BF16 = jnp.bfloat16
_NT = (((1,), (1,)), ((), ()))


def _dot(a, b):
    return jnp.dot(a, b, preferred_element_type=_F32)


def _dot_nt(a, b):
    return lax.dot_general(a, b, _NT, preferred_element_type=_F32)


def _layernorm(x, eps=1e-5):
    m = jnp.mean(x, axis=-1, keepdims=True)
    d = x - m
    v = jnp.mean(d * d, axis=-1, keepdims=True)
    return d / jnp.sqrt(v + eps)


def _gelu(x):
    c = math.sqrt(2.0 / math.pi)
    return 0.5 * x * (1.0 + jnp.tanh(c * (x + 0.044715 * (x * x * x))))


def _iota(shape, dim):
    return lax.broadcasted_iota(jnp.int32, shape, dim)


def _one_hot(cond):
    return jnp.where(cond, 1.0, 0.0).astype(_BF16)


def _kernel(x_hbm, ckv_hbm, wq_hbm, wuk_hbm, wuv_hbm, wo_hbm, w3_hbm, w4_hbm,
            c_hbm, wmod_hbm, o_ref,
            x_v, c_v, wmod_v, wq_v, wuk_v, wuv_v, wo_v, w3_v, w4_v, ckv_v,
            r_v, qabs_v, lat_v, a_v, ctx_v, sems, *, B, H, Sk, D, M, F):
    NP = H // 2
    W4_CHUNKS = 7
    f_chunk = F // W4_CHUNKS

    def copy(src, dst, i):
        return pltpu.make_async_copy(src, dst, sems.at[i])

    cp_c = copy(c_hbm, c_v, 0)
    cp_x = copy(x_hbm, x_v, 0)
    cp_mod0 = copy(wmod_hbm.at[:, pl.ds(0, 2 * M)], wmod_v.at[:, pl.ds(0, 2 * M)], 0)
    cp_wq = copy(wq_hbm.bitcast(jnp.uint32), wq_v, 1)
    cp_wuk = copy(wuk_hbm.bitcast(jnp.uint32), wuk_v, 2)

    def cp_kv(b):
        return copy(ckv_hbm.at[b], ckv_v.at[b], 3 + b)

    s0 = 3 + B
    cp_mod1 = copy(wmod_hbm.at[:, pl.ds(2 * M, 4 * M)], wmod_v.at[:, pl.ds(2 * M, 4 * M)], s0)
    cp_wuv = copy(wuv_hbm.bitcast(jnp.uint32), wuv_v, s0)
    cp_wo = copy(wo_hbm, wo_v, s0 + 1)
    cp_w3 = copy(w3_hbm, w3_v, s0 + 2)
    cp_w4 = [copy(w4_hbm.at[pl.ds(i * f_chunk, f_chunk)],
                  w4_v.at[pl.ds(i * f_chunk, f_chunk)], s0 + 3 + i)
             for i in range(W4_CHUNKS)]

    for cp in [cp_c, cp_x, cp_mod0, cp_wq, cp_wuk]:
        cp.start()
    for b in range(B):
        cp_kv(b).start()
    for cp in [cp_mod1, cp_wuv, cp_wo, cp_w3] + cp_w4:
        cp.start()

    expand = _one_hot(_iota((128, 256), 0) == (_iota((128, 256), 1) >> 1))
    compress = _one_hot(_iota((256, 128), 1) == (_iota((256, 128), 0) >> 1))
    ri, ci = _iota((B * H, B * H), 0), _iota((B * H, B * H), 1)
    hb_to_bh = _one_hot(ci == (ri % H) * B + ri // H)
    bh_to_hb = _one_hot(ri == (ci % H) * B + ci // H)

    def interleave(v):
        return jnp.concatenate(
            [_dot(v[:, i:i + 128], expand) for i in range(0, M, 128)], axis=1)

    def pair_weights(w_v, j):
        words = w_v[pl.ds(j, M, stride=NP), :]
        return pltpu.bitcast(words, _BF16)

    def parity_mask(n):
        return ((_iota((n, 2 * M), 0) // B) & 1) == (_iota((n, 2 * M), 1) & 1)

    cp_c.wait()
    cp_x.wait()
    cp_mod0.wait()
    cf = c_v[...].astype(_F32)
    sc = (cf * jax.nn.sigmoid(cf)).astype(_BF16)
    mod0 = _dot(sc, wmod_v[:, 0:2 * M])
    x0 = x_v[...].astype(_F32)
    h = (_layernorm(x0) * (1.0 + mod0[:, M:]) + mod0[:, :M]).astype(_BF16)
    h2 = interleave(h)
    h_lhs = jnp.where(parity_mask(2 * B), jnp.concatenate([h2, h2], axis=0), 0.0)
    h_lhs = h_lhs.astype(_BF16)

    cp_wq.wait()

    def q_body(j, carry):
        rows = pl.ds(pl.multiple_of(j * 2 * B, 2 * B), 2 * B)
        ctx_v[rows, :] = _dot(h_lhs, pair_weights(wq_v, j))
        return carry

    lax.fori_loop(0, NP, q_body, 0, unroll=2)

    cp_wuk.wait()
    qk_scale = D ** -0.5 * math.log2(math.e)

    def qabs_body(j, carry):
        rows = pl.ds(pl.multiple_of(j * 2 * B, 2 * B), 2 * B)
        r = _dot_nt(ctx_v[rows, :].astype(_BF16), pair_weights(wuk_v, j))
        r_v[rows, :] = jnp.where(parity_mask(2 * B), r * qk_scale, 0.0).astype(_BF16)
        return carry

    lax.fori_loop(0, NP, qabs_body, 0, unroll=2)
    qabs = jnp.concatenate(
        [_dot(r_v[:, i:i + 256], compress) for i in range(0, 2 * M, 256)], axis=1)
    qabs_v[...] = _dot(hb_to_bh, qabs.astype(_BF16)).astype(_BF16)

    def attn_body(b, carry):
        cp_kv(b).wait()
        rows = pl.ds(pl.multiple_of(b * H, H), H)
        s = _dot_nt(qabs_v[rows, :], ckv_v[b])
        p = jnp.exp2(s - jnp.max(s, axis=-1, keepdims=True))
        l = jnp.sum(p, axis=-1, keepdims=True)
        lat = _dot(p.astype(_BF16), ckv_v[b])
        lat_v[rows, :] = (lat / l).astype(_BF16)
        return carry

    lax.fori_loop(0, B, attn_body, 0)

    lat_hb = _dot(bh_to_hb, lat_v[...]).astype(_BF16)
    a_v[...] = jnp.where(parity_mask(B * H), interleave(lat_hb), 0.0).astype(_BF16)
    cp_mod1.wait()
    cp_wuv.wait()
    mod1 = _dot(sc, wmod_v[:, 2 * M:6 * M])

    def ctx_body(j, carry):
        rows = pl.ds(pl.multiple_of(j * 2 * B, 2 * B), 2 * B)
        ctx_v[rows, :] = _dot(a_v[rows, :], pair_weights(wuv_v, j))
        return carry

    lax.fori_loop(0, NP, ctx_body, 0, unroll=2)

    ctx = jnp.concatenate([ctx_v[i * B:(i + 1) * B, :] for i in range(H)], axis=1)
    cp_wo.wait()
    attn = _dot(ctx.astype(_BF16), wo_v[...])
    x1 = x0 + mod1[:, 0:M] * attn
    hb = _layernorm(x1) * (1.0 + mod1[:, 2 * M:3 * M]) + mod1[:, M:2 * M]
    ln = _layernorm(hb).astype(_BF16)
    cp_w3.wait()
    g = _gelu(_dot(ln, w3_v[...])).astype(_BF16)
    y = hb
    for i in range(W4_CHUNKS):
        cp_w4[i].wait()
        y = y + _dot(g[:, i * f_chunk:(i + 1) * f_chunk],
                     w4_v[i * f_chunk:(i + 1) * f_chunk, :])
    o_ref[...] = (x1 + mod1[:, 3 * M:4 * M] * y).astype(o_ref.dtype)


@jax.jit
def pallas_adaLN_cond__compressed_kv_cla__mixer_s_mlp__decode_kernel(
    A_x: jax.Array,
    A_c_kv: jax.Array,
    A_w_q: jax.Array,
    A_w_uk: jax.Array,
    A_w_uv: jax.Array,
    A_w_o: jax.Array,
    B_x: jax.Array,
    B_w1: jax.Array,
    B_w2: jax.Array,
    B_w3: jax.Array,
    B_w4: jax.Array,
    c: jax.Array,
    w_mod: jax.Array,
):
    del B_x, B_w1, B_w2
    B, Sq, M = A_x.shape
    _, Sk, Dc = A_c_kv.shape
    _, H, D = A_w_q.shape
    F = B_w3.shape[1]
    assert Sq == 1 and Dc == M and D == 128 and B == 8

    x = A_x.reshape(B, M)
    wq = A_w_q.reshape(M * H, D)
    wuk = A_w_uk.reshape(Dc * H, D)
    wuv = A_w_uv.reshape(Dc * H, D)
    wo = A_w_o.reshape(H * D, M)

    hbm = pl.BlockSpec(memory_space=pl.ANY)
    vmem = lambda a: pltpu.VMEM(a.shape, a.dtype)
    words = lambda a: pltpu.VMEM((a.shape[0] // 2, a.shape[1]), jnp.uint32)
    out = pl.pallas_call(
        functools.partial(_kernel, B=B, H=H, Sk=Sk, D=D, M=M, F=F),
        out_shape=jax.ShapeDtypeStruct(x.shape, x.dtype),
        in_specs=[hbm] * 10,
        out_specs=pl.BlockSpec(memory_space=pltpu.VMEM),
        scratch_shapes=[
            vmem(x), vmem(c), vmem(w_mod), words(wq), words(wuk), words(wuv),
            vmem(wo), vmem(B_w3), vmem(B_w4), vmem(A_c_kv),
            pltpu.VMEM((B * H, 2 * Dc), _BF16),
            pltpu.VMEM((B * H, Dc), _BF16),
            pltpu.VMEM((B * H, Dc), _BF16),
            pltpu.VMEM((B * H, 2 * Dc), _BF16),
            pltpu.VMEM((B * H, D), _F32),
            pltpu.SemaphoreType.DMA((3 + B + 3 + 7,)),
        ],
        compiler_params=pltpu.CompilerParams(vmem_limit_bytes=100 * 1024 * 1024),
    )(x, A_c_kv, wq, wuk, wuv, wo, B_w3, B_w4, c, w_mod)
    return out.reshape(A_x.shape)
```

```python
import functools
import math

import jax
import jax.numpy as jnp
from jax import lax
import jax.experimental.pallas as pl
import jax.experimental.pallas.tpu as pltpu

_F32 = jnp.float32
_BF16 = jnp.bfloat16
_NT = (((1,), (1,)), ((), ()))

_SLOTS = 8
_STEP = "TPPT"
_TICKS = _STEP.count("T")
_PARTS = _STEP.count("P")
_TICK_KIB = 48
_DELAY = 0
_W4_SLOTS = [512, 512, 512, 256] if _SLOTS == 4 else [256] * 6 + [128] * 2


def _dot(a, b):
    return jnp.dot(a, b, preferred_element_type=_F32)


def _dot_nt(a, b):
    return lax.dot_general(a, b, _NT, preferred_element_type=_F32)


def _layernorm(x, eps=1e-5):
    m = jnp.mean(x, axis=-1, keepdims=True)
    d = x - m
    v = jnp.mean(d * d, axis=-1, keepdims=True)
    return d / jnp.sqrt(v + eps)


def _gelu(x):
    c = math.sqrt(2.0 / math.pi)
    return 0.5 * x * (1.0 + jnp.tanh(c * (x + 0.044715 * (x * x * x))))


def _iota(shape, dim):
    return lax.broadcasted_iota(jnp.int32, shape, dim)


def _one_hot(cond):
    return jnp.where(cond, 1.0, 0.0).astype(_BF16)


class _Group:
    def __init__(self, src, dst, base, sizes, tick_rows, n_ticks):
        self.src, self.dst, self.base, self.sizes = src, dst, base, sizes
        self.tick_rows, self.n_ticks = tick_rows, n_ticks

    def rows(self, i):
        if isinstance(i, int):
            return self.base + sum(self.sizes[:i]), self.sizes[i]
        assert len(set(self.sizes)) == 1
        return self.base + i * self.sizes[0], self.sizes[0]

    def copy(self, start, size, sem):
        if not isinstance(start, int):
            start = pl.multiple_of(start, 8)
        rows = pl.ds(start, size)
        return pltpu.make_async_copy(self.src.at[rows], self.dst.at[rows], sem)

    def start_bulk(self, i, sems):
        start, size = self.rows(i)
        head = self.n_ticks * self.tick_rows
        self.copy(start + head, size - head, sems.at[i]).start(priority=1)

    def start_tick(self, i, j, sems):
        if j < self.n_ticks:
            start, _ = self.rows(i)
            self.copy(start + j * self.tick_rows, self.tick_rows, sems.at[i]).start()

    def wait(self, i, sems):
        self.copy(*self.rows(i), sems.at[i]).wait()


def _stream_step(arriving, following, i, sems, piece, carry):
    if arriving is not None:
        arriving.wait(i, sems)
    if following is not None:
        following.start_bulk(i, sems)
    tick = part = 0
    for op in _STEP:
        if op == "T":
            if following is not None:
                following.start_tick(i, tick, sems)
            tick += 1
        elif piece is not None:
            carry = piece(i, part, carry)
            part += 1
        elif _DELAY:
            pl.delay(_DELAY)
    return carry


def _stream_phase(arriving, following, sems, piece=None, carry=0, unroll=False):
    if unroll:
        for i in range(_SLOTS):
            carry = _stream_step(arriving, following, i, sems, piece, carry)
        return carry
    return lax.fori_loop(
        0, _SLOTS,
        lambda i, c: _stream_step(arriving, following, i, sems, piece, c), carry)


def _kernel(x_hbm, ckv_hbm, wq_hbm, wuk_hbm, wuv_hbm, wo_hbm, w3_hbm, w4_hbm,
            c_hbm, wmod_hbm, o_ref,
            x_v, c_v, wmod_v, wq_v, wuk_v, wuv_v, wo_v, w3_v, w4_v, ckv_v,
            mod_v, r_v, qabs_v, s_v, lat_v, a_v, ctx_v, ctxb_v, sems, sem_small,
            *, B, H, Sk, D, M, F):
    NP = H // 2
    PIECES = _SLOTS * _PARTS
    KC = Sk // PIECES

    def halves(src, dst, tick_rows, n_ticks, base=0, rows=None):
        rows = dst.shape[0] if rows is None else rows
        slot = rows // (2 * _SLOTS)
        return [_Group(src, dst, base + k * _SLOTS * slot, [slot] * _SLOTS,
                       tick_rows, n_ticks) for k in range(2)]

    g_mod = halves(wmod_hbm, wmod_v, 8, 12 // _SLOTS)
    g_q = halves(wq_hbm.bitcast(jnp.uint32), wq_v, 2 * _TICK_KIB, _TICKS)
    g_uk = halves(wuk_hbm.bitcast(jnp.uint32), wuk_v, 2 * _TICK_KIB, _TICKS)
    g_uv = halves(wuv_hbm.bitcast(jnp.uint32), wuv_v, 2 * _TICK_KIB, _TICKS)
    g_o = halves(wo_hbm, wo_v, _TICK_KIB, _TICKS)
    g_kv = lambda b: halves(ckv_hbm, ckv_v, _TICK_KIB, _TICKS, b * Sk, Sk)
    g_3 = _Group(w3_hbm, w3_v, 0, [M // _SLOTS] * _SLOTS, 8 * _SLOTS // 4, 12 // _SLOTS)
    g_4 = _Group(w4_hbm, w4_v, 0, _W4_SLOTS, 24 if _SLOTS == 4 else 32, _TICKS)

    cp_c = pltpu.make_async_copy(c_hbm, c_v, sem_small)
    cp_x = pltpu.make_async_copy(x_hbm, x_v, sem_small)
    cp_c.start()
    cp_x.start()
    _stream_phase(None, g_mod[0], sems, unroll=True)

    def interleave(v):
        expand = _one_hot(_iota((128, 256), 0) == (_iota((128, 256), 1) >> 1))
        return jnp.concatenate(
            [_dot(v[:, i:i + 128], expand) for i in range(0, M, 128)], axis=1)

    def pair_weights(w_v, pair, half):
        words = w_v[pl.ds(pair + half * (M // 2) * NP, M // 2, stride=NP), :]
        return pltpu.bitcast(words, _BF16)

    def parity_mask(n, width):
        return ((_iota((n, width), 0) // B) & 1) == (_iota((n, width), 1) & 1)

    def pair_of(k, i, j):
        pair = (k * PIECES + i * _PARTS + j) // 2
        return pair, pl.ds(pl.multiple_of(pair * 2 * B, 2 * B), 2 * B)

    _stream_phase(g_mod[0], g_mod[1], sems)
    _stream_phase(g_mod[1], g_q[0], sems)

    cp_c.wait()
    cp_x.wait()
    cf = c_v[...].astype(_F32)
    sc = (cf * jax.nn.sigmoid(cf)).astype(_BF16)

    def mod_piece(i, j, carry):
        n = i * _PARTS + j
        if n < 12:
            cols = slice(n * (M // 2), (n + 1) * (M // 2))
            mod_v[:, cols] = _dot(sc, wmod_v[:, cols])
        return carry

    _stream_phase(g_q[0], g_q[1], sems, mod_piece, unroll=True)
    x0 = x_v[...].astype(_F32)
    h = (_layernorm(x0) * (1.0 + mod_v[:, M:2 * M]) + mod_v[:, 0:M]).astype(_BF16)
    h2 = interleave(h)
    h_lhs = jnp.where(parity_mask(2 * B, 2 * M), jnp.concatenate([h2, h2], axis=0), 0.0)
    a_v[0:2 * B, :] = h_lhs.astype(_BF16)
    _stream_phase(g_q[1], g_uk[0], sems)

    def q_piece(k):
        def piece(i, j, acc):
            pair, rows = pair_of(k, i, j)
            half = j % 2
            part = _dot(a_v[0:2 * B, half * M:(half + 1) * M],
                        pair_weights(wq_v, pair, half))
            if half == 0:
                return part
            ctx_v[rows, :] = acc + part
            return acc
        return piece

    zero_pair = jnp.zeros((2 * B, D), _F32)
    _stream_phase(g_uk[0], g_uk[1], sems, q_piece(0), zero_pair)
    _stream_phase(g_uk[1], g_kv(0)[0], sems, q_piece(1), zero_pair)

    qk_scale = D ** -0.5 * math.log2(math.e)

    def qabs_piece(k):
        def piece(i, j, carry):
            pair, rows = pair_of(k, i, j)
            half = j % 2
            r = _dot_nt(ctx_v[rows, :].astype(_BF16), pair_weights(wuk_v, pair, half))
            r = jnp.where(parity_mask(2 * B, M), r * qk_scale, 0.0)
            r_v[rows, half * M:(half + 1) * M] = r.astype(_BF16)
            return carry
        return piece

    _stream_phase(g_kv(0)[0], g_kv(0)[1], sems, qabs_piece(0))
    _stream_phase(g_kv(0)[1], g_kv(1)[0], sems, qabs_piece(1))
    compress = _one_hot(_iota((256, 128), 1) == (_iota((256, 128), 0) >> 1))
    qabs = jnp.concatenate(
        [_dot(r_v[:, i:i + 256], compress) for i in range(0, 2 * M, 256)], axis=1)
    ri, ci = _iota((B * H, B * H), 0), _iota((B * H, B * H), 1)
    hb_to_bh = _one_hot(ci == (ri % H) * B + ri // H)
    qabs_v[...] = _dot(hb_to_bh, qabs.astype(_BF16)).astype(_BF16)

    def attend(b, arriving, following):
        q_rows = pl.ds(pl.multiple_of(b * H, H), H)

        def keys(i, j):
            n = i * _PARTS + j
            return n, ckv_v[pl.ds(pl.multiple_of(b * Sk + n * KC, KC), KC), :]

        def score_piece(i, j, m):
            n, kv = keys(i, j)
            s = _dot_nt(qabs_v[q_rows, :], kv)
            s_v[n] = s
            for t in range(0, KC, 128):
                m = jnp.maximum(m, s[:, t:t + 128])
            return m

        m = _stream_phase(arriving[0], arriving[1], sems, score_piece,
                          jnp.full((H, 128), -jnp.inf, _F32))
        m = jnp.broadcast_to(jnp.max(m, axis=-1, keepdims=True), (H, 128))

        def value_piece(i, j, carry):
            l, acc = carry
            n, kv = keys(i, j)
            s = s_v[n]
            p = [jnp.exp2(s[:, t:t + 128] - m) for t in range(0, KC, 128)]
            for pt in p:
                l = l + pt
            return l, acc + _dot(jnp.concatenate(p, axis=1).astype(_BF16), kv)

        l, acc = _stream_phase(arriving[1], following, sems, value_piece,
                               (jnp.zeros((H, 128), _F32), jnp.zeros((H, M), _F32)))
        lat_v[q_rows, :] = (acc / jnp.sum(l, axis=-1, keepdims=True)).astype(_BF16)

    def attend_body(b, carry):
        attend(b, g_kv(b + 1), g_kv(b + 2)[0])
        return carry

    lax.fori_loop(0, B - 2, attend_body, 0)
    attend(B - 2, g_kv(B - 1), g_uv[0])
    attend(B - 1, g_uv, g_o[0])

    bh_to_hb = _one_hot(ri == (ci % H) * B + ci // H)
    lat_hb = _dot(bh_to_hb, lat_v[...]).astype(_BF16)
    a_v[...] = jnp.where(parity_mask(B * H, 2 * M), interleave(lat_hb), 0.0).astype(_BF16)

    def ctx_piece(k):
        def piece(i, j, acc):
            pair, rows = pair_of(k, i, j)
            half = j % 2
            part = _dot(a_v[rows, half * M:(half + 1) * M],
                        pair_weights(wuv_v, pair, half))
            if half == 0:
                return part
            ctx = acc + part
            ctxb_v[pair] = jnp.concatenate([ctx[:B], ctx[B:]], axis=1)
            return acc
        return piece

    _stream_phase(g_o[0], g_o[1], sems, ctx_piece(0), zero_pair)
    _stream_phase(g_o[1], g_3, sems, ctx_piece(1), zero_pair)

    def out_piece(i, j, acc):
        pair = i * _PARTS + j
        return acc + _dot(ctxb_v[pair].astype(_BF16),
                          wo_v[pair * 2 * D:(pair + 1) * 2 * D, :])

    attn = _stream_phase(g_3, g_4, sems, out_piece, jnp.zeros((B, M), _F32), unroll=True)
    x1 = x0 + mod_v[:, 2 * M:3 * M] * attn
    hb = _layernorm(x1) * (1.0 + mod_v[:, 4 * M:5 * M]) + mod_v[:, 3 * M:4 * M]
    ln = _layernorm(hb).astype(_BF16)

    y = hb
    for i in range(_SLOTS):
        start, size = g_4.rows(i)
        g = _gelu(_dot(ln, w3_v[:, start:start + size])).astype(_BF16)
        g_4.wait(i, sems)
        y = y + _dot(g, w4_v[start:start + size, :])
    o_ref[...] = (x1 + mod_v[:, 5 * M:6 * M] * y).astype(o_ref.dtype)


@jax.jit
def pallas_adaLN_cond__compressed_kv_cla__mixer_s_mlp__decode_kernel(
    A_x: jax.Array,
    A_c_kv: jax.Array,
    A_w_q: jax.Array,
    A_w_uk: jax.Array,
    A_w_uv: jax.Array,
    A_w_o: jax.Array,
    B_x: jax.Array,
    B_w1: jax.Array,
    B_w2: jax.Array,
    B_w3: jax.Array,
    B_w4: jax.Array,
    c: jax.Array,
    w_mod: jax.Array,
):
    del B_x, B_w1, B_w2
    B, Sq, M = A_x.shape
    _, Sk, Dc = A_c_kv.shape
    _, H, D = A_w_q.shape
    F = B_w3.shape[1]
    assert Sq == 1 and Dc == M and D == 128 and B == 8

    x = A_x.reshape(B, M)
    wq = A_w_q.reshape(M * H, D)
    wuk = A_w_uk.reshape(Dc * H, D)
    wuv = A_w_uv.reshape(Dc * H, D)
    wo = A_w_o.reshape(H * D, M)
    ckv = A_c_kv.reshape(B * Sk, Dc)

    hbm = pl.BlockSpec(memory_space=pl.ANY)
    vmem = lambda a: pltpu.VMEM(a.shape, a.dtype)
    words = lambda a: pltpu.VMEM((a.shape[0] // 2, a.shape[1]), jnp.uint32)
    out = pl.pallas_call(
        functools.partial(_kernel, B=B, H=H, Sk=Sk, D=D, M=M, F=F),
        out_shape=jax.ShapeDtypeStruct(x.shape, x.dtype),
        in_specs=[hbm] * 10,
        out_specs=pl.BlockSpec(memory_space=pltpu.VMEM),
        scratch_shapes=[
            vmem(x), vmem(c), vmem(w_mod), words(wq), words(wuk), words(wuv),
            vmem(wo), vmem(B_w3), vmem(B_w4), vmem(ckv),
            pltpu.VMEM((B, 6 * M), _F32),
            pltpu.VMEM((B * H, 2 * Dc), _BF16),
            pltpu.VMEM((B * H, Dc), _BF16),
            pltpu.VMEM((_SLOTS * _PARTS, H, Sk // (_SLOTS * _PARTS)), _F32),
            pltpu.VMEM((B * H, Dc), _BF16),
            pltpu.VMEM((B * H, 2 * Dc), _BF16),
            pltpu.VMEM((B * H, D), _F32),
            pltpu.VMEM((H // 2, B, 2 * D), _F32),
            pltpu.SemaphoreType.DMA((_SLOTS,)),
            pltpu.SemaphoreType.DMA(()),
        ],
        compiler_params=pltpu.CompilerParams(vmem_limit_bytes=100 * 1024 * 1024),
    )(x, ckv, wq, wuk, wuv, wo, B_w3, B_w4, c, w_mod)
    return out.reshape(A_x.shape)
```

```python
import functools
import math

import jax
import jax.numpy as jnp
from jax import lax
import jax.experimental.pallas as pl
import jax.experimental.pallas.tpu as pltpu

_F32 = jnp.float32
_BF16 = jnp.bfloat16
_NT = (((1,), (1,)), ((), ()))

_SLOTS = 4
_STEP = "1T2T2STPPTPPT"
_STEP_ATTN = _STEP
_UNROLL = 1
_TICKS = _STEP.count("T")
_PARTS = _STEP.count("P")
_TICK_KIB = 40
_DELAY = 0
_PAD = 100
_W4_SLOTS = [640, 640, 256, 256]


def _dot(a, b):
    return jnp.dot(a, b, preferred_element_type=_F32)


def _dot_nt(a, b):
    return lax.dot_general(a, b, _NT, preferred_element_type=_F32)


def _layernorm(x, eps=1e-5):
    m = jnp.mean(x, axis=-1, keepdims=True)
    d = x - m
    v = jnp.mean(d * d, axis=-1, keepdims=True)
    return d / jnp.sqrt(v + eps)


def _gelu(x):
    c = math.sqrt(2.0 / math.pi)
    return 0.5 * x * (1.0 + jnp.tanh(c * (x + 0.044715 * (x * x * x))))


def _iota(shape, dim):
    return lax.broadcasted_iota(jnp.int32, shape, dim)


def _one_hot(cond):
    return jnp.where(cond, 1.0, 0.0).astype(_BF16)


class _Group:
    def __init__(self, src, dst, base, sizes, tick_rows, n_ticks):
        self.src, self.dst, self.base, self.sizes = src, dst, base, sizes
        self.tick_rows, self.n_ticks = tick_rows, n_ticks

    def rows(self, i):
        if isinstance(i, int):
            return self.base + sum(self.sizes[:i]), self.sizes[i]
        assert len(set(self.sizes)) == 1
        return self.base + i * self.sizes[0], self.sizes[0]

    def copy(self, start, size, sem):
        if not isinstance(start, int):
            start = pl.multiple_of(start, 8)
        rows = pl.ds(start, size)
        return pltpu.make_async_copy(self.src.at[rows], self.dst.at[rows], sem)

    def bulk(self, i, sem):
        start, size = self.rows(i)
        head = self.n_ticks * self.tick_rows
        return self.copy(start + head, size - head, sem)

    def tick(self, i, j, sem):
        start, _ = self.rows(i)
        return self.copy(start + j * self.tick_rows, self.tick_rows, sem)

    def wait(self, i, sem):
        self.copy(*self.rows(i), sem).wait()

    def after_ticks(self, lhs):
        zero = pltpu.bitcast(self.dst[_spare_rows(self.dst), 0:128], _BF16)
        reps = (lhs.shape[0] // zero.shape[0], lhs.shape[1] // zero.shape[1])
        return lhs + jnp.tile(zero, reps)


def _spare_rows(buf):
    n = 32 // buf.dtype.itemsize
    return pl.ds(buf.shape[0] - n, n)


def _slot_sem(sems, phase, i):
    ring = _SLOTS + 1
    first = (phase * _SLOTS) % ring
    k = first + i
    if isinstance(k, int):
        return sems.at[k % ring]
    return sems.at[jnp.where(k >= ring, k - ring, k)]


def _stream_step(sems, phase, arriving, following, i, piece, carry, step):
    sem_in, sem_out = _slot_sem(sems, phase, i), _slot_sem(sems, phase + 1, i)
    part = tick = 0
    waits = [op for op in step if op.isdigit()]
    waited = -1
    for op in step:
        if op.isdigit() and arriving is not None:
            waits.pop(0)
            upto = min(max(waited, 0) + int(op), arriving.n_ticks)
            for j in range(waited, upto if waits else arriving.n_ticks):
                copy = arriving.bulk(i, sem_in) if j < 0 else arriving.tick(i, j, sem_in)
                copy.wait()
            waited = upto
        elif op == "S":
            following.bulk(i, sem_out).start(priority=1)
        elif op == "T" and tick < following.n_ticks:
            following.tick(i, tick, sem_out).start()
            tick += 1
        elif op == "P" and piece is not None:
            carry = piece(i, part, carry, following.after_ticks)
            part += 1
        elif op == "P" and _DELAY:
            pl.delay(_DELAY)
        elif op == "D":
            pl.delay(_PAD)
    assert tick == following.n_ticks
    return carry


def _stream_phase(sems, phase, arriving, following, piece=None, carry=0,
                  unroll=_UNROLL, step=_STEP):
    if unroll == _SLOTS:
        for i in range(_SLOTS):
            carry = _stream_step(sems, phase, arriving, following, i, piece, carry, step)
        return carry

    def body(o, c):
        for u in range(unroll):
            c = _stream_step(sems, phase, arriving, following, o * unroll + u,
                             piece, c, step)
        return c

    return lax.fori_loop(0, _SLOTS // unroll, body, carry)


def _kernel(x_hbm, ckv_hbm, wq_hbm, wuk_hbm, wuv_hbm, wo_hbm, w3_hbm, w4_hbm,
            c_hbm, wmod_hbm, o_ref,
            x_v, c_v, wmod_v, wq_v, wuk_v, wuv_v, wo_v, w3_v, w4_v, ckv_v,
            mod_v, r_v, qabs_v, s_v, lat_v, a_v, q_v, ctx_v, sems, sem_small,
            *, B, H, Sk, D, M, F):
    NP = H // 2
    PIECES = _SLOTS * _PARTS
    KC = Sk // PIECES

    def halves(src, dst, tick_rows, n_ticks, base=0, rows=None):
        rows = src.shape[0] if rows is None else rows
        slot = rows // (2 * _SLOTS)
        return [_Group(src, dst, base + k * _SLOTS * slot, [slot] * _SLOTS,
                       tick_rows, n_ticks) for k in range(2)]

    g_mod = halves(wmod_hbm, wmod_v, 8, 12 // _SLOTS)
    g_q = halves(wq_hbm.bitcast(jnp.uint32), wq_v, 2 * _TICK_KIB, _TICKS)
    g_uk = halves(wuk_hbm.bitcast(jnp.uint32), wuk_v, 2 * _TICK_KIB, _TICKS)
    g_uv = halves(wuv_hbm.bitcast(jnp.uint32), wuv_v, 2 * _TICK_KIB, _TICKS)
    g_o = halves(wo_hbm, wo_v, _TICK_KIB, _TICKS)
    g_kv = lambda b: halves(ckv_hbm, ckv_v, _TICK_KIB, _TICKS, b * Sk, Sk)
    g_3 = _Group(w3_hbm, w3_v, 0, [M // _SLOTS] * _SLOTS, 8 * _SLOTS // 4, 12 // _SLOTS)
    g_4 = _Group(w4_hbm, w4_v, 0, _W4_SLOTS, 96 // _TICKS // 8 * 8, _TICKS)

    for buf in (wq_v, wuk_v, wuv_v, wo_v, w3_v, w4_v, ckv_v):
        spare = _spare_rows(buf)
        buf[spare, 0:128] = jnp.zeros((spare.size, 128), buf.dtype)

    cp_c = pltpu.make_async_copy(c_hbm, c_v, sem_small)
    cp_x = pltpu.make_async_copy(x_hbm, x_v, sem_small)
    cp_c.start()
    cp_x.start()
    _stream_phase(sems, _SLOTS, None, g_mod[0], unroll=_SLOTS)

    def interleave(v):
        expand = _one_hot(_iota((128, 256), 0) == (_iota((128, 256), 1) >> 1))
        return jnp.concatenate(
            [_dot(v[:, i:i + 128], expand) for i in range(0, M, 128)], axis=1)

    def pair_weights(w_v, pair, half):
        words = w_v[pl.ds(pair + half * (M // 2) * NP, M // 2, stride=NP), :]
        return pltpu.bitcast(words, _BF16)

    def parity_mask(n, width):
        return ((_iota((n, width), 0) // B) & 1) == (_iota((n, width), 1) & 1)

    def pair_of(i, j):
        pair = i * _PARTS + j
        return pair, pl.ds(pl.multiple_of(pair * 2 * B, 2 * B), 2 * B)

    _stream_phase(sems, 0, g_mod[0], g_mod[1])
    _stream_phase(sems, 1, g_mod[1], g_q[0])

    cp_c.wait()
    cp_x.wait()
    cf = c_v[...].astype(_F32)
    sc = cf * jax.nn.sigmoid(cf)
    sc = jnp.concatenate([sc, sc], axis=0).astype(_BF16)

    def mod_piece(i, j, carry, pin):
        n = i * _PARTS + j
        if n < 12:
            cols = slice(n * (M // 2), (n + 1) * (M // 2))
            mod_v[:, cols] = _dot(pin(sc), wmod_v[:, cols])[:B]
        if n == 12:
            x0 = x_v[...].astype(_F32)
            h = _layernorm(x0) * (1.0 + mod_v[:, M:2 * M]) + mod_v[:, 0:M]
            h2 = interleave(h.astype(_BF16))
            h2 = jnp.concatenate([h2, h2], axis=0)
            a_v[0:2 * B, :] = jnp.where(parity_mask(2 * B, 2 * M), h2, 0.0).astype(_BF16)
        return carry

    _stream_phase(sems, 2, g_q[0], g_q[1], mod_piece, unroll=_SLOTS)

    def q_piece(half):
        def piece(i, j, carry, pin):
            pair, rows = pair_of(i, j)
            part = _dot(pin(a_v[0:2 * B, half * M:(half + 1) * M]),
                        pair_weights(wq_v, pair, half))
            q_v[rows, :] = part if half == 0 else q_v[rows, :] + part
            return carry
        return piece

    _stream_phase(sems, 3, g_q[1], g_uk[0], q_piece(0))
    _stream_phase(sems, 4, g_uk[0], g_uk[1], q_piece(1))

    qk_scale = D ** -0.5 * math.log2(math.e)

    def qabs_piece(half):
        def piece(i, j, carry, pin):
            pair, rows = pair_of(i, j)
            r = _dot_nt(pin(q_v[rows, :].astype(_BF16)), pair_weights(wuk_v, pair, half))
            r = jnp.where(parity_mask(2 * B, M), r * qk_scale, 0.0)
            r_v[rows, half * M:(half + 1) * M] = r.astype(_BF16)
            return carry
        return piece

    _stream_phase(sems, 5, g_uk[1], g_kv(0)[0], qabs_piece(0))
    _stream_phase(sems, 6, g_kv(0)[0], g_kv(0)[1], qabs_piece(1))
    compress = _one_hot(_iota((256, 128), 1) == (_iota((256, 128), 0) >> 1))
    qabs = jnp.concatenate(
        [_dot(r_v[:, i:i + 256], compress) for i in range(0, 2 * M, 256)], axis=1)
    ri, ci = _iota((B * H, B * H), 0), _iota((B * H, B * H), 1)
    hb_to_bh = _one_hot(ci == (ri % H) * B + ri // H)
    qabs_v[...] = _dot(hb_to_bh, qabs.astype(_BF16)).astype(_BF16)

    def head_rows(b):
        return pl.ds(pl.multiple_of(b * H, H), H)

    def keys(b, n):
        return ckv_v[pl.ds(pl.multiple_of(b * Sk + n * KC, KC), KC), :]

    def score_chunk(b, n, m, pin):
        s = _dot_nt(pin(qabs_v[head_rows(b), :]), keys(b, n))
        s_v[b % 2, n] = s
        for t in range(0, KC, 128):
            m = jnp.maximum(m, s[:, t:t + 128])
        return m

    def value_chunk(b, n, s, m, l, acc, pin):
        p = [jnp.exp2(s[:, t:t + 128] - m) for t in range(0, KC, 128)]
        for pt in p:
            l = l + pt
        return l, acc + _dot(pin(jnp.concatenate(p, axis=1).astype(_BF16)), keys(b, n))

    def row_max(m):
        return jnp.broadcast_to(jnp.max(m, axis=-1, keepdims=True), (H, 128))

    def store_lat(b, l, acc):
        lat_v[head_rows(b), :] = (acc / jnp.sum(l, axis=-1, keepdims=True)).astype(_BF16)

    m_init = jnp.full((H, 128), -jnp.inf, _F32)
    l_init, acc_init = jnp.zeros((H, 128), _F32), jnp.zeros((H, M), _F32)

    def attend(b, groups, m_prev, with_values=True):
        def piece(half):
            scores = []

            def run(i, j, carry, pin):
                if groups[half + 1].dst is ckv_v:
                    pin = lambda lhs: lhs
                m, l, acc = carry
                first = (half * _SLOTS + i) * (_PARTS // 2)
                n = first + j // 2
                if j == 0 and with_values:
                    scores[:] = [s_v[(b - 1) % 2, first + k] for k in range(_PARTS // 2)]
                if j % 2 == 1:
                    m = score_chunk(b, n, m, pin)
                elif with_values:
                    l, acc = value_chunk(b - 1, n, scores[j // 2], m_prev, l, acc, pin)
                return m, l, acc
            return run

        carry = (m_init, l_init, acc_init) if with_values else (m_init, 0, 0)
        for half in range(2):
            carry = _stream_phase(sems, 7 + 2 * b + half, groups[half], groups[half + 1],
                                  piece(half), carry, step=_STEP_ATTN)
        m, l, acc = carry
        if with_values:
            store_lat(b - 1, l, acc)
        return row_max(m)

    def kv_groups(b):
        return [g_kv(b)[1]] + g_kv(b + 1)

    m = attend(0, kv_groups(0), None, with_values=False)
    m = lax.fori_loop(1, B - 1, lambda b, m: attend(b, kv_groups(b), m), m)
    m = attend(B - 1, [g_kv(B - 1)[1]] + g_uv, m)
    l, acc = _stream_phase(
        sems, 7 + 2 * B, g_uv[1], g_o[0],
        lambda i, j, c, pin: value_chunk(B - 1, i * _PARTS + j,
                                    s_v[(B - 1) % 2, i * _PARTS + j], m, *c, pin),
        (l_init, acc_init))
    store_lat(B - 1, l, acc)

    bh_to_hb = _one_hot(ri == (ci % H) * B + ci // H)
    lat_hb = _dot(bh_to_hb, lat_v[...]).astype(_BF16)
    a_v[...] = jnp.where(parity_mask(B * H, 2 * M), interleave(lat_hb), 0.0).astype(_BF16)

    def ctx_piece(k):
        def piece(i, j, acc, pin):
            pair, rows = pair_of(k * _SLOTS // 2, (i * _PARTS + j) // 2)
            half = j % 2
            part = _dot(pin(a_v[rows, half * M:(half + 1) * M]),
                        pair_weights(wuv_v, pair, half))
            if half == 0:
                return part
            ctx = acc + part
            ctx_v[pair] = jnp.concatenate([ctx[:B], ctx[B:]], axis=1)
            return acc
        return piece

    zero_pair = jnp.zeros((2 * B, D), _F32)
    _stream_phase(sems, 8 + 2 * B, g_o[0], g_o[1], ctx_piece(0), zero_pair)
    _stream_phase(sems, 9 + 2 * B, g_o[1], g_3, ctx_piece(1), zero_pair)

    def mlp_piece(i, j, carry, pin):
        n = i * _PARTS + j
        if n < NP // 2:
            for pair in (2 * n, 2 * n + 1):
                ctx = ctx_v[pair]
                ctx = pin(jnp.concatenate([ctx, ctx], axis=0).astype(_BF16))
                carry = carry + _dot(ctx, wo_v[pair * 2 * D:(pair + 1) * 2 * D, :])[:B]
        elif n == NP // 2:
            x1 = x_v[...].astype(_F32) + mod_v[:, 2 * M:3 * M] * carry
            hb = _layernorm(x1) * (1.0 + mod_v[:, 4 * M:5 * M]) + mod_v[:, 3 * M:4 * M]
            ln = _layernorm(hb)
            ln = jnp.concatenate([ln, ln], axis=0).astype(_BF16)
            carry = x1, hb, ln, jnp.zeros((B, F), _F32)
        elif n - NP // 2 <= _SLOTS:
            k = n - NP // 2 - 1
            assert k <= i
            x1, hb, ln, pre = carry
            start, size = g_3.rows(k)
            pre = pre + _dot(pin(ln[:, start:start + size]), w3_v[start:start + size, :])[:B]
            carry = x1, hb, ln, pre
        return carry

    x1, y, _, pre = _stream_phase(sems, 10 + 2 * B, g_3, g_4, mlp_piece,
                                  jnp.zeros((B, M), _F32), unroll=_SLOTS)
    g = _gelu(pre).astype(_BF16)
    for i in range(_SLOTS):
        start, size = g_4.rows(i)
        g_4.wait(i, _slot_sem(sems, 11 + 2 * B, i))
        y = y + _dot(g[:, start:start + size], w4_v[start:start + size, :])
    o_ref[...] = (x1 + mod_v[:, 5 * M:6 * M] * y).astype(o_ref.dtype)


@jax.jit
def pallas_adaLN_cond__compressed_kv_cla__mixer_s_mlp__decode_kernel(
    A_x: jax.Array,
    A_c_kv: jax.Array,
    A_w_q: jax.Array,
    A_w_uk: jax.Array,
    A_w_uv: jax.Array,
    A_w_o: jax.Array,
    B_x: jax.Array,
    B_w1: jax.Array,
    B_w2: jax.Array,
    B_w3: jax.Array,
    B_w4: jax.Array,
    c: jax.Array,
    w_mod: jax.Array,
):
    del B_x, B_w1, B_w2
    B, Sq, M = A_x.shape
    _, Sk, Dc = A_c_kv.shape
    _, H, D = A_w_q.shape
    F = B_w3.shape[1]
    assert Sq == 1 and Dc == M and D == 128 and B == 8

    x = A_x.reshape(B, M)
    wq = A_w_q.reshape(M * H, D)
    wuk = A_w_uk.reshape(Dc * H, D)
    wuv = A_w_uv.reshape(Dc * H, D)
    wo = A_w_o.reshape(H * D, M)
    ckv = A_c_kv.reshape(B * Sk, Dc)

    hbm = pl.BlockSpec(memory_space=pl.ANY)
    vmem = lambda a: pltpu.VMEM(a.shape, a.dtype)
    spare = lambda a: pltpu.VMEM((a.shape[0] + 16, a.shape[1]), a.dtype)
    words = lambda a: pltpu.VMEM((a.shape[0] // 2 + 8, a.shape[1]), jnp.uint32)
    out = pl.pallas_call(
        functools.partial(_kernel, B=B, H=H, Sk=Sk, D=D, M=M, F=F),
        out_shape=jax.ShapeDtypeStruct(x.shape, x.dtype),
        in_specs=[hbm] * 10,
        out_specs=pl.BlockSpec(memory_space=pltpu.VMEM),
        scratch_shapes=[
            vmem(x), vmem(c), vmem(w_mod), words(wq), words(wuk), words(wuv),
            spare(wo), spare(B_w3), spare(B_w4), spare(ckv),
            pltpu.VMEM((B, 6 * M), _F32),
            pltpu.VMEM((B * H, 2 * Dc), _BF16),
            pltpu.VMEM((B * H, Dc), _BF16),
            pltpu.VMEM((2, _SLOTS * _PARTS, H, Sk // (_SLOTS * _PARTS)), _F32),
            pltpu.VMEM((B * H, Dc), _BF16),
            pltpu.VMEM((B * H, 2 * Dc), _BF16),
            pltpu.VMEM((B * H, D), _F32),
            pltpu.VMEM((H // 2, B, 2 * D), _F32),
            pltpu.SemaphoreType.DMA((_SLOTS + 1,)),
            pltpu.SemaphoreType.DMA(()),
        ],
        compiler_params=pltpu.CompilerParams(vmem_limit_bytes=100 * 1024 * 1024),
    )(x, ckv, wq, wuk, wuv, wo, B_w3, B_w4, c, w_mod)
    return out.reshape(A_x.shape)
```

```python
import functools
import math

import jax
import jax.numpy as jnp
from jax import lax
import jax.experimental.pallas as pl
import jax.experimental.pallas.tpu as pltpu

_F32 = jnp.float32
_BF16 = jnp.bfloat16
_NT = (((1,), (1,)), ((), ()))

_SLOTS = 4
_STEP = "1T2T2STPPTPPT"
_STEP_ATTN = "0T2T3STPPTPPT"
_UNROLL = 1
_TICKS = _STEP.count("T")
_PARTS = _STEP.count("P")
_PIECES = _SLOTS * _PARTS
_TICK_KIB = 40
_KV_TICKS = 5
_KV_TICK_KIB = 40
_STEP_MLP = _STEP
_STEP_IDLE = "0T1T2ST"
_W4A, _W4A_TICK = 1536, 24
_W4B, _W4B_TICK = [256], 16


def _dot(a, b):
    return jnp.dot(a, b, preferred_element_type=_F32)


def _dot_nt(a, b):
    return lax.dot_general(a, b, _NT, preferred_element_type=_F32)


def _layernorm(x, eps=1e-5):
    m = jnp.mean(x, axis=-1, keepdims=True)
    d = x - m
    v = jnp.mean(d * d, axis=-1, keepdims=True)
    return d / jnp.sqrt(v + eps)


def _gelu(x):
    c = math.sqrt(2.0 / math.pi)
    return 0.5 * x * (1.0 + jnp.tanh(c * (x + 0.044715 * (x * x * x))))


class _Group:
    def __init__(self, src, dst, base, sizes, tick_rows, n_ticks):
        self.src, self.dst, self.base, self.sizes = src, dst, base, sizes
        self.tick_rows, self.n_ticks = tick_rows, n_ticks

    def rows(self, i):
        if isinstance(i, int):
            return self.base + sum(self.sizes[:i]), self.sizes[i]
        assert len(set(self.sizes)) == 1
        return self.base + i * self.sizes[0], self.sizes[0]

    def copy(self, start, size, sem):
        if not isinstance(start, int):
            start = pl.multiple_of(start, 8)
        rows = pl.ds(start, size)
        return pltpu.make_async_copy(self.src.at[rows], self.dst.at[rows], sem)

    def bulk(self, i, sem):
        start, size = self.rows(i)
        head = self.n_ticks * self.tick_rows
        return self.copy(start + head, size - head, sem)

    def tick(self, i, j, sem):
        start, _ = self.rows(i)
        return self.copy(start + j * self.tick_rows, self.tick_rows, sem)

    def wait(self, i, sem):
        self.copy(*self.rows(i), sem).wait()

    def after_ticks(self, lhs):
        zero = pltpu.bitcast(self.dst[_spare_rows(self.dst), 0:128], _BF16)
        reps = (lhs.shape[0] // zero.shape[0], lhs.shape[1] // zero.shape[1])
        return lhs + jnp.tile(zero, reps)


def _spare_rows(buf):
    n = 32 // buf.dtype.itemsize
    return pl.ds(buf.shape[0] - n, n)


def _slot_sem(sems, phase, i):
    ring = _SLOTS + 1
    first = (phase * _SLOTS) % ring
    k = first + i
    if isinstance(k, int):
        return sems.at[k % ring]
    return sems.at[jnp.where(k >= ring, k - ring, k)]


def _stream_step(sems, phase, arriving, following, i, piece, carry, step):
    sem_in, sem_out = _slot_sem(sems, phase, i), _slot_sem(sems, phase + 1, i)
    part = tick = 0
    waits = [op for op in step if op.isdigit()]
    waited = -1
    for op in step:
        if op.isdigit() and arriving is not None:
            waits.pop(0)
            upto = min(max(waited, 0) + int(op), arriving.n_ticks)
            for j in range(waited, upto if waits else arriving.n_ticks):
                copy = arriving.bulk(i, sem_in) if j < 0 else arriving.tick(i, j, sem_in)
                copy.wait()
            waited = upto
        elif op in "ST" and i >= len(following.sizes) if isinstance(i, int) else False:
            pass
        elif op == "S":
            following.bulk(i, sem_out).start(priority=1)
        elif op == "T":
            tick += 1
            last = tick == step.count("T")
            for j in range(tick - 1, following.n_ticks if last else min(tick, following.n_ticks)):
                following.tick(i, j, sem_out).start()
        elif op == "P" and piece is not None:
            carry = piece(i, part, carry, following.after_ticks)
            part += 1
    return carry


def _stream_phase(sems, phase, arriving, following, piece=None, carry=0,
                  unroll=_UNROLL, step=_STEP):
    if unroll == _SLOTS:
        for i in range(_SLOTS):
            carry = _stream_step(sems, phase, arriving, following, i, piece, carry, step)
        return carry

    def body(o, c):
        for u in range(unroll):
            c = _stream_step(sems, phase, arriving, following, o * unroll + u,
                             piece, c, step)
        return c

    return lax.fori_loop(0, _SLOTS // unroll, body, carry)


def _kernel(x_hbm, ckv_hbm, wq_hbm, wuk_hbm, wuv_hbm, wo_hbm, w3_hbm, w4_hbm,
            c_hbm, wmod_hbm, o_ref,
            x_v, c_v, wmod_v, wq_v, wuk_v, wuv_v, wo_v, w3_v, w4_v, ckv_v,
            mod_v, h_v, q_v, qabs32_v, qabs_v, s_v, lat_v, ctx_v, sems,
            *, B, H, Sk, D, M, F):
    NP = H // 2
    KC = Sk // _PIECES

    def halves(src, dst, tick_rows, n_ticks, base=0, rows=None):
        rows = src.shape[0] if rows is None else rows
        slot = rows // (2 * _SLOTS)
        return [_Group(src, dst, base + k * _SLOTS * slot, [slot] * _SLOTS,
                       tick_rows, n_ticks) for k in range(2)]

    g_mod = halves(wmod_hbm, wmod_v, 8, 12 // _SLOTS)
    g_q = halves(wq_hbm.bitcast(jnp.uint32), wq_v, 2 * _TICK_KIB, _TICKS)
    g_uk = halves(wuk_hbm.bitcast(jnp.uint32), wuk_v, 2 * _TICK_KIB, _TICKS)
    g_uv = halves(wuv_hbm.bitcast(jnp.uint32), wuv_v, 2 * _TICK_KIB, _TICKS)
    g_o = halves(wo_hbm, wo_v, _TICK_KIB, _TICKS)
    g_kv = lambda b: halves(ckv_hbm, ckv_v, _KV_TICK_KIB, _KV_TICKS, b * Sk, Sk)
    g_3 = _Group(w3_hbm, w3_v, 0, [M // _SLOTS] * _SLOTS, 16, 12 // _SLOTS)
    g_4a = _Group(w4_hbm, w4_v, 0, [_W4A // _SLOTS] * _SLOTS, _W4A_TICK, _TICKS)
    g_4b = _Group(w4_hbm, w4_v, _W4A, _W4B, _W4B_TICK, 5)
    g_mod[0].n_ticks = 0

    cp_c = pltpu.make_async_copy(c_hbm, c_v, sems.at[_SLOTS])
    cp_x = pltpu.make_async_copy(x_hbm, x_v, sems.at[_SLOTS])
    _stream_phase(sems, _SLOTS, None, g_mod[0], unroll=_SLOTS)
    cp_c.start()
    cp_x.start()
    for buf in (wmod_v, wq_v, wuk_v, wuv_v, wo_v, w3_v, w4_v, ckv_v):
        spare = _spare_rows(buf)
        buf[spare, 0:128] = jnp.zeros((spare.size, 128), buf.dtype)


    def pair_weights(w_v, pair, half):
        words = w_v[pl.ds(pair + half * (M // 2) * NP, M // 2, stride=NP), :]
        return [pltpu.bitcast(w, _F32).astype(_BF16)
                for w in (words << 16, words & jnp.uint32(0xFFFF0000))]

    def head_of_all_batches(head):
        return pl.ds(head, B, stride=H)

    def twice(v):
        return jnp.concatenate([v, v], axis=0).astype(_BF16)

    def pair_of(i, j):
        pair = i * _PARTS + j
        return pair, pl.ds(pl.multiple_of(pair * 2 * B, 2 * B), 2 * B)

    cp_c.wait()
    cp_x.wait()
    cf = c_v[...].astype(_F32)
    sc = twice(cf * jax.nn.sigmoid(cf))
    _stream_phase(sems, 0, g_mod[0], g_mod[1], step=_STEP_IDLE)

    def mod_piece(half):
        def piece(i, j, carry, pin):
            n = i * _PARTS + j
            rows = slice(half * (M // 2), (half + 1) * (M // 2))
            if n < 12:
                cols = slice(n * (M // 2), (n + 1) * (M // 2))
                part = _dot(pin(sc[:, rows]), wmod_v[rows, cols])[:B]
                mod_v[:, cols] = part if half == 0 else mod_v[:, cols] + part
            elif n == 12 and half == 1:
                x0 = x_v[...].astype(_F32)
                h = _layernorm(x0) * (1.0 + mod_v[:, M:2 * M]) + mod_v[:, 0:M]
                h_v[...] = twice(h)
            return carry
        return piece

    _stream_phase(sems, 1, g_mod[1], g_q[0], mod_piece(0), unroll=_SLOTS)
    _stream_phase(sems, 2, g_q[0], g_q[1], mod_piece(1), unroll=_SLOTS)

    def q_piece(half):
        def piece(i, j, carry, pin):
            pair, rows = pair_of(i, j)
            h = pin(h_v[:, half * (M // 2):(half + 1) * (M // 2)])
            part = jnp.concatenate(
                [_dot(h, w)[:B] for w in pair_weights(wq_v, pair, half)], axis=0)
            q_v[rows, :] = part if half == 0 else q_v[rows, :] + part
            return carry
        return piece

    _stream_phase(sems, 3, g_q[1], g_uk[0], q_piece(0))
    _stream_phase(sems, 4, g_uk[0], g_uk[1], q_piece(1))

    qk_scale = D ** -0.5 * math.log2(math.e)

    def qabs_piece(half):
        def piece(i, j, carry, pin):
            pair, rows = pair_of(i, j)
            q = pin(q_v[rows, :].astype(_BF16))
            for p, w in enumerate(pair_weights(wuk_v, pair, half)):
                r = _dot_nt(q, w)[p * B:(p + 1) * B] * qk_scale
                for k in range(M // 256):
                    qabs32_v[half * (M // 256) + k, head_of_all_batches(2 * pair + p), :] = (
                        r[:, k * 128:(k + 1) * 128])
            return carry
        return piece

    _stream_phase(sems, 5, g_uk[1], g_kv(0)[0], qabs_piece(0))
    _stream_phase(sems, 6, g_kv(0)[0], g_kv(0)[1], qabs_piece(1))
    for k in range(M // 128):
        qabs_v[:, k * 128:(k + 1) * 128] = qabs32_v[k].astype(_BF16)

    def head_rows(b):
        return pl.ds(pl.multiple_of(b * H, H), H)

    def keys(b, n):
        return ckv_v[pl.ds(pl.multiple_of(b * Sk + n * KC, KC), KC), :]

    def score_chunk(b, n, m, pin):
        s = _dot_nt(pin(qabs_v[head_rows(b), :]), keys(b, n))
        s_v[b % 2, n] = s
        for t in range(0, KC, 128):
            m = jnp.maximum(m, s[:, t:t + 128])
        return m

    def value_chunk(b, n, s, m, l, acc, pin):
        p = [jnp.exp2(s[:, t:t + 128] - m) for t in range(0, KC, 128)]
        for pt in p:
            l = l + pt
        return l, acc + _dot(pin(jnp.concatenate(p, axis=1).astype(_BF16)), keys(b, n))

    def row_max(m):
        return jnp.broadcast_to(jnp.max(m, axis=-1, keepdims=True), (H, 128))

    def store_lat(b, l, acc):
        lat = acc / jnp.sum(l, axis=-1, keepdims=True)
        for k in range(M // 128):
            lat_v[k, head_rows(b), :] = lat[:, k * 128:(k + 1) * 128]

    m_init = jnp.full((H, 128), -jnp.inf, _F32)
    l_init, acc_init = jnp.zeros((H, 128), _F32), jnp.zeros((H, M), _F32)

    def attend(b, groups, m_prev, with_values=True):
        def piece(half):
            scores = []

            def run(i, j, carry, pin):
                if groups[half + 1].dst is ckv_v:
                    pin = lambda lhs: lhs
                m, l, acc = carry
                first = (half * _SLOTS + i) * (_PARTS // 2)
                n = first + j // 2
                if j % 4 == 0 and with_values:
                    scores[:] = [s_v[(b - 1) % 2, n + k] for k in range(2)]
                if j % 2 == 1:
                    m = score_chunk(b, n, m, pin)
                elif with_values:
                    l, acc = value_chunk(b - 1, n, scores[j // 2 % 2], m_prev, l, acc, pin)
                return m, l, acc
            return run

        carry = (m_init, l_init, acc_init) if with_values else (m_init, 0, 0)
        for half in range(2):
            carry = _stream_phase(sems, 7 + 2 * b + half, groups[half], groups[half + 1],
                                  piece(half), carry, step=_STEP_ATTN)
        m, l, acc = carry
        if with_values:
            store_lat(b - 1, l, acc)
        return row_max(m)

    def kv_groups(b):
        return [g_kv(b)[1]] + g_kv(b + 1)

    m = attend(0, kv_groups(0), None, with_values=False)
    m = lax.fori_loop(1, B - 1, lambda b, m: attend(b, kv_groups(b), m), m)
    m = attend(B - 1, [g_kv(B - 1)[1]] + g_uv, m)
    l, acc = _stream_phase(
        sems, 7 + 2 * B, g_uv[1], g_o[0],
        lambda i, j, c, pin: value_chunk(B - 1, i * _PARTS + j,
                                    s_v[(B - 1) % 2, i * _PARTS + j], m, *c, pin),
        (l_init, acc_init))
    store_lat(B - 1, l, acc)

    def ctx_piece(k):
        def piece(i, j, acc, pin):
            pair, _ = pair_of(k * _SLOTS // 2, (i * _PARTS + j) // 2)
            half = j % 2
            lat = jnp.concatenate([jnp.concatenate(
                [lat_v[half * (M // 256) + t, head_of_all_batches(2 * pair + p), :]
                 for t in range(M // 256)], axis=1) for p in range(2)], axis=0)
            lat = pin(lat.astype(_BF16))
            part = jnp.concatenate(
                [_dot(lat, w)[p * B:(p + 1) * B]
                 for p, w in enumerate(pair_weights(wuv_v, pair, half))], axis=1)
            if half == 0:
                return part
            ctx_v[pair] = acc + part
            return acc
        return piece

    zero_pair = jnp.zeros((B, 2 * D), _F32)
    _stream_phase(sems, 8 + 2 * B, g_o[0], g_o[1], ctx_piece(0), zero_pair)
    _stream_phase(sems, 9 + 2 * B, g_o[1], g_3, ctx_piece(1), zero_pair)

    def mlp_piece(i, j, carry, pin):
        n = i * _PARTS + j
        if n < NP // 2:
            for pair in (2 * n, 2 * n + 1):
                ctx = pin(twice(ctx_v[pair]))
                carry = carry + _dot(ctx, wo_v[pair * 2 * D:(pair + 1) * 2 * D, :])[:B]
        elif n == NP // 2:
            x1 = x_v[...].astype(_F32) + mod_v[:, 2 * M:3 * M] * carry
            hb = _layernorm(x1) * (1.0 + mod_v[:, 4 * M:5 * M]) + mod_v[:, 3 * M:4 * M]
            carry = x1, hb, twice(_layernorm(hb)), jnp.zeros((B, F), _F32)
        elif (w3_done[0] + 1) * 128 <= (i + 1) * M // _SLOTS:
            carry = hidden_chunk(carry, pin)
        return carry

    w3_done = [0]

    def hidden_chunk(carry, pin):
        x1, hb, ln, pre = carry
        start, size = w3_done[0] * 128, 128
        w3_done[0] += 1
        pre = pre + _dot(pin(ln[:, start:start + size]), w3_v[start:start + size, :])[:B]
        return x1, hb, ln, pre

    carry = _stream_phase(sems, 10 + 2 * B, g_3, g_4a, mlp_piece,
                          jnp.zeros((B, M), _F32), unroll=_SLOTS, step=_STEP_MLP)
    while w3_done[0] < M // 128:
        carry = hidden_chunk(carry, lambda lhs: lhs)
    x1, y, _, pre = carry
    g = twice(_gelu(pre))

    def down(y, start, stop, pin):
        return y + _dot(pin(g[:, start:stop]), w4_v[start:stop, :])[:B]

    def down_piece(i, j, y, pin):
        lo, hi = ((k * _W4A // _SLOTS) // 128 for k in (i, i + 1))
        lo, hi = (lo + (hi - lo) * k // _PARTS for k in (j, j + 1))
        return down(y, lo * 128, hi * 128, pin) if hi > lo else y

    y = _stream_phase(sems, 11 + 2 * B, g_4a, g_4b, down_piece, y, unroll=_SLOTS,
                      step=_STEP_MLP)
    for i in range(len(g_4b.sizes)):
        start, size = g_4b.rows(i)
        g_4b.wait(i, _slot_sem(sems, 12 + 2 * B, i))
        y = down(y, start, start + size, lambda lhs: lhs)
    o_ref[...] = (x1 + mod_v[:, 5 * M:6 * M] * y).astype(o_ref.dtype)


@jax.jit
def pallas_adaLN_cond__compressed_kv_cla__mixer_s_mlp__decode_kernel(
    A_x: jax.Array,
    A_c_kv: jax.Array,
    A_w_q: jax.Array,
    A_w_uk: jax.Array,
    A_w_uv: jax.Array,
    A_w_o: jax.Array,
    B_x: jax.Array,
    B_w1: jax.Array,
    B_w2: jax.Array,
    B_w3: jax.Array,
    B_w4: jax.Array,
    c: jax.Array,
    w_mod: jax.Array,
):
    del B_x, B_w1, B_w2
    B, Sq, M = A_x.shape
    _, Sk, Dc = A_c_kv.shape
    _, H, D = A_w_q.shape
    F = B_w3.shape[1]
    assert Sq == 1 and Dc == M and D == 128 and B == 8

    x = A_x.reshape(B, M)
    wq = A_w_q.reshape(M * H, D)
    wuk = A_w_uk.reshape(Dc * H, D)
    wuv = A_w_uv.reshape(Dc * H, D)
    wo = A_w_o.reshape(H * D, M)
    ckv = A_c_kv.reshape(B * Sk, Dc)

    hbm = pl.BlockSpec(memory_space=pl.ANY)
    vmem = lambda a: pltpu.VMEM(a.shape, a.dtype)
    spare = lambda a: pltpu.VMEM((a.shape[0] + 16, a.shape[1]), a.dtype)
    words = lambda a: pltpu.VMEM((a.shape[0] // 2 + 8, a.shape[1]), jnp.uint32)
    out = pl.pallas_call(
        functools.partial(_kernel, B=B, H=H, Sk=Sk, D=D, M=M, F=F),
        out_shape=jax.ShapeDtypeStruct(x.shape, x.dtype),
        in_specs=[hbm] * 10,
        out_specs=pl.BlockSpec(memory_space=pltpu.VMEM),
        scratch_shapes=[
            vmem(x), vmem(c), spare(w_mod), words(wq), words(wuk), words(wuv),
            spare(wo), spare(B_w3), spare(B_w4), spare(ckv),
            pltpu.VMEM((B, 6 * M), _F32),
            pltpu.VMEM((2 * B, M), _BF16),
            pltpu.VMEM((H * B, D), _F32),
            pltpu.VMEM((Dc // 128, B * H, 128), _F32),
            pltpu.VMEM((B * H, Dc), _BF16),
            pltpu.VMEM((2, _PIECES, H, Sk // _PIECES), _F32),
            pltpu.VMEM((Dc // 128, B * H, 128), _F32),
            pltpu.VMEM((H // 2, B, 2 * D), _F32),
            pltpu.SemaphoreType.DMA((_SLOTS + 1,)),
        ],
        compiler_params=pltpu.CompilerParams(vmem_limit_bytes=100 * 1024 * 1024),
    )(x, ckv, wq, wuk, wuv, wo, B_w3, B_w4, c, w_mod)
    return out.reshape(A_x.shape)
```

```python
import functools
import math

import jax
import jax.numpy as jnp
from jax import lax
import jax.experimental.pallas as pl
import jax.experimental.pallas.tpu as pltpu

_F32 = jnp.float32
_BF16 = jnp.bfloat16
_NT = (((1,), (1,)), ((), ()))

_SLOTS = 4
_STEP = "1T2T2STPPTPPT"
_STEP_ATTN = "0T2T3STPPTPPT"
_UNROLL = 1
_TICKS = _STEP.count("T")
_PARTS = _STEP.count("P")
_PIECES = _SLOTS * _PARTS
_TICK_KIB = 40
_KV_TICKS = 5
_KV_TICK_KIB = 40
_STEP_MOD0 = "0T1T1T1STPPPPT"
_STEP_MOD1 = "0T2T1T2STPPPPT"
_STEP_MLP = _STEP
_STEP_IDLE = "0T2T1ST"
_W4A, _W4A_TICK = 1536, 24
_W4B, _W4B_TICK = [256], 16


def _dot(a, b):
    return jnp.dot(a, b, preferred_element_type=_F32)


def _dot_nt(a, b):
    return lax.dot_general(a, b, _NT, preferred_element_type=_F32)


def _layernorm(x, eps=1e-5):
    m = jnp.mean(x, axis=-1, keepdims=True)
    d = x - m
    v = jnp.mean(d * d, axis=-1, keepdims=True)
    return d / jnp.sqrt(v + eps)


def _gelu(x):
    c = math.sqrt(2.0 / math.pi)
    return 0.5 * x * (1.0 + jnp.tanh(c * (x + 0.044715 * (x * x * x))))


class _Group:
    def __init__(self, src, dst, base, sizes, tick_rows, n_ticks):
        self.src, self.dst, self.base, self.sizes = src, dst, base, sizes
        self.tick_rows, self.n_ticks = tick_rows, n_ticks

    def rows(self, i):
        if isinstance(i, int):
            return self.base + sum(self.sizes[:i]), self.sizes[i]
        assert len(set(self.sizes)) == 1
        return self.base + i * self.sizes[0], self.sizes[0]

    def copy(self, start, size, sem):
        if not isinstance(start, int):
            start = pl.multiple_of(start, 8)
        rows = pl.ds(start, size)
        return pltpu.make_async_copy(self.src.at[rows], self.dst.at[rows], sem)

    def bulk(self, i, sem):
        start, size = self.rows(i)
        head = self.n_ticks * self.tick_rows
        return self.copy(start + head, size - head, sem)

    def tick(self, i, j, sem):
        start, _ = self.rows(i)
        return self.copy(start + j * self.tick_rows, self.tick_rows, sem)

    def wait(self, i, sem):
        self.copy(*self.rows(i), sem).wait()

    def after_ticks(self, lhs):
        zero = pltpu.bitcast(self.dst[_spare_rows(self.dst), 0:128], _BF16)
        reps = (lhs.shape[0] // zero.shape[0], lhs.shape[1] // zero.shape[1])
        return lhs + jnp.tile(zero, reps)


def _spare_rows(buf):
    n = 32 // buf.dtype.itemsize
    return pl.ds(buf.shape[0] - n, n)


def _slot_sem(sems, phase, i):
    ring = _SLOTS + 1
    first = (phase * _SLOTS) % ring
    k = first + i
    if isinstance(k, int):
        return sems.at[k % ring]
    return sems.at[jnp.where(k >= ring, k - ring, k)]


def _stream_step(sems, phase, arriving, following, i, piece, carry, step):
    sem_in, sem_out = _slot_sem(sems, phase, i), _slot_sem(sems, phase + 1, i)
    part = tick = 0
    waits = [op for op in step if op.isdigit()]
    waited = -1
    for op in step:
        if op.isdigit() and arriving is not None:
            waits.pop(0)
            upto = min(max(waited, 0) + int(op), arriving.n_ticks)
            for j in range(waited, upto if waits else arriving.n_ticks):
                copy = arriving.bulk(i, sem_in) if j < 0 else arriving.tick(i, j, sem_in)
                copy.wait()
            waited = upto
        elif op in "ST" and i >= len(following.sizes) if isinstance(i, int) else False:
            pass
        elif op == "S":
            following.bulk(i, sem_out).start(priority=1)
        elif op == "T":
            tick += 1
            last = tick == step.count("T")
            for j in range(tick - 1, following.n_ticks if last else min(tick, following.n_ticks)):
                following.tick(i, j, sem_out).start()
        elif op == "P" and piece is not None:
            carry = piece(i, part, carry, following.after_ticks)
            part += 1
    return carry


def _stream_phase(sems, phase, arriving, following, piece=None, carry=0,
                  unroll=_UNROLL, step=_STEP):
    if unroll == _SLOTS:
        for i in range(_SLOTS):
            carry = _stream_step(sems, phase, arriving, following, i, piece, carry, step)
        return carry

    def body(o, c):
        for u in range(unroll):
            c = _stream_step(sems, phase, arriving, following, o * unroll + u,
                             piece, c, step)
        return c

    return lax.fori_loop(0, _SLOTS // unroll, body, carry)


def _kernel(x_hbm, ckv_hbm, wq_hbm, wuk_hbm, wuv_hbm, wo_hbm, w3_hbm, w4_hbm,
            c_hbm, wmod_hbm, o_ref,
            x_v, c_v, wmod_v, wq_v, wuk_v, wuv_v, wo_v, w3_v, w4_v, ckv_v,
            mod_v, h_v, q_v, qabs32_v, qabs_v, s_v, lat_v, ctx_v, sems,
            *, B, H, Sk, D, M, F):
    NP = H // 2
    KC = Sk // _PIECES

    def halves(src, dst, tick_rows, n_ticks, base=0, rows=None):
        rows = src.shape[0] if rows is None else rows
        slot = rows // (2 * _SLOTS)
        return [_Group(src, dst, base + k * _SLOTS * slot, [slot] * _SLOTS,
                       tick_rows, n_ticks) for k in range(2)]

    g_mod = halves(wmod_hbm, wmod_v, 8, 12 // _SLOTS)
    g_q = halves(wq_hbm.bitcast(jnp.uint32), wq_v, 2 * _TICK_KIB, _TICKS)
    g_uk = halves(wuk_hbm.bitcast(jnp.uint32), wuk_v, 2 * _TICK_KIB, _TICKS)
    g_uv = halves(wuv_hbm.bitcast(jnp.uint32), wuv_v, 2 * _TICK_KIB, _TICKS)
    g_o = halves(wo_hbm, wo_v, _TICK_KIB, _TICKS)
    g_kv = lambda b: halves(ckv_hbm, ckv_v, _KV_TICK_KIB, _KV_TICKS, b * Sk, Sk)
    g_3 = _Group(w3_hbm, w3_v, 0, [M // _SLOTS] * _SLOTS, 16, 12 // _SLOTS)
    g_4a = _Group(w4_hbm, w4_v, 0, [_W4A // _SLOTS] * _SLOTS, _W4A_TICK, _TICKS)
    g_4b = _Group(w4_hbm, w4_v, _W4A, _W4B, _W4B_TICK, 5)


    cp_c = pltpu.make_async_copy(c_hbm, c_v, sems.at[_SLOTS])
    cp_x = pltpu.make_async_copy(x_hbm, x_v, sems.at[_SLOTS])
    _stream_phase(sems, _SLOTS, None, g_mod[0], unroll=_SLOTS)
    cp_c.start()
    cp_x.start()
    for buf in (wmod_v, wq_v, wuk_v, wuv_v, wo_v, w3_v, w4_v, ckv_v):
        spare = _spare_rows(buf)
        buf[spare, 0:128] = jnp.zeros((spare.size, 128), buf.dtype)


    def pair_weights(w_v, pair, half):
        words = w_v[pl.ds(pair + half * (M // 2) * NP, M // 2, stride=NP), :]
        return [pltpu.bitcast(w, _F32).astype(_BF16)
                for w in (words << 16, words & jnp.uint32(0xFFFF0000))]

    def head_of_all_batches(head):
        return pl.ds(head, B, stride=H)

    def twice(v):
        return jnp.concatenate([v, v], axis=0).astype(_BF16)

    def pair_of(i, j):
        pair = i * _PARTS + j
        return pair, pl.ds(pl.multiple_of(pair * 2 * B, 2 * B), 2 * B)

    cp_c.wait()
    cp_x.wait()
    cf = c_v[...].astype(_F32)
    sc = twice(cf * jax.nn.sigmoid(cf))
    _stream_phase(sems, 0, g_mod[0], g_mod[1], step=_STEP_IDLE)

    def mod_piece(half):
        def piece(i, j, carry, pin):
            n = i * _PARTS + j
            rows = slice(half * (M // 2), (half + 1) * (M // 2))
            if n < 12:
                cols = slice(n * (M // 2), (n + 1) * (M // 2))
                part = _dot(pin(sc[:, rows]), wmod_v[rows, cols])[:B]
                mod_v[:, cols] = part if half == 0 else mod_v[:, cols] + part
            elif n == 12 and half == 1:
                x0 = x_v[...].astype(_F32)
                h = _layernorm(x0) * (1.0 + mod_v[:, M:2 * M]) + mod_v[:, 0:M]
                h_v[...] = twice(h)
            return carry
        return piece

    _stream_phase(sems, 1, g_mod[1], g_q[0], mod_piece(0), unroll=_SLOTS, step=_STEP_MOD0)
    _stream_phase(sems, 2, g_q[0], g_q[1], mod_piece(1), unroll=_SLOTS, step=_STEP_MOD1)

    def q_piece(half):
        def piece(i, j, carry, pin):
            pair, rows = pair_of(i, j)
            h = pin(h_v[:, half * (M // 2):(half + 1) * (M // 2)])
            part = jnp.concatenate(
                [_dot(h, w)[:B] for w in pair_weights(wq_v, pair, half)], axis=0)
            q_v[rows, :] = part if half == 0 else q_v[rows, :] + part
            return carry
        return piece

    _stream_phase(sems, 3, g_q[1], g_uk[0], q_piece(0))
    _stream_phase(sems, 4, g_uk[0], g_uk[1], q_piece(1))

    qk_scale = D ** -0.5 * math.log2(math.e)

    def qabs_piece(half):
        def piece(i, j, carry, pin):
            pair, rows = pair_of(i, j)
            q = pin(q_v[rows, :].astype(_BF16))
            for p, w in enumerate(pair_weights(wuk_v, pair, half)):
                r = _dot_nt(q, w)[p * B:(p + 1) * B] * qk_scale
                for k in range(M // 256):
                    qabs32_v[half * (M // 256) + k, head_of_all_batches(2 * pair + p), :] = (
                        r[:, k * 128:(k + 1) * 128])
            return carry
        return piece

    _stream_phase(sems, 5, g_uk[1], g_kv(0)[0], qabs_piece(0))
    _stream_phase(sems, 6, g_kv(0)[0], g_kv(0)[1], qabs_piece(1))
    for k in range(M // 128):
        qabs_v[:, k * 128:(k + 1) * 128] = qabs32_v[k].astype(_BF16)

    def head_rows(b):
        return pl.ds(pl.multiple_of(b * H, H), H)

    def keys(b, n):
        return ckv_v[pl.ds(pl.multiple_of(b * Sk + n * KC, KC), KC), :]

    def score_chunk(b, n, m, pin):
        s = _dot_nt(pin(qabs_v[head_rows(b), :]), keys(b, n))
        s_v[b % 2, n] = s
        for t in range(0, KC, 128):
            m = jnp.maximum(m, s[:, t:t + 128])
        return m

    def value_chunk(b, n, s, m, l, acc, pin):
        p = [jnp.exp2(s[:, t:t + 128] - m) for t in range(0, KC, 128)]
        for pt in p:
            l = l + pt
        return l, acc + _dot(pin(jnp.concatenate(p, axis=1).astype(_BF16)), keys(b, n))

    def row_max(m):
        return jnp.broadcast_to(jnp.max(m, axis=-1, keepdims=True), (H, 128))

    def store_lat(b, l, acc):
        lat = acc / jnp.sum(l, axis=-1, keepdims=True)
        for k in range(M // 128):
            lat_v[k, head_rows(b), :] = lat[:, k * 128:(k + 1) * 128]

    m_init = jnp.full((H, 128), -jnp.inf, _F32)
    l_init, acc_init = jnp.zeros((H, 128), _F32), jnp.zeros((H, M), _F32)

    def attend(b, groups, m_prev, with_values=True):
        def piece(half):
            scores = []

            def run(i, j, carry, pin):
                if groups[half + 1].dst is ckv_v:
                    pin = lambda lhs: lhs
                m, l, acc = carry
                first = (half * _SLOTS + i) * (_PARTS // 2)
                n = first + j // 2
                if j % 4 == 0 and with_values:
                    scores[:] = [s_v[(b - 1) % 2, n + k] for k in range(2)]
                if j % 2 == 1:
                    m = score_chunk(b, n, m, pin)
                elif with_values:
                    l, acc = value_chunk(b - 1, n, scores[j // 2 % 2], m_prev, l, acc, pin)
                return m, l, acc
            return run

        carry = (m_init, l_init, acc_init) if with_values else (m_init, 0, 0)
        for half in range(2):
            carry = _stream_phase(sems, 7 + 2 * b + half, groups[half], groups[half + 1],
                                  piece(half), carry, step=_STEP_ATTN)
        m, l, acc = carry
        if with_values:
            store_lat(b - 1, l, acc)
        return row_max(m)

    def kv_groups(b):
        return [g_kv(b)[1]] + g_kv(b + 1)

    m = attend(0, kv_groups(0), None, with_values=False)
    m = lax.fori_loop(1, B - 1, lambda b, m: attend(b, kv_groups(b), m), m)
    m = attend(B - 1, [g_kv(B - 1)[1]] + g_uv, m)
    l, acc = _stream_phase(
        sems, 7 + 2 * B, g_uv[1], g_o[0],
        lambda i, j, c, pin: value_chunk(B - 1, i * _PARTS + j,
                                    s_v[(B - 1) % 2, i * _PARTS + j], m, *c, pin),
        (l_init, acc_init))
    store_lat(B - 1, l, acc)

    def ctx_piece(k):
        def piece(i, j, acc, pin):
            pair, _ = pair_of(k * _SLOTS // 2, (i * _PARTS + j) // 2)
            half = j % 2
            lat = jnp.concatenate([jnp.concatenate(
                [lat_v[half * (M // 256) + t, head_of_all_batches(2 * pair + p), :]
                 for t in range(M // 256)], axis=1) for p in range(2)], axis=0)
            lat = pin(lat.astype(_BF16))
            part = jnp.concatenate(
                [_dot(lat, w)[p * B:(p + 1) * B]
                 for p, w in enumerate(pair_weights(wuv_v, pair, half))], axis=1)
            if half == 0:
                return part
            ctx_v[pair] = acc + part
            return acc
        return piece

    zero_pair = jnp.zeros((B, 2 * D), _F32)
    _stream_phase(sems, 8 + 2 * B, g_o[0], g_o[1], ctx_piece(0), zero_pair)
    _stream_phase(sems, 9 + 2 * B, g_o[1], g_3, ctx_piece(1), zero_pair)

    def mlp_piece(i, j, carry, pin):
        n = i * _PARTS + j
        if n < NP // 2:
            for pair in (2 * n, 2 * n + 1):
                ctx = pin(twice(ctx_v[pair]))
                carry = carry + _dot(ctx, wo_v[pair * 2 * D:(pair + 1) * 2 * D, :])[:B]
        elif n == NP // 2:
            x1 = x_v[...].astype(_F32) + mod_v[:, 2 * M:3 * M] * carry
            hb = _layernorm(x1) * (1.0 + mod_v[:, 4 * M:5 * M]) + mod_v[:, 3 * M:4 * M]
            carry = x1, hb, twice(_layernorm(hb)), jnp.zeros((B, F), _F32)
        elif (w3_done[0] + 1) * 128 <= (i + 1) * M // _SLOTS:
            carry = hidden_chunk(carry, pin)
        return carry

    w3_done = [0]

    def hidden_chunk(carry, pin):
        x1, hb, ln, pre = carry
        start, size = w3_done[0] * 128, 128
        w3_done[0] += 1
        pre = pre + _dot(pin(ln[:, start:start + size]), w3_v[start:start + size, :])[:B]
        return x1, hb, ln, pre

    carry = _stream_phase(sems, 10 + 2 * B, g_3, g_4a, mlp_piece,
                          jnp.zeros((B, M), _F32), unroll=_SLOTS, step=_STEP_MLP)
    while w3_done[0] < M // 128:
        carry = hidden_chunk(carry, lambda lhs: lhs)
    x1, y, _, pre = carry
    g = twice(_gelu(pre))

    def down(y, start, stop, pin):
        return y + _dot(pin(g[:, start:stop]), w4_v[start:stop, :])[:B]

    def down_piece(i, j, y, pin):
        lo, hi = ((k * _W4A // _SLOTS) // 128 for k in (i, i + 1))
        lo, hi = (lo + (hi - lo) * k // _PARTS for k in (j, j + 1))
        return down(y, lo * 128, hi * 128, pin) if hi > lo else y

    y = _stream_phase(sems, 11 + 2 * B, g_4a, g_4b, down_piece, y, unroll=_SLOTS,
                      step=_STEP_MLP)
    for i in range(len(g_4b.sizes)):
        start, size = g_4b.rows(i)
        g_4b.wait(i, _slot_sem(sems, 12 + 2 * B, i))
        y = down(y, start, start + size, lambda lhs: lhs)
    o_ref[...] = (x1 + mod_v[:, 5 * M:6 * M] * y).astype(o_ref.dtype)


@jax.jit
def pallas_adaLN_cond__compressed_kv_cla__mixer_s_mlp__decode_kernel(
    A_x: jax.Array,
    A_c_kv: jax.Array,
    A_w_q: jax.Array,
    A_w_uk: jax.Array,
    A_w_uv: jax.Array,
    A_w_o: jax.Array,
    B_x: jax.Array,
    B_w1: jax.Array,
    B_w2: jax.Array,
    B_w3: jax.Array,
    B_w4: jax.Array,
    c: jax.Array,
    w_mod: jax.Array,
):
    del B_x, B_w1, B_w2
    B, Sq, M = A_x.shape
    _, Sk, Dc = A_c_kv.shape
    _, H, D = A_w_q.shape
    F = B_w3.shape[1]
    assert Sq == 1 and Dc == M and D == 128 and B == 8

    x = A_x.reshape(B, M)
    wq = A_w_q.reshape(M * H, D)
    wuk = A_w_uk.reshape(Dc * H, D)
    wuv = A_w_uv.reshape(Dc * H, D)
    wo = A_w_o.reshape(H * D, M)
    ckv = A_c_kv.reshape(B * Sk, Dc)

    hbm = pl.BlockSpec(memory_space=pl.ANY)
    vmem = lambda a: pltpu.VMEM(a.shape, a.dtype)
    spare = lambda a: pltpu.VMEM((a.shape[0] + 16, a.shape[1]), a.dtype)
    words = lambda a: pltpu.VMEM((a.shape[0] // 2 + 8, a.shape[1]), jnp.uint32)
    out = pl.pallas_call(
        functools.partial(_kernel, B=B, H=H, Sk=Sk, D=D, M=M, F=F),
        out_shape=jax.ShapeDtypeStruct(x.shape, x.dtype),
        in_specs=[hbm] * 10,
        out_specs=pl.BlockSpec(memory_space=pltpu.VMEM),
        scratch_shapes=[
            vmem(x), vmem(c), spare(w_mod), words(wq), words(wuk), words(wuv),
            spare(wo), spare(B_w3), spare(B_w4), spare(ckv),
            pltpu.VMEM((B, 6 * M), _F32),
            pltpu.VMEM((2 * B, M), _BF16),
            pltpu.VMEM((H * B, D), _F32),
            pltpu.VMEM((Dc // 128, B * H, 128), _F32),
            pltpu.VMEM((B * H, Dc), _BF16),
            pltpu.VMEM((2, _PIECES, H, Sk // _PIECES), _F32),
            pltpu.VMEM((Dc // 128, B * H, 128), _F32),
            pltpu.VMEM((H // 2, B, 2 * D), _F32),
            pltpu.SemaphoreType.DMA((_SLOTS + 1,)),
        ],
        compiler_params=pltpu.CompilerParams(vmem_limit_bytes=100 * 1024 * 1024),
    )(x, ckv, wq, wuk, wuv, wo, B_w3, B_w4, c, w_mod)
    return out.reshape(A_x.shape)
```

```python
import functools
import math

import jax
import jax.numpy as jnp
from jax import lax
import jax.experimental.pallas as pl
import jax.experimental.pallas.tpu as pltpu

_F32 = jnp.float32
_BF16 = jnp.bfloat16
_NT = (((1,), (1,)), ((), ()))

_SLOTS = 4
_STEP = "1T2T2STPPTPPT"
_STEP_ATTN = "0T2T3STPPTPPT"
_UNROLL = 1
_PARTS = _STEP.count("P")
_PIECES = _SLOTS * _PARTS
_TICK_KIB = [32, 32, 32, 32, 48]
_KV_TICK_KIB = [48, 32, 24, 40, 64]
_STEP_MOD0 = "0T1T1T1STPPPPT"
_STEP_MOD1 = "0T2T1T2STPPPPT"
_STEP_MLP = _STEP
_STEP_IDLE = "0T2T1ST"
_W4A, _W4A_TICK = 1536, [24] * 5
_W4B, _W4B_TICK = [256], [16] * 5
_W3_TICK = [8] * 5


def _dot(a, b):
    return jnp.dot(a, b, preferred_element_type=_F32)


def _dot_nt(a, b):
    return lax.dot_general(a, b, _NT, preferred_element_type=_F32)


def _layernorm(x, eps=1e-5):
    m = jnp.mean(x, axis=-1, keepdims=True)
    d = x - m
    v = jnp.mean(d * d, axis=-1, keepdims=True)
    return d / jnp.sqrt(v + eps)


def _gelu(x):
    c = math.sqrt(2.0 / math.pi)
    return 0.5 * x * (1.0 + jnp.tanh(c * (x + 0.044715 * (x * x * x))))


class _Group:
    def __init__(self, src, dst, base, sizes, tick_rows):
        self.src, self.dst, self.base, self.sizes = src, dst, base, sizes
        self.tick_rows, self.n_ticks = tick_rows, len(tick_rows)

    def rows(self, i):
        if isinstance(i, int):
            return self.base + sum(self.sizes[:i]), self.sizes[i]
        assert len(set(self.sizes)) == 1
        return self.base + i * self.sizes[0], self.sizes[0]

    def copy(self, start, size, sem):
        if not isinstance(start, int):
            start = pl.multiple_of(start, 8)
        rows = pl.ds(start, size)
        return pltpu.make_async_copy(self.src.at[rows], self.dst.at[rows], sem)

    def bulk(self, i, sem):
        start, size = self.rows(i)
        head = sum(self.tick_rows)
        return self.copy(start + head, size - head, sem)

    def tick(self, i, j, sem):
        start, _ = self.rows(i)
        return self.copy(start + sum(self.tick_rows[:j]), self.tick_rows[j], sem)

    def wait(self, i, sem):
        self.copy(*self.rows(i), sem).wait()

    def after_ticks(self, lhs):
        zero = pltpu.bitcast(self.dst[_spare_rows(self.dst), 0:128], _BF16)
        reps = (lhs.shape[0] // zero.shape[0], lhs.shape[1] // zero.shape[1])
        return lhs + jnp.tile(zero, reps)


def _spare_rows(buf):
    n = 32 // buf.dtype.itemsize
    return pl.ds(buf.shape[0] - n, n)


def _slot_sem(sems, phase, i):
    ring = _SLOTS + 1
    first = (phase * _SLOTS) % ring
    k = first + i
    if isinstance(k, int):
        return sems.at[k % ring]
    return sems.at[jnp.where(k >= ring, k - ring, k)]


def _stream_step(sems, phase, arriving, following, i, piece, carry, step):
    sem_in, sem_out = _slot_sem(sems, phase, i), _slot_sem(sems, phase + 1, i)
    part = tick = 0
    waits = [op for op in step if op.isdigit()]
    waited = -1
    for op in step:
        if op.isdigit() and arriving is not None:
            waits.pop(0)
            upto = min(max(waited, 0) + int(op), arriving.n_ticks)
            for j in range(waited, upto if waits else arriving.n_ticks):
                copy = arriving.bulk(i, sem_in) if j < 0 else arriving.tick(i, j, sem_in)
                copy.wait()
            waited = upto
        elif op in "ST" and i >= len(following.sizes) if isinstance(i, int) else False:
            pass
        elif op == "S":
            following.bulk(i, sem_out).start(priority=1)
        elif op == "T":
            tick += 1
            last = tick == step.count("T")
            for j in range(tick - 1, following.n_ticks if last else min(tick, following.n_ticks)):
                following.tick(i, j, sem_out).start()
        elif op == "P" and piece is not None:
            carry = piece(i, part, carry, following.after_ticks)
            part += 1
    return carry


def _stream_phase(sems, phase, arriving, following, piece=None, carry=0,
                  unroll=_UNROLL, step=_STEP):
    if unroll == _SLOTS:
        for i in range(_SLOTS):
            carry = _stream_step(sems, phase, arriving, following, i, piece, carry, step)
        return carry

    def body(o, c):
        for u in range(unroll):
            c = _stream_step(sems, phase, arriving, following, o * unroll + u,
                             piece, c, step)
        return c

    return lax.fori_loop(0, _SLOTS // unroll, body, carry)


def _kernel(x_hbm, ckv_hbm, wq_hbm, wuk_hbm, wuv_hbm, wo_hbm, w3_hbm, w4_hbm,
            c_hbm, wmod_hbm, o_ref,
            x_v, c_v, wmod_v, wq_v, wuk_v, wuv_v, wo_v, w3_v, w4_v, ckv_v,
            mod_v, h_v, q_v, qabs32_v, qabs_v, s_v, lat_v, ctx_v, sems,
            *, B, H, Sk, D, M, F):
    NP = H // 2
    KC = Sk // _PIECES

    def halves(src, dst, tick_rows, base=0, rows=None):
        rows = src.shape[0] if rows is None else rows
        slot = rows // (2 * _SLOTS)
        return [_Group(src, dst, base + k * _SLOTS * slot, [slot] * _SLOTS,
                       tick_rows) for k in range(2)]

    g_mod = halves(wmod_hbm, wmod_v, [8] * 3)
    g_q = halves(wq_hbm.bitcast(jnp.uint32), wq_v, [2 * t for t in _TICK_KIB])
    g_uk = halves(wuk_hbm.bitcast(jnp.uint32), wuk_v, [2 * t for t in _TICK_KIB])
    g_uv = halves(wuv_hbm.bitcast(jnp.uint32), wuv_v, [2 * t for t in _TICK_KIB])
    g_o = halves(wo_hbm, wo_v, _TICK_KIB)
    g_kv = lambda b: halves(ckv_hbm, ckv_v, _KV_TICK_KIB, b * Sk, Sk)
    g_3 = _Group(w3_hbm, w3_v, 0, [M // _SLOTS] * _SLOTS, _W3_TICK)
    g_4a = _Group(w4_hbm, w4_v, 0, [_W4A // _SLOTS] * _SLOTS, _W4A_TICK)
    g_4b = _Group(w4_hbm, w4_v, _W4A, _W4B, _W4B_TICK)


    cp_c = pltpu.make_async_copy(c_hbm, c_v, sems.at[_SLOTS])
    cp_x = pltpu.make_async_copy(x_hbm, x_v, sems.at[_SLOTS])
    _stream_phase(sems, _SLOTS, None, g_mod[0], unroll=_SLOTS)
    cp_c.start()
    cp_x.start()
    for buf in (wmod_v, wq_v, wuk_v, wuv_v, wo_v, w3_v, w4_v, ckv_v):
        spare = _spare_rows(buf)
        buf[spare, 0:128] = jnp.zeros((spare.size, 128), buf.dtype)


    def pair_weights(w_v, pair, half):
        words = w_v[pl.ds(pair + half * (M // 2) * NP, M // 2, stride=NP), :]
        return [pltpu.bitcast(w, _F32).astype(_BF16)
                for w in (words << 16, words & jnp.uint32(0xFFFF0000))]

    def head_of_all_batches(head):
        return pl.ds(head, B, stride=H)

    def twice(v):
        return jnp.concatenate([v, v], axis=0).astype(_BF16)

    def pair_of(i, j):
        pair = i * _PARTS + j
        return pair, pl.ds(pl.multiple_of(pair * 2 * B, 2 * B), 2 * B)

    cp_c.wait()
    cp_x.wait()
    cf = c_v[...].astype(_F32)
    sc = twice(cf * jax.nn.sigmoid(cf))
    _stream_phase(sems, 0, g_mod[0], g_mod[1], step=_STEP_IDLE)

    def mod_piece(half):
        def piece(i, j, carry, pin):
            n = i * _PARTS + j
            rows = slice(half * (M // 2), (half + 1) * (M // 2))
            if n < 12:
                cols = slice(n * (M // 2), (n + 1) * (M // 2))
                part = _dot(pin(sc[:, rows]), wmod_v[rows, cols])[:B]
                mod_v[:, cols] = part if half == 0 else mod_v[:, cols] + part
            elif n == 12 and half == 1:
                x0 = x_v[...].astype(_F32)
                h = _layernorm(x0) * (1.0 + mod_v[:, M:2 * M]) + mod_v[:, 0:M]
                h_v[...] = twice(h)
            return carry
        return piece

    _stream_phase(sems, 1, g_mod[1], g_q[0], mod_piece(0), unroll=_SLOTS, step=_STEP_MOD0)
    _stream_phase(sems, 2, g_q[0], g_q[1], mod_piece(1), unroll=_SLOTS, step=_STEP_MOD1)

    def q_piece(half):
        def piece(i, j, carry, pin):
            pair, rows = pair_of(i, j)
            h = pin(h_v[:, half * (M // 2):(half + 1) * (M // 2)])
            part = jnp.concatenate(
                [_dot(h, w)[:B] for w in pair_weights(wq_v, pair, half)], axis=0)
            q_v[rows, :] = part if half == 0 else q_v[rows, :] + part
            return carry
        return piece

    _stream_phase(sems, 3, g_q[1], g_uk[0], q_piece(0))
    _stream_phase(sems, 4, g_uk[0], g_uk[1], q_piece(1))

    qk_scale = D ** -0.5 * math.log2(math.e)

    def qabs_piece(half):
        def piece(i, j, carry, pin):
            pair, rows = pair_of(i, j)
            q = pin(q_v[rows, :].astype(_BF16))
            for p, w in enumerate(pair_weights(wuk_v, pair, half)):
                r = _dot_nt(q, w)[p * B:(p + 1) * B] * qk_scale
                for k in range(M // 256):
                    qabs32_v[half * (M // 256) + k, head_of_all_batches(2 * pair + p), :] = (
                        r[:, k * 128:(k + 1) * 128])
            return carry
        return piece

    _stream_phase(sems, 5, g_uk[1], g_kv(0)[0], qabs_piece(0))
    _stream_phase(sems, 6, g_kv(0)[0], g_kv(0)[1], qabs_piece(1))
    for k in range(M // 128):
        qabs_v[:, k * 128:(k + 1) * 128] = qabs32_v[k].astype(_BF16)

    def head_rows(b):
        return pl.ds(pl.multiple_of(b * H, H), H)

    def keys(b, n):
        return ckv_v[pl.ds(pl.multiple_of(b * Sk + n * KC, KC), KC), :]

    def score_chunk(b, n, m, pin):
        s = _dot_nt(pin(qabs_v[head_rows(b), :]), keys(b, n))
        s_v[b % 2, n] = s
        for t in range(0, KC, 128):
            m = jnp.maximum(m, s[:, t:t + 128])
        return m

    def value_chunk(b, n, s, m, l, acc, pin):
        p = [jnp.exp2(s[:, t:t + 128] - m) for t in range(0, KC, 128)]
        for pt in p:
            l = l + pt
        return l, acc + _dot(pin(jnp.concatenate(p, axis=1).astype(_BF16)), keys(b, n))

    def row_max(m):
        return jnp.broadcast_to(jnp.max(m, axis=-1, keepdims=True), (H, 128))

    def store_lat(b, l, acc):
        lat = acc / jnp.sum(l, axis=-1, keepdims=True)
        for k in range(M // 128):
            lat_v[k, head_rows(b), :] = lat[:, k * 128:(k + 1) * 128]

    m_init = jnp.full((H, 128), -jnp.inf, _F32)
    l_init, acc_init = jnp.zeros((H, 128), _F32), jnp.zeros((H, M), _F32)

    def attend(b, groups, m_prev, with_values=True):
        def piece(half):
            scores = []

            def run(i, j, carry, pin):
                if groups[half + 1].dst is ckv_v:
                    pin = lambda lhs: lhs
                m, l, acc = carry
                first = (half * _SLOTS + i) * (_PARTS // 2)
                n = first + j // 2
                if j % 4 == 0 and with_values:
                    scores[:] = [s_v[(b - 1) % 2, n + k] for k in range(2)]
                if j % 2 == 1:
                    m = score_chunk(b, n, m, pin)
                elif with_values:
                    l, acc = value_chunk(b - 1, n, scores[j // 2 % 2], m_prev, l, acc, pin)
                return m, l, acc
            return run

        carry = (m_init, l_init, acc_init) if with_values else (m_init, 0, 0)
        for half in range(2):
            carry = _stream_phase(sems, 7 + 2 * b + half, groups[half], groups[half + 1],
                                  piece(half), carry, step=_STEP_ATTN)
        m, l, acc = carry
        if with_values:
            store_lat(b - 1, l, acc)
        return row_max(m)

    def kv_groups(b):
        return [g_kv(b)[1]] + g_kv(b + 1)

    m = attend(0, kv_groups(0), None, with_values=False)
    m = lax.fori_loop(1, B - 1, lambda b, m: attend(b, kv_groups(b), m), m)
    m = attend(B - 1, [g_kv(B - 1)[1]] + g_uv, m)
    l, acc = _stream_phase(
        sems, 7 + 2 * B, g_uv[1], g_o[0],
        lambda i, j, c, pin: value_chunk(B - 1, i * _PARTS + j,
                                    s_v[(B - 1) % 2, i * _PARTS + j], m, *c, pin),
        (l_init, acc_init))
    store_lat(B - 1, l, acc)

    def ctx_piece(k):
        def piece(i, j, acc, pin):
            pair, _ = pair_of(k * _SLOTS // 2, (i * _PARTS + j) // 2)
            half = j % 2
            lat = jnp.concatenate([jnp.concatenate(
                [lat_v[half * (M // 256) + t, head_of_all_batches(2 * pair + p), :]
                 for t in range(M // 256)], axis=1) for p in range(2)], axis=0)
            lat = pin(lat.astype(_BF16))
            part = jnp.concatenate(
                [_dot(lat, w)[p * B:(p + 1) * B]
                 for p, w in enumerate(pair_weights(wuv_v, pair, half))], axis=1)
            if half == 0:
                return part
            ctx_v[pair] = acc + part
            return acc
        return piece

    zero_pair = jnp.zeros((B, 2 * D), _F32)
    _stream_phase(sems, 8 + 2 * B, g_o[0], g_o[1], ctx_piece(0), zero_pair)
    _stream_phase(sems, 9 + 2 * B, g_o[1], g_3, ctx_piece(1), zero_pair)

    def mlp_piece(i, j, carry, pin):
        n = i * _PARTS + j
        if n < NP // 2:
            for pair in (2 * n, 2 * n + 1):
                ctx = pin(twice(ctx_v[pair]))
                carry = carry + _dot(ctx, wo_v[pair * 2 * D:(pair + 1) * 2 * D, :])[:B]
        elif n == NP // 2:
            x1 = x_v[...].astype(_F32) + mod_v[:, 2 * M:3 * M] * carry
            hb = _layernorm(x1) * (1.0 + mod_v[:, 4 * M:5 * M]) + mod_v[:, 3 * M:4 * M]
            carry = x1, hb, twice(_layernorm(hb)), jnp.zeros((B, F), _F32)
        elif (w3_done[0] + 1) * 128 <= (i + 1) * M // _SLOTS:
            carry = hidden_chunk(carry, pin)
        return carry

    w3_done = [0]

    def hidden_chunk(carry, pin):
        x1, hb, ln, pre = carry
        start, size = w3_done[0] * 128, 128
        w3_done[0] += 1
        pre = pre + _dot(pin(ln[:, start:start + size]), w3_v[start:start + size, :])[:B]
        return x1, hb, ln, pre

    carry = _stream_phase(sems, 10 + 2 * B, g_3, g_4a, mlp_piece,
                          jnp.zeros((B, M), _F32), unroll=_SLOTS, step=_STEP_MLP)
    while w3_done[0] < M // 128:
        carry = hidden_chunk(carry, lambda lhs: lhs)
    x1, y, _, pre = carry
    g = twice(_gelu(pre))

    def down(y, start, stop, pin):
        return y + _dot(pin(g[:, start:stop]), w4_v[start:stop, :])[:B]

    def down_piece(i, j, y, pin):
        lo, hi = ((k * _W4A // _SLOTS) // 128 for k in (i, i + 1))
        lo, hi = (lo + (hi - lo) * k // _PARTS for k in (j, j + 1))
        return down(y, lo * 128, hi * 128, pin) if hi > lo else y

    y = _stream_phase(sems, 11 + 2 * B, g_4a, g_4b, down_piece, y, unroll=_SLOTS,
                      step=_STEP_MLP)
    for i in range(len(g_4b.sizes)):
        start, size = g_4b.rows(i)
        g_4b.wait(i, _slot_sem(sems, 12 + 2 * B, i))
        y = down(y, start, start + size, lambda lhs: lhs)
    o_ref[...] = (x1 + mod_v[:, 5 * M:6 * M] * y).astype(o_ref.dtype)


@jax.jit
def pallas_adaLN_cond__compressed_kv_cla__mixer_s_mlp__decode_kernel(
    A_x: jax.Array,
    A_c_kv: jax.Array,
    A_w_q: jax.Array,
    A_w_uk: jax.Array,
    A_w_uv: jax.Array,
    A_w_o: jax.Array,
    B_x: jax.Array,
    B_w1: jax.Array,
    B_w2: jax.Array,
    B_w3: jax.Array,
    B_w4: jax.Array,
    c: jax.Array,
    w_mod: jax.Array,
):
    del B_x, B_w1, B_w2
    B, Sq, M = A_x.shape
    _, Sk, Dc = A_c_kv.shape
    _, H, D = A_w_q.shape
    F = B_w3.shape[1]
    assert Sq == 1 and Dc == M and D == 128 and B == 8

    x = A_x.reshape(B, M)
    wq = A_w_q.reshape(M * H, D)
    wuk = A_w_uk.reshape(Dc * H, D)
    wuv = A_w_uv.reshape(Dc * H, D)
    wo = A_w_o.reshape(H * D, M)
    ckv = A_c_kv.reshape(B * Sk, Dc)

    hbm = pl.BlockSpec(memory_space=pl.ANY)
    vmem = lambda a: pltpu.VMEM(a.shape, a.dtype)
    spare = lambda a: pltpu.VMEM((a.shape[0] + 16, a.shape[1]), a.dtype)
    words = lambda a: pltpu.VMEM((a.shape[0] // 2 + 8, a.shape[1]), jnp.uint32)
    out = pl.pallas_call(
        functools.partial(_kernel, B=B, H=H, Sk=Sk, D=D, M=M, F=F),
        out_shape=jax.ShapeDtypeStruct(x.shape, x.dtype),
        in_specs=[hbm] * 10,
        out_specs=pl.BlockSpec(memory_space=pltpu.VMEM),
        scratch_shapes=[
            vmem(x), vmem(c), spare(w_mod), words(wq), words(wuk), words(wuv),
            spare(wo), spare(B_w3), spare(B_w4), spare(ckv),
            pltpu.VMEM((B, 6 * M), _F32),
            pltpu.VMEM((2 * B, M), _BF16),
            pltpu.VMEM((H * B, D), _F32),
            pltpu.VMEM((Dc // 128, B * H, 128), _F32),
            pltpu.VMEM((B * H, Dc), _BF16),
            pltpu.VMEM((2, _PIECES, H, Sk // _PIECES), _F32),
            pltpu.VMEM((Dc // 128, B * H, 128), _F32),
            pltpu.VMEM((H // 2, B, 2 * D), _F32),
            pltpu.SemaphoreType.DMA((_SLOTS + 1,)),
        ],
        compiler_params=pltpu.CompilerParams(
            vmem_limit_bytes=100 * 1024 * 1024,
            disable_semaphore_checks=True),
    )(x, ckv, wq, wuk, wuv, wo, B_w3, B_w4, c, w_mod)
    return out.reshape(A_x.shape)
```

```python
import functools
import math

import jax
import jax.numpy as jnp
from jax import lax
import jax.experimental.pallas as pl
import jax.experimental.pallas.tpu as pltpu

_F32 = jnp.float32
_BF16 = jnp.bfloat16

_SLOTS = 4
_RING = _SLOTS + 1
_PARTS = 4
_PIECES = _SLOTS * _PARTS

_STEP = "1T2T2STPPTPPT"
_STEP_ATTN = "0T2T3STPPTPPT"
_STEP_IDLE = "0T2T1ST"
_STEP_MOD = ("0T1T1T1STPPPPT", "0T2T1T2STPPPPT")

_TICK_KIB = (32, 32, 32, 32, 48)
_KV_TICK_KIB = (48, 32, 24, 40, 64)


def _dot(a, b):
    return jnp.dot(a, b, preferred_element_type=_F32)


def _dot_nt(a, b):
    return lax.dot_general(a, b, (((1,), (1,)), ((), ())),
                           preferred_element_type=_F32)


def _layernorm(x, eps=1e-5):
    d = x - jnp.mean(x, axis=-1, keepdims=True)
    return d / jnp.sqrt(jnp.mean(d * d, axis=-1, keepdims=True) + eps)


def _gelu(x):
    c = math.sqrt(2.0 / math.pi)
    return 0.5 * x * (1.0 + jnp.tanh(c * (x + 0.044715 * (x * x * x))))


def _lhs(v):
    return jnp.concatenate([v, v], axis=0).astype(_BF16)


def _identity(v):
    return v


def _spare_rows(buf):
    n = 32 // buf.dtype.itemsize
    return pl.ds(buf.shape[0] - n, n)


class _Group:
    def __init__(self, src, dst, base, slot_rows, tick_rows, n_slots=_SLOTS):
        self.src, self.dst, self.base = src, dst, base
        self.slot_rows, self.tick_rows, self.n_slots = slot_rows, tick_rows, n_slots
        self.n_ticks = len(tick_rows)

    def _copy(self, i, offset, size, sem):
        start = self.base + i * self.slot_rows + offset
        if not isinstance(start, int):
            start = pl.multiple_of(start, 8)
        rows = pl.ds(start, size)
        return pltpu.make_async_copy(self.src.at[rows], self.dst.at[rows], sem)

    def bulk(self, i, sem):
        head = sum(self.tick_rows)
        return self._copy(i, head, self.slot_rows - head, sem)

    def tick(self, i, j, sem):
        return self._copy(i, sum(self.tick_rows[:j]), self.tick_rows[j], sem)

    def slot(self, i, sem):
        return self._copy(i, 0, self.slot_rows, sem)

    def after_ticks(self, lhs):
        zero = pltpu.bitcast(self.dst[_spare_rows(self.dst), 0:128], _BF16)
        reps = (lhs.shape[0] // zero.shape[0], lhs.shape[1] // zero.shape[1])
        return lhs + jnp.tile(zero, reps)


def _slot_sem(sems, phase, i):
    k = (phase * _SLOTS) % _RING + i
    if isinstance(k, int):
        return sems.at[k % _RING]
    return sems.at[jnp.where(k >= _RING, k - _RING, k)]


def _stream_step(program, sems, phase, arriving, following, i, piece, carry):
    sem_in, sem_out = _slot_sem(sems, phase, i), _slot_sem(sems, phase + 1, i)
    request = following.n_slots == _SLOTS or i < following.n_slots
    waits_left = sum(op.isdigit() for op in program)
    waited, started, part = -1, 0, 0
    for pos, op in enumerate(program):
        if op.isdigit():
            waits_left -= 1
            upto = min(max(waited, 0) + int(op), arriving.n_ticks)
            for j in range(waited, upto if waits_left else arriving.n_ticks):
                copy = arriving.bulk(i, sem_in) if j < 0 else arriving.tick(i, j, sem_in)
                copy.wait()
            waited = upto
        elif op == "S" and request:
            following.bulk(i, sem_out).start(priority=1)
        elif op == "T" and request:
            upto = started + 1 if "T" in program[pos + 1:] else following.n_ticks
            for j in range(started, min(upto, following.n_ticks)):
                following.tick(i, j, sem_out).start()
            started = upto
        elif op == "P":
            carry = piece(i, part, carry, following.after_ticks)
            part += 1
    return carry


def _stream_phase(program, sems, phase, arriving, following, piece=None, carry=0,
                  unroll=False):
    step = functools.partial(_stream_step, program, sems, phase, arriving, following)
    if unroll:
        for i in range(_SLOTS):
            carry = step(i, piece, carry)
        return carry
    return lax.fori_loop(0, _SLOTS, lambda i, c: step(i, piece, c), carry)


def _kernel(x_hbm, ckv_hbm, wq_hbm, wuk_hbm, wuv_hbm, wo_hbm, w3_hbm, w4_hbm,
            c_hbm, wmod_hbm, o_ref,
            x_v, c_v, wmod_v, wq_v, wuk_v, wuv_v, wo_v, w3_v, w4_v, ckv_v,
            mod_v, h_v, q_v, qabs32_v, qabs_v, s_v, lat_v, ctx_v, sems,
            *, B, H, Sk, D, M, F):
    NP = H // 2
    KC = Sk // _PIECES
    assert NP == _PIECES

    def halves(src, dst, tick_rows, base=0, rows=None):
        slot = (src.shape[0] if rows is None else rows) // (2 * _SLOTS)
        return [_Group(src, dst, base + k * _SLOTS * slot, slot, tick_rows)
                for k in range(2)]

    def head_weights(src, dst):
        return halves(src.bitcast(jnp.uint32), dst, [2 * t for t in _TICK_KIB])

    def g_kv(b):
        return halves(ckv_hbm, ckv_v, _KV_TICK_KIB, b * Sk, Sk)

    g_mod = halves(wmod_hbm, wmod_v, [8] * 3)
    g_q = head_weights(wq_hbm, wq_v)
    g_uk = head_weights(wuk_hbm, wuk_v)
    g_uv = head_weights(wuv_hbm, wuv_v)
    g_o = halves(wo_hbm, wo_v, _TICK_KIB)
    g_3 = _Group(w3_hbm, w3_v, 0, M // _SLOTS, [8] * 5)
    f_last = 256
    g_4 = _Group(w4_hbm, w4_v, 0, (F - f_last) // _SLOTS, [24] * 5)
    g_end = _Group(w4_hbm, w4_v, F - f_last, f_last, [16] * 5, n_slots=1)

    _stream_phase("ST", sems, -1, None, g_mod[0], unroll=True)
    cp_c = pltpu.make_async_copy(c_hbm, c_v, sems.at[_SLOTS])
    cp_x = pltpu.make_async_copy(x_hbm, x_v, sems.at[_SLOTS])
    cp_c.start()
    cp_x.start()
    for buf in (wmod_v, wq_v, wuk_v, wuv_v, wo_v, w3_v, w4_v, ckv_v):
        spare = _spare_rows(buf)
        buf[spare, 0:128] = jnp.zeros((spare.size, 128), buf.dtype)

    def pair_weights(w_v, pair, half):
        words = w_v[pl.ds(pair + half * (M // 2) * NP, M // 2, stride=NP), :]
        return [pltpu.bitcast(w, _F32).astype(_BF16)
                for w in (words << 16, words & jnp.uint32(0xFFFF0000))]

    def pair_rows(pair):
        return pl.ds(pl.multiple_of(pair * 2 * B, 2 * B), 2 * B)

    def head_rows(head):
        return pl.ds(head, B, stride=H)

    def batch_rows(b):
        return pl.ds(b * H if isinstance(b, int) else pl.multiple_of(b * H, H), H)

    cp_c.wait()
    cp_x.wait()
    cf = c_v[...].astype(_F32)
    sc = _lhs(cf * jax.nn.sigmoid(cf))
    _stream_phase(_STEP_IDLE, sems, 0, g_mod[0], g_mod[1])

    def mod(k):
        return mod_v[:, k * M:(k + 1) * M]

    def mod_piece(half, i, j, carry, pin):
        n = i * _PARTS + j
        rows = slice(half * (M // 2), (half + 1) * (M // 2))
        if n < 12:
            cols = slice(n * (M // 2), (n + 1) * (M // 2))
            part = _dot(pin(sc[:, rows]), wmod_v[rows, cols])[:B]
            mod_v[:, cols] = part if half == 0 else mod_v[:, cols] + part
        elif n == 12 and half == 1:
            h_v[...] = _lhs(_layernorm(x_v[...].astype(_F32)) * (1.0 + mod(1)) + mod(0))
        return carry

    _stream_phase(_STEP_MOD[0], sems, 1, g_mod[1], g_q[0],
                  functools.partial(mod_piece, 0), unroll=True)
    _stream_phase(_STEP_MOD[1], sems, 2, g_q[0], g_q[1],
                  functools.partial(mod_piece, 1), unroll=True)

    def q_piece(half, i, j, carry, pin):
        pair = i * _PARTS + j
        h = pin(h_v[:, half * (M // 2):(half + 1) * (M // 2)])
        part = jnp.concatenate(
            [_dot(h, w)[:B] for w in pair_weights(wq_v, pair, half)], axis=0)
        rows = pair_rows(pair)
        q_v[rows, :] = part if half == 0 else q_v[rows, :] + part
        return carry

    _stream_phase(_STEP, sems, 3, g_q[1], g_uk[0], functools.partial(q_piece, 0))
    _stream_phase(_STEP, sems, 4, g_uk[0], g_uk[1], functools.partial(q_piece, 1))

    def qabs_piece(half, i, j, carry, pin):
        pair = i * _PARTS + j
        q = pin(q_v[pair_rows(pair), :].astype(_BF16))
        for p, w in enumerate(pair_weights(wuk_v, pair, half)):
            r = _dot_nt(q, w)[p * B:(p + 1) * B] * (D ** -0.5 * math.log2(math.e))
            for k in range(M // 256):
                qabs32_v[half * (M // 256) + k, head_rows(2 * pair + p), :] = (
                    r[:, k * 128:(k + 1) * 128])
        return carry

    _stream_phase(_STEP, sems, 5, g_uk[1], g_kv(0)[0], functools.partial(qabs_piece, 0))
    _stream_phase(_STEP, sems, 6, *g_kv(0), functools.partial(qabs_piece, 1))
    for k in range(M // 128):
        qabs_v[:, k * 128:(k + 1) * 128] = qabs32_v[k, 0:B * H, :].astype(_BF16)

    def keys(b, n):
        return ckv_v[pl.ds(pl.multiple_of(b * Sk + n * KC, KC), KC), :]

    def score_chunk(b, n, m, pin):
        s = _dot_nt(pin(qabs_v[batch_rows(b), :]), keys(b, n))
        s_v[b % 2, n] = s
        for t in range(0, KC, 128):
            m = jnp.maximum(m, s[:, t:t + 128])
        return m

    def value_chunk(b, n, s, m, l, acc, pin):
        p = [jnp.exp2(s[:, t:t + 128] - m) for t in range(0, KC, 128)]
        for pt in p:
            l = l + pt
        p = pin(jnp.concatenate(p, axis=1).astype(_BF16))
        return l, acc + _dot(p, keys(b, n))

    def store_lat(b, l, acc):
        lat = acc / jnp.sum(l, axis=-1, keepdims=True)
        for k in range(M // 128):
            lat_v[k, batch_rows(b), :] = lat[:, k * 128:(k + 1) * 128]

    m_init = jnp.full((H, 128), -jnp.inf, _F32)
    l_init, acc_init = jnp.zeros((H, 128), _F32), jnp.zeros((H, M), _F32)

    def attend(b, groups, m_prev):
        scores = []

        def piece(half, i, j, carry, pin):
            m, l, acc = carry
            if groups[half + 1].dst is ckv_v:
                pin = _identity
            n = (half * _SLOTS + i) * (_PARTS // 2) + j // 2
            if j % 2 == 1:
                m = score_chunk(b, n, m, pin)
            elif m_prev is not None:
                if j == 0:
                    scores[:] = [s_v[(b - 1) % 2, n + k] for k in range(_PARTS // 2)]
                l, acc = value_chunk(b - 1, n, scores[j // 2], m_prev, l, acc, pin)
            return m, l, acc

        carry = (m_init, 0, 0) if m_prev is None else (m_init, l_init, acc_init)
        for half in range(2):
            carry = _stream_phase(_STEP_ATTN, sems, 7 + 2 * b + half, groups[half],
                                  groups[half + 1], functools.partial(piece, half), carry)
        m, l, acc = carry
        if m_prev is not None:
            store_lat(b - 1, l, acc)
        return jnp.broadcast_to(jnp.max(m, axis=-1, keepdims=True), (H, 128))

    def kv_groups(b):
        return [g_kv(b)[1]] + g_kv(b + 1)

    def last_values(i, j, carry, pin):
        n = i * _PARTS + j
        return value_chunk(B - 1, n, s_v[(B - 1) % 2, n], m_last, *carry, pin)

    m = attend(0, kv_groups(0), None)
    m = lax.fori_loop(1, B - 1, lambda b, m: attend(b, kv_groups(b), m), m)
    m_last = attend(B - 1, [g_kv(B - 1)[1]] + g_uv, m)
    store_lat(B - 1, *_stream_phase(_STEP, sems, 7 + 2 * B, g_uv[1], g_o[0],
                                    last_values, (l_init, acc_init)))

    def ctx_piece(k, i, j, acc, pin):
        pair, half = (k * _PIECES + i * _PARTS + j) // 2, j % 2
        lat = jnp.concatenate([jnp.concatenate(
            [lat_v[half * (M // 256) + t, head_rows(2 * pair + p), :]
             for t in range(M // 256)], axis=1) for p in range(2)], axis=0)
        lat = pin(lat.astype(_BF16))
        part = jnp.concatenate(
            [_dot(lat, w)[p * B:(p + 1) * B]
             for p, w in enumerate(pair_weights(wuv_v, pair, half))], axis=1)
        if half == 0:
            return part
        ctx_v[pair] = acc + part
        return acc

    ctx_init = jnp.zeros((B, 2 * D), _F32)
    _stream_phase(_STEP, sems, 8 + 2 * B, g_o[0], g_o[1],
                  functools.partial(ctx_piece, 0), ctx_init)
    _stream_phase(_STEP, sems, 9 + 2 * B, g_o[1], g_3,
                  functools.partial(ctx_piece, 1), ctx_init)

    def up_piece(i, j, carry, pin):
        n = i * _PARTS + j
        if n < NP // 2:
            for pair in (2 * n, 2 * n + 1):
                w = wo_v[pair * 2 * D:(pair + 1) * 2 * D, :]
                carry = carry + _dot(pin(_lhs(ctx_v[pair])), w)[:B]
        elif n == NP // 2:
            x1 = x_v[...].astype(_F32) + mod(2) * carry
            hb = _layernorm(x1) * (1.0 + mod(4)) + mod(3)
            carry = x1, hb, _lhs(_layernorm(hb)), jnp.zeros((B, F), _F32)
        elif n - NP // 2 <= _SLOTS:
            k = n - NP // 2 - 1
            assert k <= i
            x1, hb, ln, pre = carry
            rows = slice(k * g_3.slot_rows, (k + 1) * g_3.slot_rows)
            carry = x1, hb, ln, pre + _dot(pin(ln[:, rows]), w3_v[rows, :])[:B]
        return carry

    x1, y, _, pre = _stream_phase(_STEP, sems, 10 + 2 * B, g_3, g_4, up_piece,
                                  jnp.zeros((B, M), _F32), unroll=True)
    g = _lhs(_gelu(pre))

    def down_piece(i, j, y, pin):
        if (j + 1) * 128 > g_4.slot_rows:
            return y
        rows = slice(i * g_4.slot_rows + j * 128, i * g_4.slot_rows + (j + 1) * 128)
        return y + _dot(pin(g[:, rows]), w4_v[rows, :])[:B]

    assert g_4.slot_rows % 128 == 0 and g_4.slot_rows <= 128 * _PARTS
    y = _stream_phase(_STEP, sems, 11 + 2 * B, g_4, g_end, down_piece, y, unroll=True)
    g_end.slot(0, _slot_sem(sems, 12 + 2 * B, 0)).wait()
    y = y + _dot(g[:, F - f_last:], w4_v[F - f_last:F, :])[:B]
    o_ref[...] = (x1 + mod(5) * y).astype(o_ref.dtype)


@jax.jit
def pallas_adaLN_cond__compressed_kv_cla__mixer_s_mlp__decode_kernel(
    A_x: jax.Array,
    A_c_kv: jax.Array,
    A_w_q: jax.Array,
    A_w_uk: jax.Array,
    A_w_uv: jax.Array,
    A_w_o: jax.Array,
    B_x: jax.Array,
    B_w1: jax.Array,
    B_w2: jax.Array,
    B_w3: jax.Array,
    B_w4: jax.Array,
    c: jax.Array,
    w_mod: jax.Array,
):
    del B_x, B_w1, B_w2
    B, Sq, M = A_x.shape
    _, Sk, Dc = A_c_kv.shape
    _, H, D = A_w_q.shape
    F = B_w3.shape[1]
    assert Sq == 1 and Dc == M and D == 128 and B == 8

    x = A_x.reshape(B, M)
    ckv = A_c_kv.reshape(B * Sk, Dc)
    wq = A_w_q.reshape(M * H, D)
    wuk = A_w_uk.reshape(Dc * H, D)
    wuv = A_w_uv.reshape(Dc * H, D)
    wo = A_w_o.reshape(H * D, M)

    def streamed(a):
        return pltpu.VMEM((a.shape[0] + 16, a.shape[1]), a.dtype)

    def streamed_words(a):
        return pltpu.VMEM((a.shape[0] // 2 + 16, a.shape[1]), jnp.uint32)

    out = pl.pallas_call(
        functools.partial(_kernel, B=B, H=H, Sk=Sk, D=D, M=M, F=F),
        out_shape=jax.ShapeDtypeStruct(x.shape, x.dtype),
        in_specs=[pl.BlockSpec(memory_space=pl.ANY)] * 10,
        out_specs=pl.BlockSpec(memory_space=pltpu.VMEM),
        scratch_shapes=[
            pltpu.VMEM(x.shape, x.dtype), pltpu.VMEM(c.shape, c.dtype),
            streamed(w_mod), streamed_words(wq), streamed_words(wuk),
            streamed_words(wuv), streamed(wo), streamed(B_w3), streamed(B_w4),
            streamed(ckv),
            pltpu.VMEM((B, 6 * M), _F32),
            pltpu.VMEM((2 * B, M), _BF16),
            pltpu.VMEM((H * B, D), _F32),
            pltpu.VMEM((Dc // 128, (B + 1) * H, 128), _F32),
            pltpu.VMEM((B * H, Dc), _BF16),
            pltpu.VMEM((2, _PIECES, H, Sk // _PIECES), _F32),
            pltpu.VMEM((Dc // 128, (B + 1) * H, 128), _F32),
            pltpu.VMEM((H // 2, B, 2 * D), _F32),
            pltpu.SemaphoreType.DMA((_RING,)),
        ],
        compiler_params=pltpu.CompilerParams(
            vmem_limit_bytes=100 * 1024 * 1024,
            disable_semaphore_checks=True,
        ),
    )(x, ckv, wq, wuk, wuv, wo, B_w3, B_w4, c, w_mod)
    return out.reshape(A_x.shape)
```

```python
import functools
import math

import jax
import jax.numpy as jnp
from jax import lax
import jax.experimental.pallas as pl
import jax.experimental.pallas.tpu as pltpu

_F32 = jnp.float32
_BF16 = jnp.bfloat16

_SLOTS = 4
_RING = _SLOTS + 1
_PARTS = 4
_PIECES = _SLOTS * _PARTS

_STEP = "1T2T2STPPTPPT"
_STEP_ATTN = "bTPbT9STPPTPT"
_STEP_MLP = "1T2T2STPPTPPT"
_STEP_IDLE = "0T2T1ST"
_STEP_MOD = ("0T1T1T1STPPPPT", "0T2T1T2STPPPPT")

_TICK_KIB = (32, 32, 32, 32, 48)
_KV_TICK_KIB = (48, 32, 24, 40, 64)


def _dot(a, b):
    return jnp.dot(a, b, preferred_element_type=_F32)


def _dot_nt(a, b):
    return lax.dot_general(a, b, (((1,), (1,)), ((), ())),
                           preferred_element_type=_F32)


def _layernorm(x, eps=1e-5):
    d = x - jnp.mean(x, axis=-1, keepdims=True)
    return d / jnp.sqrt(jnp.mean(d * d, axis=-1, keepdims=True) + eps)


def _gelu(x):
    c = math.sqrt(2.0 / math.pi)
    return 0.5 * x * (1.0 + jnp.tanh(c * (x + 0.044715 * (x * x * x))))


def _lhs(v):
    return jnp.concatenate([v, v], axis=0).astype(_BF16)


def _identity(v):
    return v


def _spare_rows(buf):
    n = 32 // buf.dtype.itemsize
    return pl.ds(buf.shape[0] - n, n)


class _Group:
    def __init__(self, src, dst, base, slot_rows, tick_rows, n_slots=_SLOTS):
        self.src, self.dst, self.base = src, dst, base
        self.slot_rows, self.tick_rows, self.n_slots = slot_rows, tick_rows, n_slots
        self.n_ticks = len(tick_rows)

    def _copy(self, i, offset, size, sem):
        start = self.base + i * self.slot_rows + offset
        if not isinstance(start, int):
            start = pl.multiple_of(start, 8)
        rows = pl.ds(start, size)
        return pltpu.make_async_copy(self.src.at[rows], self.dst.at[rows], sem)

    def bulk(self, i, sem):
        head = sum(self.tick_rows)
        return self._copy(i, head, self.slot_rows - head, sem)

    def tick(self, i, j, sem):
        return self._copy(i, sum(self.tick_rows[:j]), self.tick_rows[j], sem)

    def slot(self, i, sem):
        return self._copy(i, 0, self.slot_rows, sem)

    def after_ticks(self, lhs):
        zero = pltpu.bitcast(self.dst[_spare_rows(self.dst), 0:128], _BF16)
        reps = (lhs.shape[0] // zero.shape[0], lhs.shape[1] // zero.shape[1])
        return lhs + jnp.tile(zero, reps)


def _slot_sem(sems, phase, i):
    k = (phase * _SLOTS) % _RING + i
    if isinstance(k, int):
        return sems.at[k % _RING]
    return sems.at[jnp.where(k >= _RING, k - _RING, k)]


def _stream_step(program, sems, phase, arriving, following, i, piece, carry):
    sem_in, sem_out = _slot_sem(sems, phase, i), _slot_sem(sems, phase + 1, i)
    request = following.n_slots == _SLOTS or i < following.n_slots
    waits_left = sum(op.isdigit() for op in program)
    bulk_waited, waited, started, part = False, 0, 0, 0
    for pos, op in enumerate(program):
        if op == "b":
            arriving.tick(i, waited, sem_in).wait()
            waited += 1
        elif op.isdigit():
            waits_left -= 1
            if not bulk_waited:
                arriving.bulk(i, sem_in).wait()
                bulk_waited = True
            upto = min(waited + int(op), arriving.n_ticks) if waits_left else arriving.n_ticks
            for j in range(waited, upto):
                arriving.tick(i, j, sem_in).wait()
            waited = upto
        elif op == "S" and request:
            following.bulk(i, sem_out).start(priority=1)
        elif op == "T" and request:
            upto = started + 1 if "T" in program[pos + 1:] else following.n_ticks
            for j in range(started, min(upto, following.n_ticks)):
                following.tick(i, j, sem_out).start()
            started = upto
        elif op == "P":
            carry = piece(i, part, carry, following.after_ticks)
            part += 1
    return carry


def _stream_phase(program, sems, phase, arriving, following, piece=None, carry=0,
                  unroll=False):
    step = functools.partial(_stream_step, program, sems, phase, arriving, following)
    if unroll:
        for i in range(_SLOTS):
            carry = step(i, piece, carry)
        return carry
    return lax.fori_loop(0, _SLOTS, lambda i, c: step(i, piece, c), carry)


def _kernel(x_hbm, ckv_hbm, wq_hbm, wuk_hbm, wuv_hbm, wo_hbm, w3_hbm, w4_hbm,
            c_hbm, wmod_hbm, o_ref,
            x_v, c_v, wmod_v, wq_v, wuk_v, wuv_v, wo_v, w3_v, w4_v, ckv_v,
            mod_v, h_v, q_v, qabs32_v, qabs_v, s_v, lat_v, ctx_v, sems,
            *, B, H, Sk, D, M, F):
    NP = H // 2
    KC = Sk // _PIECES
    assert NP == _PIECES

    def halves(src, dst, tick_rows, base=0, rows=None):
        slot = (src.shape[0] if rows is None else rows) // (2 * _SLOTS)
        return [_Group(src, dst, base + k * _SLOTS * slot, slot, tick_rows)
                for k in range(2)]

    def head_weights(src, dst):
        return halves(src.bitcast(jnp.uint32), dst, [2 * t for t in _TICK_KIB])

    def g_kv(b):
        return halves(ckv_hbm, ckv_v, _KV_TICK_KIB, b * Sk, Sk)

    g_mod = halves(wmod_hbm, wmod_v, [8] * 3)
    g_q = head_weights(wq_hbm, wq_v)
    g_uk = head_weights(wuk_hbm, wuk_v)
    g_uv = head_weights(wuv_hbm, wuv_v)
    g_o = halves(wo_hbm, wo_v, _TICK_KIB)
    g_3 = _Group(w3_hbm, w3_v, 0, M // _SLOTS, [8] * 5)
    f_last = 256
    g_4 = _Group(w4_hbm, w4_v, 0, (F - f_last) // _SLOTS, [24] * 5)
    g_end = _Group(w4_hbm, w4_v, F - f_last, f_last, [16] * 5, n_slots=1)

    _stream_phase("ST", sems, -1, None, g_mod[0], unroll=True)
    cp_c = pltpu.make_async_copy(c_hbm, c_v, sems.at[_SLOTS])
    cp_x = pltpu.make_async_copy(x_hbm, x_v, sems.at[_SLOTS])
    cp_c.start()
    cp_x.start()
    for buf in (wmod_v, wq_v, wuk_v, wuv_v, wo_v, w3_v, w4_v, ckv_v):
        spare = _spare_rows(buf)
        buf[spare, 0:128] = jnp.zeros((spare.size, 128), buf.dtype)

    def pair_weights(w_v, pair, half):
        words = w_v[pl.ds(pair + half * (M // 2) * NP, M // 2, stride=NP), :]
        return [pltpu.bitcast(w, _F32).astype(_BF16)
                for w in (words << 16, words & jnp.uint32(0xFFFF0000))]

    def pair_rows(pair):
        return pl.ds(pl.multiple_of(pair * 2 * B, 2 * B), 2 * B)

    def head_rows(head):
        return pl.ds(head, B, stride=H)

    def batch_rows(b):
        return pl.ds(b * H if isinstance(b, int) else pl.multiple_of(b * H, H), H)

    cp_c.wait()
    cp_x.wait()
    cf = c_v[...].astype(_F32)
    sc = _lhs(cf * jax.nn.sigmoid(cf))
    _stream_phase(_STEP_IDLE, sems, 0, g_mod[0], g_mod[1])

    def mod(k):
        return mod_v[:, k * M:(k + 1) * M]

    def mod_piece(half, i, j, carry, pin):
        n = i * _PARTS + j
        rows = slice(half * (M // 2), (half + 1) * (M // 2))
        if n < 12:
            cols = slice(n * (M // 2), (n + 1) * (M // 2))
            part = _dot(pin(sc[:, rows]), wmod_v[rows, cols])[:B]
            mod_v[:, cols] = part if half == 0 else mod_v[:, cols] + part
        elif n == 12 and half == 1:
            h_v[...] = _lhs(_layernorm(x_v[...].astype(_F32)) * (1.0 + mod(1)) + mod(0))
        return carry

    _stream_phase(_STEP_MOD[0], sems, 1, g_mod[1], g_q[0],
                  functools.partial(mod_piece, 0), unroll=True)
    _stream_phase(_STEP_MOD[1], sems, 2, g_q[0], g_q[1],
                  functools.partial(mod_piece, 1), unroll=True)

    def q_piece(half, i, j, carry, pin):
        pair = i * _PARTS + j
        h = pin(h_v[:, half * (M // 2):(half + 1) * (M // 2)])
        part = jnp.concatenate(
            [_dot(h, w)[:B] for w in pair_weights(wq_v, pair, half)], axis=0)
        rows = pair_rows(pair)
        q_v[rows, :] = part if half == 0 else q_v[rows, :] + part
        return carry

    _stream_phase(_STEP, sems, 3, g_q[1], g_uk[0], functools.partial(q_piece, 0))
    _stream_phase(_STEP, sems, 4, g_uk[0], g_uk[1], functools.partial(q_piece, 1))

    def qabs_piece(half, i, j, carry, pin):
        pair = i * _PARTS + j
        q = pin(q_v[pair_rows(pair), :].astype(_BF16))
        for p, w in enumerate(pair_weights(wuk_v, pair, half)):
            r = _dot_nt(q, w)[p * B:(p + 1) * B] * (D ** -0.5 * math.log2(math.e))
            for k in range(M // 256):
                qabs32_v[half * (M // 256) + k, head_rows(2 * pair + p), :] = (
                    r[:, k * 128:(k + 1) * 128])
        return carry

    _stream_phase(_STEP, sems, 5, g_uk[1], g_kv(0)[0], functools.partial(qabs_piece, 0))
    _stream_phase(_STEP, sems, 6, *g_kv(0), functools.partial(qabs_piece, 1))
    for k in range(M // 128):
        qabs_v[:, k * 128:(k + 1) * 128] = qabs32_v[k, 0:B * H, :].astype(_BF16)

    def keys(b, n):
        return ckv_v[pl.ds(pl.multiple_of(b * Sk + n * KC, KC), KC), :]

    def score_chunk(b, n, m, pin):
        s = _dot_nt(pin(qabs_v[batch_rows(b), :]), keys(b, n))
        s_v[b % 2, n] = s
        for t in range(0, KC, 128):
            m = jnp.maximum(m, s[:, t:t + 128])
        return m

    def value_chunk(b, n, s, m, l, acc, pin):
        p = [jnp.exp2(s[:, t:t + 128] - m) for t in range(0, KC, 128)]
        for pt in p:
            l = l + pt
        p = pin(jnp.concatenate(p, axis=1).astype(_BF16))
        return l, acc + _dot(p, keys(b, n))

    def store_lat(b, l, acc):
        lat = acc / jnp.sum(l, axis=-1, keepdims=True)
        for k in range(M // 128):
            lat_v[k, batch_rows(b), :] = lat[:, k * 128:(k + 1) * 128]

    m_init = jnp.full((H, 128), -jnp.inf, _F32)
    l_init, acc_init = jnp.zeros((H, 128), _F32), jnp.zeros((H, M), _F32)

    def attend(b, groups, m_prev):
        scores = []

        def piece(half, i, j, carry, pin):
            m, l, acc = carry
            if groups[half + 1].dst is ckv_v:
                pin = _identity
            n = (half * _SLOTS + i) * (_PARTS // 2) + j // 2
            if j % 2 == 1:
                m = score_chunk(b, n, m, pin)
            elif m_prev is not None:
                if "b" in _STEP_ATTN:
                    scores[:] = [s_v[(b - 1) % 2, n]] * 2
                elif j == 0:
                    scores[:] = [s_v[(b - 1) % 2, n + k] for k in range(_PARTS // 2)]
                l, acc = value_chunk(b - 1, n, scores[j // 2], m_prev, l, acc, pin)
            return m, l, acc

        carry = (m_init, 0, 0) if m_prev is None else (m_init, l_init, acc_init)
        for half in range(2):
            carry = _stream_phase(_STEP_ATTN, sems, 7 + 2 * b + half, groups[half],
                                  groups[half + 1], functools.partial(piece, half), carry)
        m, l, acc = carry
        if m_prev is not None:
            store_lat(b - 1, l, acc)
        return jnp.broadcast_to(jnp.max(m, axis=-1, keepdims=True), (H, 128))

    def kv_groups(b):
        return [g_kv(b)[1]] + g_kv(b + 1)

    def last_values(i, j, carry, pin):
        n = i * _PARTS + j
        return value_chunk(B - 1, n, s_v[(B - 1) % 2, n], m_last, *carry, pin)

    m = attend(0, kv_groups(0), None)
    m = lax.fori_loop(1, B - 1, lambda b, m: attend(b, kv_groups(b), m), m)
    m_last = attend(B - 1, [g_kv(B - 1)[1]] + g_uv, m)
    store_lat(B - 1, *_stream_phase(_STEP, sems, 7 + 2 * B, g_uv[1], g_o[0],
                                    last_values, (l_init, acc_init)))

    def ctx_piece(k, i, j, acc, pin):
        pair, half = (k * _PIECES + i * _PARTS + j) // 2, j % 2
        lat = jnp.concatenate([jnp.concatenate(
            [lat_v[half * (M // 256) + t, head_rows(2 * pair + p), :]
             for t in range(M // 256)], axis=1) for p in range(2)], axis=0)
        lat = pin(lat.astype(_BF16))
        part = jnp.concatenate(
            [_dot(lat, w)[p * B:(p + 1) * B]
             for p, w in enumerate(pair_weights(wuv_v, pair, half))], axis=1)
        if half == 0:
            return part
        ctx_v[pair] = acc + part
        return acc

    ctx_init = jnp.zeros((B, 2 * D), _F32)
    _stream_phase(_STEP, sems, 8 + 2 * B, g_o[0], g_o[1],
                  functools.partial(ctx_piece, 0), ctx_init)
    _stream_phase(_STEP, sems, 9 + 2 * B, g_o[1], g_3,
                  functools.partial(ctx_piece, 1), ctx_init)

    def up_piece(i, j, carry, pin):
        n = i * _PARTS + j
        if n < NP // 2:
            for pair in (2 * n, 2 * n + 1):
                w = wo_v[pair * 2 * D:(pair + 1) * 2 * D, :]
                carry = carry + _dot(pin(_lhs(ctx_v[pair])), w)[:B]
        elif n == NP // 2:
            x1 = x_v[...].astype(_F32) + mod(2) * carry
            hb = _layernorm(x1) * (1.0 + mod(4)) + mod(3)
            carry = x1, hb, _lhs(_layernorm(hb)), jnp.zeros((B, F), _F32)
        elif n - NP // 2 <= _SLOTS:
            k = n - NP // 2 - 1
            assert k <= i
            x1, hb, ln, pre = carry
            rows = slice(k * g_3.slot_rows, (k + 1) * g_3.slot_rows)
            carry = x1, hb, ln, pre + _dot(pin(ln[:, rows]), w3_v[rows, :])[:B]
        return carry

    x1, y, _, pre = _stream_phase(_STEP_MLP, sems, 10 + 2 * B, g_3, g_4, up_piece,
                                  jnp.zeros((B, M), _F32), unroll=True)
    g = _lhs(_gelu(pre))

    def down_piece(i, j, y, pin):
        if (j + 1) * 128 > g_4.slot_rows:
            return y
        rows = slice(i * g_4.slot_rows + j * 128, i * g_4.slot_rows + (j + 1) * 128)
        return y + _dot(pin(g[:, rows]), w4_v[rows, :])[:B]

    assert g_4.slot_rows % 128 == 0 and g_4.slot_rows <= 128 * _PARTS
    y = _stream_phase(_STEP_MLP, sems, 11 + 2 * B, g_4, g_end, down_piece, y, unroll=True)
    g_end.slot(0, _slot_sem(sems, 12 + 2 * B, 0)).wait()
    y = y + _dot(g[:, F - f_last:], w4_v[F - f_last:F, :])[:B]
    o_ref[...] = (x1 + mod(5) * y).astype(o_ref.dtype)


@jax.jit
def pallas_adaLN_cond__compressed_kv_cla__mixer_s_mlp__decode_kernel(
    A_x: jax.Array,
    A_c_kv: jax.Array,
    A_w_q: jax.Array,
    A_w_uk: jax.Array,
    A_w_uv: jax.Array,
    A_w_o: jax.Array,
    B_x: jax.Array,
    B_w1: jax.Array,
    B_w2: jax.Array,
    B_w3: jax.Array,
    B_w4: jax.Array,
    c: jax.Array,
    w_mod: jax.Array,
):
    del B_x, B_w1, B_w2
    B, Sq, M = A_x.shape
    _, Sk, Dc = A_c_kv.shape
    _, H, D = A_w_q.shape
    F = B_w3.shape[1]
    assert Sq == 1 and Dc == M and D == 128 and B == 8

    x = A_x.reshape(B, M)
    ckv = A_c_kv.reshape(B * Sk, Dc)
    wq = A_w_q.reshape(M * H, D)
    wuk = A_w_uk.reshape(Dc * H, D)
    wuv = A_w_uv.reshape(Dc * H, D)
    wo = A_w_o.reshape(H * D, M)

    def streamed(a):
        return pltpu.VMEM((a.shape[0] + 16, a.shape[1]), a.dtype)

    def streamed_words(a):
        return pltpu.VMEM((a.shape[0] // 2 + 16, a.shape[1]), jnp.uint32)

    out = pl.pallas_call(
        functools.partial(_kernel, B=B, H=H, Sk=Sk, D=D, M=M, F=F),
        out_shape=jax.ShapeDtypeStruct(x.shape, x.dtype),
        in_specs=[pl.BlockSpec(memory_space=pl.ANY)] * 10,
        out_specs=pl.BlockSpec(memory_space=pltpu.VMEM),
        scratch_shapes=[
            pltpu.VMEM(x.shape, x.dtype), pltpu.VMEM(c.shape, c.dtype),
            streamed(w_mod), streamed_words(wq), streamed_words(wuk),
            streamed_words(wuv), streamed(wo), streamed(B_w3), streamed(B_w4),
            streamed(ckv),
            pltpu.VMEM((B, 6 * M), _F32),
            pltpu.VMEM((2 * B, M), _BF16),
            pltpu.VMEM((H * B, D), _F32),
            pltpu.VMEM((Dc // 128, (B + 1) * H, 128), _F32),
            pltpu.VMEM((B * H, Dc), _BF16),
            pltpu.VMEM((2, _PIECES, H, Sk // _PIECES), _F32),
            pltpu.VMEM((Dc // 128, (B + 1) * H, 128), _F32),
            pltpu.VMEM((H // 2, B, 2 * D), _F32),
            pltpu.SemaphoreType.DMA((_RING,)),
        ],
        compiler_params=pltpu.CompilerParams(
            vmem_limit_bytes=100 * 1024 * 1024,
            disable_semaphore_checks=True,
        ),
    )(x, ckv, wq, wuk, wuv, wo, B_w3, B_w4, c, w_mod)
    return out.reshape(A_x.shape)
```

```python
import functools
import math

import jax
import jax.numpy as jnp
from jax import lax
import jax.experimental.pallas as pl
import jax.experimental.pallas.tpu as pltpu

_F32 = jnp.float32
_BF16 = jnp.bfloat16

_SLOTS = 4
_RING = _SLOTS + 1
_PARTS = 4
_PIECES = _SLOTS * _PARTS

_STEP = "1T2T2STPPTPPT"
_STEP_ATTN = "bTPPT0T9STPPT"
_STEP_MLP = "1T2T2STPPTPPT"
_STEP_IDLE = "0T2T1ST"
_STEP_MOD = ("0T1T1T1STPPPPT", "0T2T1T2STPPPPT")

_TICK_KIB = (32, 32, 32, 32, 64)
_KV_TICK_KIB = (32, 32, 32, 32, 64)
_SHIFT_KIB = 48
_MOD_TICK = (8, 8, 8)
_MOD_SHIFT = 0
_W3_TICK = (8, 8, 8, 8, 8)
_W4_SHIFT = 32
_W4_TICK = (16, 16, 32, 32, 32)
_END_TICK = (16, 16, 32)


def _dot(a, b):
    return jnp.dot(a, b, preferred_element_type=_F32)


def _dot_nt(a, b):
    return lax.dot_general(a, b, (((1,), (1,)), ((), ())),
                           preferred_element_type=_F32)


def _layernorm(x, eps=1e-5):
    d = x - jnp.mean(x, axis=-1, keepdims=True)
    return d / jnp.sqrt(jnp.mean(d * d, axis=-1, keepdims=True) + eps)


def _gelu(x):
    c = math.sqrt(2.0 / math.pi)
    return 0.5 * x * (1.0 + jnp.tanh(c * (x + 0.044715 * (x * x * x))))


def _lhs(v):
    return jnp.concatenate([v, v], axis=0).astype(_BF16)


def _identity(v):
    return v


def _spare_rows(buf):
    n = 32 // buf.dtype.itemsize
    return pl.ds(buf.shape[0] - n, n)


class _Group:
    def __init__(self, src, dst, base, slot_rows, tick_rows, n_slots=_SLOTS,
                 cut=0, is_last=False):
        self.src, self.dst, self.base = src, dst, base
        self.slot_rows, self.tick_rows, self.n_slots = slot_rows, tick_rows, n_slots
        self.n_ticks = len(tick_rows)
        self.cut, self.is_last = cut, is_last

    def _copy(self, i, offset, size, sem):
        start = self.base + i * self.slot_rows + offset
        if not isinstance(start, int):
            start = pl.multiple_of(start, 8)
        rows = pl.ds(start, size)
        return pltpu.make_async_copy(self.src.at[rows], self.dst.at[rows], sem)

    def with_bulk(self, i, sem, action):
        head = sum(self.tick_rows)
        size = self.slot_rows - head
        if not self.cut or self.is_last is False:
            return action(self._copy(i, head, size, sem))
        short = self.is_last & (i == self.n_slots - 1)
        if isinstance(short, bool):
            return action(self._copy(i, head, size - self.cut * short, sem))
        pl.when(short)(lambda: action(self._copy(i, head, size - self.cut, sem)))
        pl.when(~short)(lambda: action(self._copy(i, head, size, sem)))

    def tick(self, i, j, sem):
        size = self.tick_rows[j]
        offset = sum(t for k, t in enumerate(self.tick_rows) if (-t, k) < (-size, j))
        return self._copy(i, offset, size, sem)

    def slot(self, i, sem):
        return self._copy(i, 0, self.slot_rows, sem)

    def after_ticks(self, lhs):
        zero = pltpu.bitcast(self.dst[_spare_rows(self.dst), 0:128], _BF16)
        reps = (lhs.shape[0] // zero.shape[0], lhs.shape[1] // zero.shape[1])
        return lhs + jnp.tile(zero, reps)


def _slot_sem(sems, phase, i):
    k = (phase * _SLOTS) % _RING + i
    if isinstance(k, int):
        return sems.at[k % _RING]
    return sems.at[jnp.where(k >= _RING, k - _RING, k)]


def _stream_step(program, sems, phase, arriving, following, i, piece, carry):
    sem_in, sem_out = _slot_sem(sems, phase, i), _slot_sem(sems, phase + 1, i)
    request = following.n_slots == _SLOTS or i < following.n_slots
    waits_left = sum(op.isdigit() for op in program)
    bulk_waited, waited, started, part = False, 0, 0, 0
    for pos, op in enumerate(program):
        if op == "b":
            arriving.tick(i, waited, sem_in).wait()
            waited += 1
        elif op.isdigit():
            waits_left -= 1
            if not bulk_waited:
                arriving.with_bulk(i, sem_in, lambda copy: copy.wait())
                bulk_waited = True
            upto = min(waited + int(op), arriving.n_ticks) if waits_left else arriving.n_ticks
            for j in range(waited, upto):
                arriving.tick(i, j, sem_in).wait()
            waited = upto
        elif op == "S" and request:
            following.with_bulk(i, sem_out, lambda copy: copy.start(priority=1))
        elif op == "T" and request:
            upto = started + 1 if "T" in program[pos + 1:] else following.n_ticks
            for j in range(started, min(upto, following.n_ticks)):
                following.tick(i, j, sem_out).start()
            started = upto
        elif op == "P":
            carry = piece(i, part, carry, following.after_ticks)
            part += 1
    return carry


def _stream_phase(program, sems, phase, arriving, following, piece=None, carry=0,
                  unroll=False):
    step = functools.partial(_stream_step, program, sems, phase, arriving, following)
    if unroll:
        for i in range(_SLOTS):
            carry = step(i, piece, carry)
        return carry
    return lax.fori_loop(0, _SLOTS, lambda i, c: step(i, piece, c), carry)


def _kernel(x_hbm, ckv_hbm, wq_hbm, wuk_hbm, wuv_hbm, wo_hbm, w3_hbm, w4_hbm,
            c_hbm, wmod_hbm, o_ref,
            x_v, c_v, wmod_v, wq_v, wuk_v, wuv_v, wo_v, w3_v, w4_v, ckv_v,
            mod_v, h_v, q_v, qabs32_v, qabs_v, s_v, lat_v, ctx_v, sems,
            *, B, H, Sk, D, M, F):
    NP = H // 2
    KC = Sk // _PIECES
    assert NP == _PIECES

    def halves(src, dst, tick_rows, shift, base=0, rows=None, is_last=True):
        slot = (src.shape[0] if rows is None else rows) // (2 * _SLOTS)
        return [_Group(src, dst, shift + base + k * _SLOTS * slot, slot, tick_rows,
                       cut=shift, is_last=is_last if k == 1 else False)
                for k in range(2)]

    def head_weights(src, dst):
        return halves(src.bitcast(jnp.uint32), dst, [2 * t for t in _TICK_KIB],
                      2 * _SHIFT_KIB)

    def g_kv(b):
        return halves(ckv_hbm, ckv_v, _KV_TICK_KIB, _SHIFT_KIB, b * Sk, Sk, b == B - 1)

    g_mod = halves(wmod_hbm, wmod_v, _MOD_TICK, _MOD_SHIFT)
    g_q = head_weights(wq_hbm, wq_v)
    g_uk = head_weights(wuk_hbm, wuk_v)
    g_uv = head_weights(wuv_hbm, wuv_v)
    g_o = halves(wo_hbm, wo_v, _TICK_KIB, _SHIFT_KIB)
    g_3 = _Group(w3_hbm, w3_v, 0, M // _SLOTS, _W3_TICK)
    f_last = 256
    g_4 = _Group(w4_hbm, w4_v, _W4_SHIFT, (F - f_last) // _SLOTS, _W4_TICK)
    g_end = _Group(w4_hbm, w4_v, F - f_last + _W4_SHIFT, f_last - _W4_SHIFT,
                   _END_TICK, n_slots=1)

    _stream_phase("ST", sems, -1, None, g_mod[0], unroll=True)
    small = [pltpu.make_async_copy(c_hbm, c_v, sems.at[_SLOTS]),
             pltpu.make_async_copy(x_hbm, x_v, sems.at[_SLOTS])]
    for first in (g_mod[0], g_q[0], g_uk[0], g_kv(0)[0], g_uv[0], g_o[0], g_4):
        if first.base:
            rows = pl.ds(0, first.base)
            small.append(pltpu.make_async_copy(
                first.src.at[rows], first.dst.at[rows], sems.at[_SLOTS]))
    for copy in small:
        copy.start()
    for buf in (wmod_v, wq_v, wuk_v, wuv_v, wo_v, w3_v, w4_v, ckv_v):
        spare = _spare_rows(buf)
        buf[spare, 0:128] = jnp.zeros((spare.size, 128), buf.dtype)

    def pair_weights(w_v, pair, half):
        words = w_v[pl.ds(pair + half * (M // 2) * NP, M // 2, stride=NP), :]
        return [pltpu.bitcast(w, _F32).astype(_BF16)
                for w in (words << 16, words & jnp.uint32(0xFFFF0000))]

    def pair_rows(pair):
        return pl.ds(pl.multiple_of(pair * 2 * B, 2 * B), 2 * B)

    def head_rows(head):
        return pl.ds(head, B, stride=H)

    def batch_rows(b):
        return pl.ds(b * H if isinstance(b, int) else pl.multiple_of(b * H, H), H)

    for copy in small:
        copy.wait()
    cf = c_v[...].astype(_F32)
    sc = _lhs(cf * jax.nn.sigmoid(cf))
    _stream_phase(_STEP_IDLE, sems, 0, g_mod[0], g_mod[1])

    def mod(k):
        return mod_v[:, k * M:(k + 1) * M]

    def mod_piece(half, i, j, carry, pin):
        n = i * _PARTS + j
        rows = slice(half * (M // 2), (half + 1) * (M // 2))
        if n < 12:
            cols = slice(n * (M // 2), (n + 1) * (M // 2))
            part = _dot(pin(sc[:, rows]), wmod_v[rows, cols])[:B]
            mod_v[:, cols] = part if half == 0 else mod_v[:, cols] + part
        elif n == 12 and half == 1:
            h_v[...] = _lhs(_layernorm(x_v[...].astype(_F32)) * (1.0 + mod(1)) + mod(0))
        return carry

    _stream_phase(_STEP_MOD[0], sems, 1, g_mod[1], g_q[0],
                  functools.partial(mod_piece, 0), unroll=True)
    _stream_phase(_STEP_MOD[1], sems, 2, g_q[0], g_q[1],
                  functools.partial(mod_piece, 1), unroll=True)

    def q_piece(half, i, j, carry, pin):
        pair = i * _PARTS + j
        h = pin(h_v[:, half * (M // 2):(half + 1) * (M // 2)])
        part = jnp.concatenate(
            [_dot(h, w)[:B] for w in pair_weights(wq_v, pair, half)], axis=0)
        rows = pair_rows(pair)
        q_v[rows, :] = part if half == 0 else q_v[rows, :] + part
        return carry

    _stream_phase(_STEP, sems, 3, g_q[1], g_uk[0], functools.partial(q_piece, 0))
    _stream_phase(_STEP, sems, 4, g_uk[0], g_uk[1], functools.partial(q_piece, 1))

    def qabs_piece(half, i, j, carry, pin):
        pair = i * _PARTS + j
        q = pin(q_v[pair_rows(pair), :].astype(_BF16))
        for p, w in enumerate(pair_weights(wuk_v, pair, half)):
            r = _dot_nt(q, w)[p * B:(p + 1) * B] * (D ** -0.5 * math.log2(math.e))
            for k in range(M // 256):
                qabs32_v[half * (M // 256) + k, head_rows(2 * pair + p), :] = (
                    r[:, k * 128:(k + 1) * 128])
        return carry

    _stream_phase(_STEP, sems, 5, g_uk[1], g_kv(0)[0], functools.partial(qabs_piece, 0))
    _stream_phase(_STEP, sems, 6, *g_kv(0), functools.partial(qabs_piece, 1))
    for k in range(M // 128):
        qabs_v[:, k * 128:(k + 1) * 128] = qabs32_v[k, 0:B * H, :].astype(_BF16)

    def keys(b, n):
        return ckv_v[pl.ds(pl.multiple_of(b * Sk + n * KC, KC), KC), :]

    def score_chunk(b, n, m, pin):
        s = _dot_nt(pin(qabs_v[batch_rows(b), :]), keys(b, n))
        s_v[b % 2, n] = s
        for t in range(0, KC, 128):
            m = jnp.maximum(m, s[:, t:t + 128])
        return m

    def value_chunk(b, n, s, m, l, acc, pin):
        p = [jnp.exp2(s[:, t:t + 128] - m) for t in range(0, KC, 128)]
        for pt in p:
            l = l + pt
        p = pin(jnp.concatenate(p, axis=1).astype(_BF16))
        return l, acc + _dot(p, keys(b, n))

    def store_lat(b, l, acc):
        lat = acc / jnp.sum(l, axis=-1, keepdims=True)
        for k in range(M // 128):
            lat_v[k, batch_rows(b), :] = lat[:, k * 128:(k + 1) * 128]

    m_init = jnp.full((H, 128), -jnp.inf, _F32)
    l_init, acc_init = jnp.zeros((H, 128), _F32), jnp.zeros((H, M), _F32)

    def attend(b, groups, m_prev):
        scores = []

        def piece(half, i, j, carry, pin):
            m, l, acc = carry
            if groups[half + 1].dst is ckv_v:
                pin = _identity
            n = (half * _SLOTS + i) * (_PARTS // 2) + j // 2
            if j % 2 == 1:
                m = score_chunk(b, n, m, pin)
            elif m_prev is not None:
                if "b" in _STEP_ATTN:
                    scores[:] = [s_v[(b - 1) % 2, n]] * 2
                elif j == 0:
                    scores[:] = [s_v[(b - 1) % 2, n + k] for k in range(_PARTS // 2)]
                l, acc = value_chunk(b - 1, n, scores[j // 2], m_prev, l, acc, pin)
            return m, l, acc

        carry = (m_init, 0, 0) if m_prev is None else (m_init, l_init, acc_init)
        for half in range(2):
            carry = _stream_phase(_STEP_ATTN, sems, 7 + 2 * b + half, groups[half],
                                  groups[half + 1], functools.partial(piece, half), carry)
        m, l, acc = carry
        if m_prev is not None:
            store_lat(b - 1, l, acc)
        return jnp.broadcast_to(jnp.max(m, axis=-1, keepdims=True), (H, 128))

    def kv_groups(b):
        return [g_kv(b)[1]] + g_kv(b + 1)

    def last_values(i, j, carry, pin):
        n = i * _PARTS + j
        return value_chunk(B - 1, n, s_v[(B - 1) % 2, n], m_last, *carry, pin)

    m = attend(0, kv_groups(0), None)
    m = lax.fori_loop(1, B - 1, lambda b, m: attend(b, kv_groups(b), m), m)
    m_last = attend(B - 1, [g_kv(B - 1)[1]] + g_uv, m)
    store_lat(B - 1, *_stream_phase(_STEP, sems, 7 + 2 * B, g_uv[1], g_o[0],
                                    last_values, (l_init, acc_init)))

    def ctx_piece(k, i, j, acc, pin):
        pair, half = (k * _PIECES + i * _PARTS + j) // 2, j % 2
        lat = jnp.concatenate([jnp.concatenate(
            [lat_v[half * (M // 256) + t, head_rows(2 * pair + p), :]
             for t in range(M // 256)], axis=1) for p in range(2)], axis=0)
        lat = pin(lat.astype(_BF16))
        part = jnp.concatenate(
            [_dot(lat, w)[p * B:(p + 1) * B]
             for p, w in enumerate(pair_weights(wuv_v, pair, half))], axis=1)
        if half == 0:
            return part
        ctx_v[pair] = acc + part
        return acc

    ctx_init = jnp.zeros((B, 2 * D), _F32)
    _stream_phase(_STEP, sems, 8 + 2 * B, g_o[0], g_o[1],
                  functools.partial(ctx_piece, 0), ctx_init)
    _stream_phase(_STEP, sems, 9 + 2 * B, g_o[1], g_3,
                  functools.partial(ctx_piece, 1), ctx_init)

    def up_piece(i, j, carry, pin):
        n = i * _PARTS + j
        if n < NP // 2:
            for pair in (2 * n, 2 * n + 1):
                w = wo_v[pair * 2 * D:(pair + 1) * 2 * D, :]
                carry = carry + _dot(pin(_lhs(ctx_v[pair])), w)[:B]
        elif n == NP // 2:
            x1 = x_v[...].astype(_F32) + mod(2) * carry
            hb = _layernorm(x1) * (1.0 + mod(4)) + mod(3)
            carry = x1, hb, _lhs(_layernorm(hb)), jnp.zeros((B, F), _F32)
        elif n - NP // 2 <= _SLOTS:
            k = n - NP // 2 - 1
            assert k <= i
            x1, hb, ln, pre = carry
            rows = slice(k * g_3.slot_rows, (k + 1) * g_3.slot_rows)
            carry = x1, hb, ln, pre + _dot(pin(ln[:, rows]), w3_v[rows, :])[:B]
        return carry

    x1, y, _, pre = _stream_phase(_STEP_MLP, sems, 10 + 2 * B, g_3, g_4, up_piece,
                                  jnp.zeros((B, M), _F32), unroll=True)
    g = _lhs(_gelu(pre))

    def down_piece(i, j, y, pin):
        if (j + 1) * 128 > g_4.slot_rows:
            return y
        rows = slice(i * g_4.slot_rows + j * 128, i * g_4.slot_rows + (j + 1) * 128)
        return y + _dot(pin(g[:, rows]), w4_v[rows, :])[:B]

    assert g_4.slot_rows % 128 == 0 and g_4.slot_rows <= 128 * _PARTS
    y = _stream_phase(_STEP_MLP, sems, 11 + 2 * B, g_4, g_end, down_piece, y, unroll=True)
    g_end.slot(0, _slot_sem(sems, 12 + 2 * B, 0)).wait()
    y = y + _dot(g[:, F - f_last:], w4_v[F - f_last:F, :])[:B]
    o_ref[...] = (x1 + mod(5) * y).astype(o_ref.dtype)


@jax.jit
def pallas_adaLN_cond__compressed_kv_cla__mixer_s_mlp__decode_kernel(
    A_x: jax.Array,
    A_c_kv: jax.Array,
    A_w_q: jax.Array,
    A_w_uk: jax.Array,
    A_w_uv: jax.Array,
    A_w_o: jax.Array,
    B_x: jax.Array,
    B_w1: jax.Array,
    B_w2: jax.Array,
    B_w3: jax.Array,
    B_w4: jax.Array,
    c: jax.Array,
    w_mod: jax.Array,
):
    del B_x, B_w1, B_w2
    B, Sq, M = A_x.shape
    _, Sk, Dc = A_c_kv.shape
    _, H, D = A_w_q.shape
    F = B_w3.shape[1]
    assert Sq == 1 and Dc == M and D == 128 and B == 8

    x = A_x.reshape(B, M)
    ckv = A_c_kv.reshape(B * Sk, Dc)
    wq = A_w_q.reshape(M * H, D)
    wuk = A_w_uk.reshape(Dc * H, D)
    wuv = A_w_uv.reshape(Dc * H, D)
    wo = A_w_o.reshape(H * D, M)

    def streamed(a):
        return pltpu.VMEM((a.shape[0] + 16, a.shape[1]), a.dtype)

    def streamed_words(a):
        return pltpu.VMEM((a.shape[0] // 2 + 16, a.shape[1]), jnp.uint32)

    out = pl.pallas_call(
        functools.partial(_kernel, B=B, H=H, Sk=Sk, D=D, M=M, F=F),
        out_shape=jax.ShapeDtypeStruct(x.shape, x.dtype),
        in_specs=[pl.BlockSpec(memory_space=pl.ANY)] * 10,
        out_specs=pl.BlockSpec(memory_space=pltpu.VMEM),
        scratch_shapes=[
            pltpu.VMEM(x.shape, x.dtype), pltpu.VMEM(c.shape, c.dtype),
            streamed(w_mod), streamed_words(wq), streamed_words(wuk),
            streamed_words(wuv), streamed(wo), streamed(B_w3), streamed(B_w4),
            streamed(ckv),
            pltpu.VMEM((B, 6 * M), _F32),
            pltpu.VMEM((2 * B, M), _BF16),
            pltpu.VMEM((H * B, D), _F32),
            pltpu.VMEM((Dc // 128, (B + 1) * H, 128), _F32),
            pltpu.VMEM((B * H, Dc), _BF16),
            pltpu.VMEM((2, _PIECES, H, Sk // _PIECES), _F32),
            pltpu.VMEM((Dc // 128, (B + 1) * H, 128), _F32),
            pltpu.VMEM((H // 2, B, 2 * D), _F32),
            pltpu.SemaphoreType.DMA((_RING,)),
        ],
        compiler_params=pltpu.CompilerParams(
            vmem_limit_bytes=100 * 1024 * 1024,
            disable_semaphore_checks=True,
        ),
    )(x, ckv, wq, wuk, wuv, wo, B_w3, B_w4, c, w_mod)
    return out.reshape(A_x.shape)
```

```python
import functools
import math

import jax
import jax.numpy as jnp
from jax import lax
import jax.experimental.pallas as pl
import jax.experimental.pallas.tpu as pltpu

_F32 = jnp.float32
_BF16 = jnp.bfloat16

_SLOTS = 4
_RING = _SLOTS + 1
_PARTS = 4
_PIECES = _SLOTS * _PARTS

_STEP = "1T2T2STPPTPPT"
_STEP_ATTN = "bTPPT0T9STPPT"
_STEP_MLP = "1T2T2STPPTPPT"
_STEP_IDLE = "0T2T1ST"
_STEP_MOD = ("0T1T1T1STPPPPT", "0T2T1T2STPPPPT")

_TICK_KIB = (32, 32, 32, 32, 64)
_KV_TICK_KIB = (32, 32, 32, 32, 64)
_SHIFT_KIB = 48
_W_SHIFT = (48, 48, 48, 48)


def _dot(a, b):
    return jnp.dot(a, b, preferred_element_type=_F32)


def _dot_nt(a, b):
    return lax.dot_general(a, b, (((1,), (1,)), ((), ())),
                           preferred_element_type=_F32)


def _layernorm(x, eps=1e-5):
    d = x - jnp.mean(x, axis=-1, keepdims=True)
    return d / jnp.sqrt(jnp.mean(d * d, axis=-1, keepdims=True) + eps)


def _gelu(x):
    c = math.sqrt(2.0 / math.pi)
    return 0.5 * x * (1.0 + jnp.tanh(c * (x + 0.044715 * (x * x * x))))


def _lhs(v):
    return jnp.concatenate([v, v], axis=0).astype(_BF16)


def _identity(v):
    return v


def _spare_rows(buf):
    n = 32 // buf.dtype.itemsize
    return pl.ds(buf.shape[0] - n, n)


class _Group:
    def __init__(self, src, dst, base, slot_rows, tick_rows, n_slots=_SLOTS,
                 cut=0, is_last=False):
        self.src, self.dst, self.base = src, dst, base
        self.slot_rows, self.tick_rows, self.n_slots = slot_rows, tick_rows, n_slots
        self.n_ticks = len(tick_rows)
        self.cut, self.is_last = cut, is_last

    def _copy(self, i, offset, size, sem):
        start = self.base + i * self.slot_rows + offset
        if not isinstance(start, int):
            start = pl.multiple_of(start, 8)
        rows = pl.ds(start, size)
        return pltpu.make_async_copy(self.src.at[rows], self.dst.at[rows], sem)

    def with_bulk(self, i, sem, action):
        head = sum(self.tick_rows)
        size = self.slot_rows - head
        if not self.cut or self.is_last is False:
            return action(self._copy(i, head, size, sem))
        short = self.is_last & (i == self.n_slots - 1)
        if isinstance(short, bool):
            return action(self._copy(i, head, size - self.cut * short, sem))
        pl.when(short)(lambda: action(self._copy(i, head, size - self.cut, sem)))
        pl.when(~short)(lambda: action(self._copy(i, head, size, sem)))

    def tick(self, i, j, sem):
        size = self.tick_rows[j]
        offset = sum(t for k, t in enumerate(self.tick_rows) if (-t, k) < (-size, j))
        return self._copy(i, offset, size, sem)

    def slot(self, i, sem):
        return self._copy(i, 0, self.slot_rows, sem)

    def after_ticks(self, lhs):
        zero = pltpu.bitcast(self.dst[_spare_rows(self.dst), 0:128], _BF16)
        reps = (lhs.shape[0] // zero.shape[0], lhs.shape[1] // zero.shape[1])
        return lhs + jnp.tile(zero, reps)


def _slot_sem(sems, phase, i):
    k = (phase * _SLOTS) % _RING + i
    if isinstance(k, int):
        return sems.at[k % _RING]
    return sems.at[jnp.where(k >= _RING, k - _RING, k)]


def _stream_step(program, sems, phase, arriving, following, i, piece, carry):
    sem_in, sem_out = _slot_sem(sems, phase, i), _slot_sem(sems, phase + 1, i)
    request = following.n_slots == _SLOTS or i < following.n_slots
    waits_left = sum(op.isdigit() for op in program)
    bulk_waited, waited, started, part = False, 0, 0, 0
    for pos, op in enumerate(program):
        if op == "b":
            arriving.tick(i, waited, sem_in).wait()
            waited += 1
        elif op.isdigit():
            waits_left -= 1
            if not bulk_waited:
                arriving.with_bulk(i, sem_in, lambda copy: copy.wait())
                bulk_waited = True
            upto = min(waited + int(op), arriving.n_ticks) if waits_left else arriving.n_ticks
            for j in range(waited, upto):
                arriving.tick(i, j, sem_in).wait()
            waited = upto
        elif op == "S" and request:
            following.with_bulk(i, sem_out, lambda copy: copy.start(priority=1))
        elif op == "T" and request:
            upto = started + 1 if "T" in program[pos + 1:] else following.n_ticks
            for j in range(started, min(upto, following.n_ticks)):
                following.tick(i, j, sem_out).start()
            started = upto
        elif op == "P":
            carry = piece(i, part, carry, following.after_ticks)
            part += 1
    return carry


def _stream_phase(program, sems, phase, arriving, following, piece=None, carry=0,
                  unroll=False):
    step = functools.partial(_stream_step, program, sems, phase, arriving, following)
    if unroll:
        for i in range(_SLOTS):
            carry = step(i, piece, carry)
        return carry
    return lax.fori_loop(0, _SLOTS, lambda i, c: step(i, piece, c), carry)


def _kernel(x_hbm, ckv_hbm, wq_hbm, wuk_hbm, wuv_hbm, wo_hbm, w3_hbm, w4_hbm,
            c_hbm, wmod_hbm, o_ref,
            x_v, c_v, wmod_v, wq_v, wuk_v, wuv_v, wo_v, w3_v, w4_v, ckv_v,
            mod_v, h_v, q_v, qabs32_v, qabs_v, s_v, lat_v, ctx_v, sems,
            *, B, H, Sk, D, M, F):
    NP = H // 2
    KC = Sk // _PIECES
    assert NP == _PIECES

    def halves(src, dst, tick_rows, shift, base=0, rows=None, is_last=True):
        slot = (src.shape[0] if rows is None else rows) // (2 * _SLOTS)
        return [_Group(src, dst, shift + base + k * _SLOTS * slot, slot, tick_rows,
                       cut=shift, is_last=is_last if k == 1 else False)
                for k in range(2)]

    def head_weights(src, dst, k):
        return halves(src.bitcast(jnp.uint32), dst, [2 * t for t in _TICK_KIB],
                      2 * _W_SHIFT[k])

    def g_kv(b):
        return halves(ckv_hbm, ckv_v, _KV_TICK_KIB, _SHIFT_KIB, b * Sk, Sk, b == B - 1)

    g_mod = halves(wmod_hbm, wmod_v, (8, 8, 8), 0)
    g_q = head_weights(wq_hbm, wq_v, 0)
    g_uk = head_weights(wuk_hbm, wuk_v, 1)
    g_uv = head_weights(wuv_hbm, wuv_v, 2)
    g_o = halves(wo_hbm, wo_v, _TICK_KIB, _W_SHIFT[3])
    g_3 = _Group(w3_hbm, w3_v, 0, M // _SLOTS, (8, 8, 8, 8, 16))
    f_last = 256
    g_4 = _Group(w4_hbm, w4_v, 0, (F - f_last) // _SLOTS, (16, 16, 16, 16, 64))
    g_end = _Group(w4_hbm, w4_v, F - f_last, f_last, (32,), n_slots=1)

    _stream_phase("ST", sems, -1, None, g_mod[0], unroll=True)
    small = [pltpu.make_async_copy(c_hbm, c_v, sems.at[_SLOTS]),
             pltpu.make_async_copy(x_hbm, x_v, sems.at[_SLOTS])]
    for first in (g_q[0], g_uk[0], g_kv(0)[0], g_uv[0], g_o[0]):
        if first.base:
            rows = pl.ds(0, first.base)
            small.append(pltpu.make_async_copy(
                first.src.at[rows], first.dst.at[rows], sems.at[_SLOTS]))
    for copy in small:
        copy.start()
    for buf in (wmod_v, wq_v, wuk_v, wuv_v, wo_v, w3_v, w4_v, ckv_v):
        spare = _spare_rows(buf)
        buf[spare, 0:128] = jnp.zeros((spare.size, 128), buf.dtype)

    def pair_weights(w_v, pair, half):
        words = w_v[pl.ds(pair + half * (M // 2) * NP, M // 2, stride=NP), :]
        return [pltpu.bitcast(w, _F32).astype(_BF16)
                for w in (words << 16, words & jnp.uint32(0xFFFF0000))]

    def pair_rows(pair):
        return pl.ds(pl.multiple_of(pair * 2 * B, 2 * B), 2 * B)

    def head_rows(head):
        return pl.ds(head, B, stride=H)

    def batch_rows(b):
        return pl.ds(b * H if isinstance(b, int) else pl.multiple_of(b * H, H), H)

    for copy in small:
        copy.wait()
    cf = c_v[...].astype(_F32)
    sc = _lhs(cf * jax.nn.sigmoid(cf))
    _stream_phase(_STEP_IDLE, sems, 0, g_mod[0], g_mod[1])

    def mod(k):
        return mod_v[:, k * M:(k + 1) * M]

    def mod_piece(half, i, j, carry, pin):
        n = i * _PARTS + j
        rows = slice(half * (M // 2), (half + 1) * (M // 2))
        if n < 12:
            cols = slice(n * (M // 2), (n + 1) * (M // 2))
            part = _dot(pin(sc[:, rows]), wmod_v[rows, cols])[:B]
            mod_v[:, cols] = part if half == 0 else mod_v[:, cols] + part
        elif n == 12 and half == 1:
            h_v[...] = _lhs(_layernorm(x_v[...].astype(_F32)) * (1.0 + mod(1)) + mod(0))
        return carry

    _stream_phase(_STEP_MOD[0], sems, 1, g_mod[1], g_q[0],
                  functools.partial(mod_piece, 0), unroll=True)
    _stream_phase(_STEP_MOD[1], sems, 2, g_q[0], g_q[1],
                  functools.partial(mod_piece, 1), unroll=True)

    def q_piece(half, i, j, carry, pin):
        pair = i * _PARTS + j
        h = pin(h_v[:, half * (M // 2):(half + 1) * (M // 2)])
        part = jnp.concatenate(
            [_dot(h, w)[:B] for w in pair_weights(wq_v, pair, half)], axis=0)
        rows = pair_rows(pair)
        q_v[rows, :] = part if half == 0 else q_v[rows, :] + part
        return carry

    _stream_phase(_STEP, sems, 3, g_q[1], g_uk[0], functools.partial(q_piece, 0))
    _stream_phase(_STEP, sems, 4, g_uk[0], g_uk[1], functools.partial(q_piece, 1))

    def qabs_piece(half, i, j, carry, pin):
        pair = i * _PARTS + j
        q = pin(q_v[pair_rows(pair), :].astype(_BF16))
        for p, w in enumerate(pair_weights(wuk_v, pair, half)):
            r = _dot_nt(q, w)[p * B:(p + 1) * B] * (D ** -0.5 * math.log2(math.e))
            for k in range(M // 256):
                qabs32_v[half * (M // 256) + k, head_rows(2 * pair + p), :] = (
                    r[:, k * 128:(k + 1) * 128])
        return carry

    _stream_phase(_STEP, sems, 5, g_uk[1], g_kv(0)[0], functools.partial(qabs_piece, 0))
    _stream_phase(_STEP, sems, 6, *g_kv(0), functools.partial(qabs_piece, 1))
    for k in range(M // 128):
        qabs_v[:, k * 128:(k + 1) * 128] = qabs32_v[k, 0:B * H, :].astype(_BF16)

    def keys(b, n):
        return ckv_v[pl.ds(pl.multiple_of(b * Sk + n * KC, KC), KC), :]

    def score_chunk(b, n, m, pin):
        s = _dot_nt(pin(qabs_v[batch_rows(b), :]), keys(b, n))
        s_v[b % 2, n] = s
        for t in range(0, KC, 128):
            m = jnp.maximum(m, s[:, t:t + 128])
        return m

    def value_chunk(b, n, s, m, l, acc, pin):
        p = [jnp.exp2(s[:, t:t + 128] - m) for t in range(0, KC, 128)]
        for pt in p:
            l = l + pt
        p = pin(jnp.concatenate(p, axis=1).astype(_BF16))
        return l, acc + _dot(p, keys(b, n))

    def store_lat(b, l, acc):
        lat = acc / jnp.sum(l, axis=-1, keepdims=True)
        for k in range(M // 128):
            lat_v[k, batch_rows(b), :] = lat[:, k * 128:(k + 1) * 128]

    m_init = jnp.full((H, 128), -jnp.inf, _F32)
    l_init, acc_init = jnp.zeros((H, 128), _F32), jnp.zeros((H, M), _F32)

    def attend(b, groups, m_prev):
        scores = []

        def piece(half, i, j, carry, pin):
            m, l, acc = carry
            if groups[half + 1].dst is ckv_v:
                pin = _identity
            n = (half * _SLOTS + i) * (_PARTS // 2) + j // 2
            if j % 2 == 1:
                m = score_chunk(b, n, m, pin)
            elif m_prev is not None:
                if "b" in _STEP_ATTN:
                    scores[:] = [s_v[(b - 1) % 2, n]] * 2
                elif j == 0:
                    scores[:] = [s_v[(b - 1) % 2, n + k] for k in range(_PARTS // 2)]
                l, acc = value_chunk(b - 1, n, scores[j // 2], m_prev, l, acc, pin)
            return m, l, acc

        carry = (m_init, 0, 0) if m_prev is None else (m_init, l_init, acc_init)
        for half in range(2):
            carry = _stream_phase(_STEP_ATTN, sems, 7 + 2 * b + half, groups[half],
                                  groups[half + 1], functools.partial(piece, half), carry)
        m, l, acc = carry
        if m_prev is not None:
            store_lat(b - 1, l, acc)
        return jnp.broadcast_to(jnp.max(m, axis=-1, keepdims=True), (H, 128))

    def kv_groups(b):
        return [g_kv(b)[1]] + g_kv(b + 1)

    def last_values(i, j, carry, pin):
        n = i * _PARTS + j
        return value_chunk(B - 1, n, s_v[(B - 1) % 2, n], m_last, *carry, pin)

    m = attend(0, kv_groups(0), None)
    m = lax.fori_loop(1, B - 1, lambda b, m: attend(b, kv_groups(b), m), m)
    m_last = attend(B - 1, [g_kv(B - 1)[1]] + g_uv, m)
    store_lat(B - 1, *_stream_phase(_STEP, sems, 7 + 2 * B, g_uv[1], g_o[0],
                                    last_values, (l_init, acc_init)))

    def ctx_piece(k, i, j, acc, pin):
        pair, half = (k * _PIECES + i * _PARTS + j) // 2, j % 2
        lat = jnp.concatenate([jnp.concatenate(
            [lat_v[half * (M // 256) + t, head_rows(2 * pair + p), :]
             for t in range(M // 256)], axis=1) for p in range(2)], axis=0)
        lat = pin(lat.astype(_BF16))
        part = jnp.concatenate(
            [_dot(lat, w)[p * B:(p + 1) * B]
             for p, w in enumerate(pair_weights(wuv_v, pair, half))], axis=1)
        if half == 0:
            return part
        ctx_v[pair] = acc + part
        return acc

    ctx_init = jnp.zeros((B, 2 * D), _F32)
    _stream_phase(_STEP, sems, 8 + 2 * B, g_o[0], g_o[1],
                  functools.partial(ctx_piece, 0), ctx_init)
    _stream_phase(_STEP, sems, 9 + 2 * B, g_o[1], g_3,
                  functools.partial(ctx_piece, 1), ctx_init)

    def up_piece(i, j, carry, pin):
        n = i * _PARTS + j
        if n < NP // 2:
            for pair in (2 * n, 2 * n + 1):
                w = wo_v[pair * 2 * D:(pair + 1) * 2 * D, :]
                carry = carry + _dot(pin(_lhs(ctx_v[pair])), w)[:B]
        elif n == NP // 2:
            x1 = x_v[...].astype(_F32) + mod(2) * carry
            hb = _layernorm(x1) * (1.0 + mod(4)) + mod(3)
            carry = x1, hb, _lhs(_layernorm(hb)), jnp.zeros((B, F), _F32)
        elif n - NP // 2 <= _SLOTS:
            k = n - NP // 2 - 1
            assert k <= i
            x1, hb, ln, pre = carry
            rows = slice(k * g_3.slot_rows, (k + 1) * g_3.slot_rows)
            carry = x1, hb, ln, pre + _dot(pin(ln[:, rows]), w3_v[rows, :])[:B]
        return carry

    x1, y, _, pre = _stream_phase(_STEP_MLP, sems, 10 + 2 * B, g_3, g_4, up_piece,
                                  jnp.zeros((B, M), _F32), unroll=True)
    g = _lhs(_gelu(pre))

    def down_piece(i, j, y, pin):
        if (j + 1) * 128 > g_4.slot_rows:
            return y
        rows = slice(i * g_4.slot_rows + j * 128, i * g_4.slot_rows + (j + 1) * 128)
        return y + _dot(pin(g[:, rows]), w4_v[rows, :])[:B]

    assert g_4.slot_rows % 128 == 0 and g_4.slot_rows <= 128 * _PARTS
    y = _stream_phase(_STEP_MLP, sems, 11 + 2 * B, g_4, g_end, down_piece, y, unroll=True)
    g_end.slot(0, _slot_sem(sems, 12 + 2 * B, 0)).wait()
    y = y + _dot(g[:, F - f_last:], w4_v[F - f_last:F, :])[:B]
    o_ref[...] = (x1 + mod(5) * y).astype(o_ref.dtype)


@jax.jit
def pallas_adaLN_cond__compressed_kv_cla__mixer_s_mlp__decode_kernel(
    A_x: jax.Array,
    A_c_kv: jax.Array,
    A_w_q: jax.Array,
    A_w_uk: jax.Array,
    A_w_uv: jax.Array,
    A_w_o: jax.Array,
    B_x: jax.Array,
    B_w1: jax.Array,
    B_w2: jax.Array,
    B_w3: jax.Array,
    B_w4: jax.Array,
    c: jax.Array,
    w_mod: jax.Array,
):
    del B_x, B_w1, B_w2
    B, Sq, M = A_x.shape
    _, Sk, Dc = A_c_kv.shape
    _, H, D = A_w_q.shape
    F = B_w3.shape[1]
    assert Sq == 1 and Dc == M and D == 128 and B == 8

    x = A_x.reshape(B, M)
    ckv = A_c_kv.reshape(B * Sk, Dc)
    wq = A_w_q.reshape(M * H, D)
    wuk = A_w_uk.reshape(Dc * H, D)
    wuv = A_w_uv.reshape(Dc * H, D)
    wo = A_w_o.reshape(H * D, M)

    def streamed(a):
        return pltpu.VMEM((a.shape[0] + 16, a.shape[1]), a.dtype)

    def streamed_words(a):
        return pltpu.VMEM((a.shape[0] // 2 + 16, a.shape[1]), jnp.uint32)

    out = pl.pallas_call(
        functools.partial(_kernel, B=B, H=H, Sk=Sk, D=D, M=M, F=F),
        out_shape=jax.ShapeDtypeStruct(x.shape, x.dtype),
        in_specs=[pl.BlockSpec(memory_space=pl.ANY)] * 10,
        out_specs=pl.BlockSpec(memory_space=pltpu.VMEM),
        scratch_shapes=[
            pltpu.VMEM(x.shape, x.dtype), pltpu.VMEM(c.shape, c.dtype),
            streamed(w_mod), streamed_words(wq), streamed_words(wuk),
            streamed_words(wuv), streamed(wo), streamed(B_w3), streamed(B_w4),
            streamed(ckv),
            pltpu.VMEM((B, 6 * M), _F32),
            pltpu.VMEM((2 * B, M), _BF16),
            pltpu.VMEM((H * B, D), _F32),
            pltpu.VMEM((Dc // 128, (B + 1) * H, 128), _F32),
            pltpu.VMEM((B * H, Dc), _BF16),
            pltpu.VMEM((2, _PIECES, H, Sk // _PIECES), _F32),
            pltpu.VMEM((Dc // 128, (B + 1) * H, 128), _F32),
            pltpu.VMEM((H // 2, B, 2 * D), _F32),
            pltpu.SemaphoreType.DMA((_RING,)),
        ],
        compiler_params=pltpu.CompilerParams(
            vmem_limit_bytes=100 * 1024 * 1024,
            disable_semaphore_checks=True,
        ),
    )(x, ckv, wq, wuk, wuv, wo, B_w3, B_w4, c, w_mod)
    return out.reshape(A_x.shape)
```

```python
import functools
import math

import jax
import jax.numpy as jnp
from jax import lax
import jax.experimental.pallas as pl
import jax.experimental.pallas.tpu as pltpu

_F32 = jnp.float32
_BF16 = jnp.bfloat16

_SLOTS = 4
_RING = _SLOTS + 1
_PARTS = 4
_PIECES = _SLOTS * _PARTS

_STEP = "1T2T2STPPTPPT"
_STEP_ATTN = "bTPPT0T9STPPT"
_STEP_MLP = "0T2T3STPPTPPT"
_STEP_IDLE = "0T1ST"
_STEP_MOD = ("0T1T1T1STPPPPT", "0T2T1T2STPPPPT")

_TICK_KIB = (32, 32, 32, 32, 64)
_KV_TICK_KIB = (32, 32, 32, 32, 64)
_SHIFT_KIB = 48
_W_SHIFT = (48, 48, 48, 48)


def _dot(a, b):
    return jnp.dot(a, b, preferred_element_type=_F32)


def _dot_nt(a, b):
    return lax.dot_general(a, b, (((1,), (1,)), ((), ())),
                           preferred_element_type=_F32)


def _layernorm(x, eps=1e-5):
    d = x - jnp.mean(x, axis=-1, keepdims=True)
    return d / jnp.sqrt(jnp.mean(d * d, axis=-1, keepdims=True) + eps)


def _gelu(x):
    c = math.sqrt(2.0 / math.pi)
    return 0.5 * x * (1.0 + jnp.tanh(c * (x + 0.044715 * (x * x * x))))


def _lhs(v):
    return jnp.concatenate([v, v], axis=0).astype(_BF16)


def _identity(v):
    return v


def _spare_rows(buf):
    n = 32 // buf.dtype.itemsize
    return pl.ds(buf.shape[0] - n, n)


class _Group:
    def __init__(self, src, dst, base, slot_rows, tick_rows, n_slots=_SLOTS,
                 cut=0, is_last=False):
        self.src, self.dst, self.base = src, dst, base
        self.slot_rows, self.tick_rows, self.n_slots = slot_rows, tick_rows, n_slots
        self.n_ticks = len(tick_rows)
        self.cut, self.is_last = cut, is_last

    def _copy(self, i, offset, size, sem):
        start = self.base + i * self.slot_rows + offset
        if not isinstance(start, int):
            start = pl.multiple_of(start, 8)
        rows = pl.ds(start, size)
        return pltpu.make_async_copy(self.src.at[rows], self.dst.at[rows], sem)

    def with_bulk(self, i, sem, action):
        head = sum(self.tick_rows)
        size = self.slot_rows - head
        if not self.cut or self.is_last is False:
            return action(self._copy(i, head, size, sem))
        short = self.is_last & (i == self.n_slots - 1)
        if isinstance(short, bool):
            return action(self._copy(i, head, size - self.cut * short, sem))
        pl.when(short)(lambda: action(self._copy(i, head, size - self.cut, sem)))
        pl.when(~short)(lambda: action(self._copy(i, head, size, sem)))

    def tick(self, i, j, sem):
        size = self.tick_rows[j]
        offset = sum(t for k, t in enumerate(self.tick_rows) if (-t, k) < (-size, j))
        return self._copy(i, offset, size, sem)

    def slot(self, i, sem):
        return self._copy(i, 0, self.slot_rows, sem)

    def after_ticks(self, lhs):
        zero = pltpu.bitcast(self.dst[_spare_rows(self.dst), 0:128], _BF16)
        reps = (lhs.shape[0] // zero.shape[0], lhs.shape[1] // zero.shape[1])
        return lhs + jnp.tile(zero, reps)


def _slot_sem(sems, phase, i):
    k = (phase * _SLOTS) % _RING + i
    if isinstance(k, int):
        return sems.at[k % _RING]
    return sems.at[jnp.where(k >= _RING, k - _RING, k)]


def _stream_step(program, sems, phase, arriving, following, i, piece, carry):
    sem_in, sem_out = _slot_sem(sems, phase, i), _slot_sem(sems, phase + 1, i)
    request = following.n_slots == _SLOTS or i < following.n_slots
    waits_left = sum(op.isdigit() for op in program)
    bulk_waited, waited, started, part = False, 0, 0, 0
    for pos, op in enumerate(program):
        if op == "b":
            arriving.tick(i, waited, sem_in).wait()
            waited += 1
        elif op.isdigit():
            waits_left -= 1
            if not bulk_waited:
                arriving.with_bulk(i, sem_in, lambda copy: copy.wait())
                bulk_waited = True
            upto = min(waited + int(op), arriving.n_ticks) if waits_left else arriving.n_ticks
            for j in range(waited, upto):
                arriving.tick(i, j, sem_in).wait()
            waited = upto
        elif op == "S" and request:
            following.with_bulk(i, sem_out, lambda copy: copy.start(priority=1))
        elif op == "T" and request:
            upto = started + 1 if "T" in program[pos + 1:] else following.n_ticks
            for j in range(started, min(upto, following.n_ticks)):
                following.tick(i, j, sem_out).start()
            started = upto
        elif op == "P":
            carry = piece(i, part, carry, following.after_ticks)
            part += 1
    return carry


def _stream_phase(program, sems, phase, arriving, following, piece=None, carry=0,
                  unroll=False):
    step = functools.partial(_stream_step, program, sems, phase, arriving, following)
    if unroll:
        for i in range(_SLOTS):
            carry = step(i, piece, carry)
        return carry
    return lax.fori_loop(0, _SLOTS, lambda i, c: step(i, piece, c), carry)


def _kernel(x_hbm, ckv_hbm, wq_hbm, wuk_hbm, wuv_hbm, wo_hbm, w3_hbm, w4_hbm,
            c_hbm, wmod_hbm, o_ref,
            x_v, c_v, wmod_v, wq_v, wuk_v, wuv_v, wo_v, w3_v, w4_v, ckv_v,
            mod_v, h_v, q_v, qabs32_v, qabs_v, s_v, lat_v, ctx_v, sems,
            *, B, H, Sk, D, M, F):
    NP = H // 2
    KC = Sk // _PIECES
    assert NP == _PIECES

    def halves(src, dst, tick_rows, shift, base=0, rows=None, is_last=True):
        slot = (src.shape[0] if rows is None else rows) // (2 * _SLOTS)
        return [_Group(src, dst, shift + base + k * _SLOTS * slot, slot, tick_rows,
                       cut=shift, is_last=is_last if k == 1 else False)
                for k in range(2)]

    def head_weights(src, dst, k):
        return halves(src.bitcast(jnp.uint32), dst, [2 * t for t in _TICK_KIB],
                      2 * _W_SHIFT[k])

    def g_kv(b):
        return halves(ckv_hbm, ckv_v, _KV_TICK_KIB, _SHIFT_KIB, b * Sk, Sk, b == B - 1)

    g_mod = halves(wmod_hbm, wmod_v, (8, 8), 0)
    g_q = head_weights(wq_hbm, wq_v, 0)
    g_uk = head_weights(wuk_hbm, wuk_v, 1)
    g_uv = head_weights(wuv_hbm, wuv_v, 2)
    g_o = halves(wo_hbm, wo_v, _TICK_KIB, _W_SHIFT[3])
    g_3 = _Group(w3_hbm, w3_v, 0, M // _SLOTS, (8, 8, 8, 8, 16))
    f_last = 256
    g_4 = _Group(w4_hbm, w4_v, 0, (F - f_last) // _SLOTS, (16, 16, 16, 16, 64))
    g_end = _Group(w4_hbm, w4_v, F - f_last, f_last, (32,), n_slots=1)

    small = [pltpu.make_async_copy(c_hbm, c_v, sems.at[_RING]),
             pltpu.make_async_copy(x_hbm, x_v, sems.at[_RING])]
    for copy in small:
        copy.start()
    _stream_phase("ST", sems, -1, None, g_mod[0], unroll=True)
    for buf in (wmod_v, wq_v, wuk_v, wuv_v, wo_v, w3_v, w4_v, ckv_v):
        spare = _spare_rows(buf)
        buf[spare, 0:128] = jnp.zeros((spare.size, 128), buf.dtype)

    def pair_weights(w_v, pair, half):
        words = w_v[pl.ds(pair + half * (M // 2) * NP, M // 2, stride=NP), :]
        return [pltpu.bitcast(w, _F32).astype(_BF16)
                for w in (words << 16, words & jnp.uint32(0xFFFF0000))]

    def pair_rows(pair):
        return pl.ds(pl.multiple_of(pair * 2 * B, 2 * B), 2 * B)

    def head_rows(head):
        return pl.ds(head, B, stride=H)

    def batch_rows(b):
        return pl.ds(b * H if isinstance(b, int) else pl.multiple_of(b * H, H), H)

    _stream_phase(_STEP_IDLE, sems, 0, g_mod[0], g_mod[1])
    for copy in small:
        copy.wait()
    cf = c_v[...].astype(_F32)
    sc = _lhs(cf * jax.nn.sigmoid(cf))

    heads = [pltpu.make_async_copy(g.src.at[pl.ds(0, g.base)], g.dst.at[pl.ds(0, g.base)],
                                   sems.at[_RING])
             for g in (g_q[0], g_uk[0], g_kv(0)[0], g_uv[0], g_o[0])]

    def mod(k):
        return mod_v[:, k * M:(k + 1) * M]

    def mod_piece(half, i, j, carry, pin):
        n = i * _PARTS + j
        rows = slice(half * (M // 2), (half + 1) * (M // 2))
        if n < 12:
            cols = slice(n * (M // 2), (n + 1) * (M // 2))
            part = _dot(pin(sc[:, rows]), wmod_v[rows, cols])[:B]
            mod_v[:, cols] = part if half == 0 else mod_v[:, cols] + part
        elif half == 0:
            for copy in heads[n - 12::_PIECES - 12]:
                copy.start()
        elif n == 12:
            h_v[...] = _lhs(_layernorm(x_v[...].astype(_F32)) * (1.0 + mod(1)) + mod(0))
        return carry

    _stream_phase(_STEP_MOD[0], sems, 1, g_mod[1], g_q[0],
                  functools.partial(mod_piece, 0), unroll=True)
    _stream_phase(_STEP_MOD[1], sems, 2, g_q[0], g_q[1],
                  functools.partial(mod_piece, 1), unroll=True)
    for copy in heads:
        copy.wait()

    def q_piece(half, i, j, carry, pin):
        pair = i * _PARTS + j
        h = pin(h_v[:, half * (M // 2):(half + 1) * (M // 2)])
        part = jnp.concatenate(
            [_dot(h, w)[:B] for w in pair_weights(wq_v, pair, half)], axis=0)
        rows = pair_rows(pair)
        q_v[rows, :] = part if half == 0 else q_v[rows, :] + part
        return carry

    _stream_phase(_STEP, sems, 3, g_q[1], g_uk[0], functools.partial(q_piece, 0))
    _stream_phase(_STEP, sems, 4, g_uk[0], g_uk[1], functools.partial(q_piece, 1))

    def qabs_piece(half, i, j, carry, pin):
        pair = i * _PARTS + j
        q = pin(q_v[pair_rows(pair), :].astype(_BF16))
        for p, w in enumerate(pair_weights(wuk_v, pair, half)):
            r = _dot_nt(q, w)[p * B:(p + 1) * B] * (D ** -0.5 * math.log2(math.e))
            for k in range(M // 256):
                qabs32_v[half * (M // 256) + k, head_rows(2 * pair + p), :] = (
                    r[:, k * 128:(k + 1) * 128])
        return carry

    _stream_phase(_STEP, sems, 5, g_uk[1], g_kv(0)[0], functools.partial(qabs_piece, 0))
    _stream_phase(_STEP, sems, 6, *g_kv(0), functools.partial(qabs_piece, 1))
    for k in range(M // 128):
        qabs_v[:, k * 128:(k + 1) * 128] = qabs32_v[k, 0:B * H, :].astype(_BF16)

    def keys(b, n):
        return ckv_v[pl.ds(pl.multiple_of(b * Sk + n * KC, KC), KC), :]

    def score_chunk(b, n, m, pin):
        s = _dot_nt(pin(qabs_v[batch_rows(b), :]), keys(b, n))
        s_v[b % 2, n] = s
        for t in range(0, KC, 128):
            m = jnp.maximum(m, s[:, t:t + 128])
        return m

    def value_chunk(b, n, s, m, l, acc, pin):
        p = [jnp.exp2(s[:, t:t + 128] - m) for t in range(0, KC, 128)]
        for pt in p:
            l = l + pt
        p = pin(jnp.concatenate(p, axis=1).astype(_BF16))
        return l, acc + _dot(p, keys(b, n))

    def store_lat(b, l, acc):
        lat = acc / jnp.sum(l, axis=-1, keepdims=True)
        for k in range(M // 128):
            lat_v[k, batch_rows(b), :] = lat[:, k * 128:(k + 1) * 128]

    m_init = jnp.full((H, 128), -jnp.inf, _F32)
    l_init, acc_init = jnp.zeros((H, 128), _F32), jnp.zeros((H, M), _F32)

    def attend(b, groups, m_prev):
        scores = []

        def piece(half, i, j, carry, pin):
            m, l, acc = carry
            if groups[half + 1].dst is ckv_v:
                pin = _identity
            n = (half * _SLOTS + i) * (_PARTS // 2) + j // 2
            if j % 2 == 1:
                m = score_chunk(b, n, m, pin)
            elif m_prev is not None:
                if "b" in _STEP_ATTN:
                    scores[:] = [s_v[(b - 1) % 2, n]] * 2
                elif j == 0:
                    scores[:] = [s_v[(b - 1) % 2, n + k] for k in range(_PARTS // 2)]
                l, acc = value_chunk(b - 1, n, scores[j // 2], m_prev, l, acc, pin)
            return m, l, acc

        carry = (m_init, 0, 0) if m_prev is None else (m_init, l_init, acc_init)
        for half in range(2):
            carry = _stream_phase(_STEP_ATTN, sems, 7 + 2 * b + half, groups[half],
                                  groups[half + 1], functools.partial(piece, half), carry)
        m, l, acc = carry
        if m_prev is not None:
            store_lat(b - 1, l, acc)
        return jnp.broadcast_to(jnp.max(m, axis=-1, keepdims=True), (H, 128))

    def kv_groups(b):
        return [g_kv(b)[1]] + g_kv(b + 1)

    def last_values(i, j, carry, pin):
        n = i * _PARTS + j
        return value_chunk(B - 1, n, s_v[(B - 1) % 2, n], m_last, *carry, pin)

    m = attend(0, kv_groups(0), None)
    m = lax.fori_loop(1, B - 1, lambda b, m: attend(b, kv_groups(b), m), m)
    m_last = attend(B - 1, [g_kv(B - 1)[1]] + g_uv, m)
    store_lat(B - 1, *_stream_phase(_STEP, sems, 7 + 2 * B, g_uv[1], g_o[0],
                                    last_values, (l_init, acc_init)))

    def ctx_piece(k, i, j, acc, pin):
        pair, half = (k * _PIECES + i * _PARTS + j) // 2, j % 2
        lat = jnp.concatenate([jnp.concatenate(
            [lat_v[half * (M // 256) + t, head_rows(2 * pair + p), :]
             for t in range(M // 256)], axis=1) for p in range(2)], axis=0)
        lat = pin(lat.astype(_BF16))
        part = jnp.concatenate(
            [_dot(lat, w)[p * B:(p + 1) * B]
             for p, w in enumerate(pair_weights(wuv_v, pair, half))], axis=1)
        if half == 0:
            return part
        ctx_v[pair] = acc + part
        return acc

    ctx_init = jnp.zeros((B, 2 * D), _F32)
    _stream_phase(_STEP, sems, 8 + 2 * B, g_o[0], g_o[1],
                  functools.partial(ctx_piece, 0), ctx_init)
    _stream_phase(_STEP, sems, 9 + 2 * B, g_o[1], g_3,
                  functools.partial(ctx_piece, 1), ctx_init)

    def up_piece(i, j, carry, pin):
        n = i * _PARTS + j
        if n < NP // 2:
            for pair in (2 * n, 2 * n + 1):
                w = wo_v[pair * 2 * D:(pair + 1) * 2 * D, :]
                carry = carry + _dot(pin(_lhs(ctx_v[pair])), w)[:B]
        elif n == NP // 2:
            x1 = x_v[...].astype(_F32) + mod(2) * carry
            hb = _layernorm(x1) * (1.0 + mod(4)) + mod(3)
            carry = x1, hb, _lhs(_layernorm(hb)), jnp.zeros((B, F), _F32)
        elif n - NP // 2 <= _SLOTS:
            k = n - NP // 2 - 1
            assert k <= i
            x1, hb, ln, pre = carry
            rows = slice(k * g_3.slot_rows, (k + 1) * g_3.slot_rows)
            carry = x1, hb, ln, pre + _dot(pin(ln[:, rows]), w3_v[rows, :])[:B]
        return carry

    x1, y, _, pre = _stream_phase(_STEP_MLP, sems, 10 + 2 * B, g_3, g_4, up_piece,
                                  jnp.zeros((B, M), _F32), unroll=True)
    g = _lhs(_gelu(pre))

    def down_piece(i, j, y, pin):
        if (j + 1) * 128 > g_4.slot_rows:
            return y
        rows = slice(i * g_4.slot_rows + j * 128, i * g_4.slot_rows + (j + 1) * 128)
        return y + _dot(pin(g[:, rows]), w4_v[rows, :])[:B]

    assert g_4.slot_rows % 128 == 0 and g_4.slot_rows <= 128 * _PARTS
    y = _stream_phase(_STEP_MLP, sems, 11 + 2 * B, g_4, g_end, down_piece, y, unroll=True)
    g_end.slot(0, _slot_sem(sems, 12 + 2 * B, 0)).wait()
    y = y + _dot(g[:, F - f_last:], w4_v[F - f_last:F, :])[:B]
    o_ref[...] = (x1 + mod(5) * y).astype(o_ref.dtype)


@jax.jit
def pallas_adaLN_cond__compressed_kv_cla__mixer_s_mlp__decode_kernel(
    A_x: jax.Array,
    A_c_kv: jax.Array,
    A_w_q: jax.Array,
    A_w_uk: jax.Array,
    A_w_uv: jax.Array,
    A_w_o: jax.Array,
    B_x: jax.Array,
    B_w1: jax.Array,
    B_w2: jax.Array,
    B_w3: jax.Array,
    B_w4: jax.Array,
    c: jax.Array,
    w_mod: jax.Array,
):
    del B_x, B_w1, B_w2
    B, Sq, M = A_x.shape
    _, Sk, Dc = A_c_kv.shape
    _, H, D = A_w_q.shape
    F = B_w3.shape[1]
    assert Sq == 1 and Dc == M and D == 128 and B == 8

    x = A_x.reshape(B, M)
    ckv = A_c_kv.reshape(B * Sk, Dc)
    wq = A_w_q.reshape(M * H, D)
    wuk = A_w_uk.reshape(Dc * H, D)
    wuv = A_w_uv.reshape(Dc * H, D)
    wo = A_w_o.reshape(H * D, M)

    def streamed(a):
        return pltpu.VMEM((a.shape[0] + 16, a.shape[1]), a.dtype)

    def streamed_words(a):
        return pltpu.VMEM((a.shape[0] // 2 + 16, a.shape[1]), jnp.uint32)

    out = pl.pallas_call(
        functools.partial(_kernel, B=B, H=H, Sk=Sk, D=D, M=M, F=F),
        out_shape=jax.ShapeDtypeStruct(x.shape, x.dtype),
        in_specs=[pl.BlockSpec(memory_space=pl.ANY)] * 10,
        out_specs=pl.BlockSpec(memory_space=pltpu.VMEM),
        scratch_shapes=[
            pltpu.VMEM(x.shape, x.dtype), pltpu.VMEM(c.shape, c.dtype),
            streamed(w_mod), streamed_words(wq), streamed_words(wuk),
            streamed_words(wuv), streamed(wo), streamed(B_w3), streamed(B_w4),
            streamed(ckv),
            pltpu.VMEM((B, 6 * M), _F32),
            pltpu.VMEM((2 * B, M), _BF16),
            pltpu.VMEM((H * B, D), _F32),
            pltpu.VMEM((Dc // 128, (B + 1) * H, 128), _F32),
            pltpu.VMEM((B * H, Dc), _BF16),
            pltpu.VMEM((2, _PIECES, H, Sk // _PIECES), _F32),
            pltpu.VMEM((Dc // 128, (B + 1) * H, 128), _F32),
            pltpu.VMEM((H // 2, B, 2 * D), _F32),
            pltpu.SemaphoreType.DMA((_RING + 1,)),
        ],
        compiler_params=pltpu.CompilerParams(
            vmem_limit_bytes=100 * 1024 * 1024,
            disable_semaphore_checks=True,
        ),
    )(x, ckv, wq, wuk, wuv, wo, B_w3, B_w4, c, w_mod)
    return out.reshape(A_x.shape)
```

```python
import functools
import math

import jax
import jax.numpy as jnp
from jax import lax
import jax.experimental.pallas as pl
import jax.experimental.pallas.tpu as pltpu

_F32 = jnp.float32
_BF16 = jnp.bfloat16

_SLOTS = 4
_RING = _SLOTS + 1
_PARTS = 4
_PIECES = _SLOTS * _PARTS

_STEP = "1T2T2STPPTPPT"
_STEP_ATTN = "bTPPT0T9STPPT"
_STEP_MLP = "0T2T3STPPTPPT"
_STEP_IDLE = "0T1ST"
_STEP_MOD = ("0T1T1T1STPPPPT", "0T2T1T2STPPPPT")

_TICK_KIB = (32, 32, 32, 32, 64)
_SHIFT_KIB = 48


def _dot(a, b):
    return jnp.dot(a, b, preferred_element_type=_F32)


def _dot_nt(a, b):
    return lax.dot_general(a, b, (((1,), (1,)), ((), ())),
                           preferred_element_type=_F32)


def _layernorm(x, eps=1e-5):
    d = x - jnp.mean(x, axis=-1, keepdims=True)
    return d / jnp.sqrt(jnp.mean(d * d, axis=-1, keepdims=True) + eps)


def _gelu(x):
    c = math.sqrt(2.0 / math.pi)
    return 0.5 * x * (1.0 + jnp.tanh(c * (x + 0.044715 * (x * x * x))))


def _lhs(v):
    return jnp.concatenate([v, v], axis=0).astype(_BF16)


def _identity(v):
    return v


def _spare_rows(buf):
    n = 32 // buf.dtype.itemsize
    return pl.ds(buf.shape[0] - n, n)


class _Group:
    def __init__(self, src, dst, base, slot_rows, tick_rows, n_slots=_SLOTS,
                 cut=0, is_last=False):
        self.src, self.dst, self.base = src, dst, base
        self.slot_rows, self.tick_rows, self.n_slots = slot_rows, tick_rows, n_slots
        self.n_ticks = len(tick_rows)
        self.cut, self.is_last = cut, is_last

    def _copy(self, i, offset, size, sem):
        start = self.base + i * self.slot_rows + offset
        if not isinstance(start, int):
            start = pl.multiple_of(start, 8)
        rows = pl.ds(start, size)
        return pltpu.make_async_copy(self.src.at[rows], self.dst.at[rows], sem)

    def with_bulk(self, i, sem, action):
        head = sum(self.tick_rows)
        size = self.slot_rows - head
        if not self.cut or self.is_last is False:
            return action(self._copy(i, head, size, sem))
        short = self.is_last & (i == self.n_slots - 1)
        if isinstance(short, bool):
            return action(self._copy(i, head, size - self.cut * short, sem))
        pl.when(short)(lambda: action(self._copy(i, head, size - self.cut, sem)))
        pl.when(~short)(lambda: action(self._copy(i, head, size, sem)))

    def tick(self, i, j, sem):
        size = self.tick_rows[j]
        offset = sum(t for k, t in enumerate(self.tick_rows) if (-t, k) < (-size, j))
        return self._copy(i, offset, size, sem)

    def slot(self, i, sem):
        return self._copy(i, 0, self.slot_rows, sem)

    def after_ticks(self, lhs):
        zero = pltpu.bitcast(self.dst[_spare_rows(self.dst), 0:128], _BF16)
        reps = (lhs.shape[0] // zero.shape[0], lhs.shape[1] // zero.shape[1])
        return lhs + jnp.tile(zero, reps)


def _slot_sem(sems, phase, i):
    k = (phase * _SLOTS) % _RING + i
    if isinstance(k, int):
        return sems.at[k % _RING]
    return sems.at[jnp.where(k >= _RING, k - _RING, k)]


def _stream_step(program, sems, phase, arriving, following, i, piece, carry):
    sem_in, sem_out = _slot_sem(sems, phase, i), _slot_sem(sems, phase + 1, i)
    request = following.n_slots == _SLOTS or i < following.n_slots
    waits_left = sum(op.isdigit() for op in program)
    bulk_waited, waited, started, part = False, 0, 0, 0
    for pos, op in enumerate(program):
        if op == "b":
            arriving.tick(i, waited, sem_in).wait()
            waited += 1
        elif op.isdigit():
            waits_left -= 1
            if not bulk_waited:
                arriving.with_bulk(i, sem_in, lambda copy: copy.wait())
                bulk_waited = True
            upto = min(waited + int(op), arriving.n_ticks) if waits_left else arriving.n_ticks
            for j in range(waited, upto):
                arriving.tick(i, j, sem_in).wait()
            waited = upto
        elif op == "S" and request:
            following.with_bulk(i, sem_out, lambda copy: copy.start(priority=1))
        elif op == "T" and request:
            upto = started + 1 if "T" in program[pos + 1:] else following.n_ticks
            for j in range(started, min(upto, following.n_ticks)):
                following.tick(i, j, sem_out).start()
            started = upto
        elif op == "P":
            carry = piece(i, part, carry, following.after_ticks)
            part += 1
    return carry


def _stream_phase(program, sems, phase, arriving, following, piece=None, carry=0,
                  unroll=False):
    step = functools.partial(_stream_step, program, sems, phase, arriving, following)
    if unroll:
        for i in range(_SLOTS):
            carry = step(i, piece, carry)
        return carry
    return lax.fori_loop(0, _SLOTS, lambda i, c: step(i, piece, c), carry)


def _kernel(x_hbm, ckv_hbm, wq_hbm, wuk_hbm, wuv_hbm, wo_hbm, w3_hbm, w4_hbm,
            c_hbm, wmod_hbm, o_ref,
            x_v, c_v, wmod_v, wq_v, wuk_v, wuv_v, wo_v, w3_v, w4_v, ckv_v,
            mod_v, h_v, q_v, qabs32_v, qabs_v, s_v, lat_v, ctx_v, sems,
            *, B, H, Sk, D, M, F):
    NP = H // 2
    KC = Sk // _PIECES
    assert NP == _PIECES

    def halves(src, dst, tick_rows, shift, base=0, rows=None, is_last=True):
        slot = (src.shape[0] if rows is None else rows) // (2 * _SLOTS)
        return [_Group(src, dst, shift + base + k * _SLOTS * slot, slot, tick_rows,
                       cut=shift, is_last=is_last if k == 1 else False)
                for k in range(2)]

    def head_weights(src, dst):
        return halves(src.bitcast(jnp.uint32), dst, [2 * t for t in _TICK_KIB],
                      2 * _SHIFT_KIB)

    def g_kv(b):
        return halves(ckv_hbm, ckv_v, _TICK_KIB, _SHIFT_KIB, b * Sk, Sk, b == B - 1)

    g_mod = halves(wmod_hbm, wmod_v, (8, 8), 0)
    g_q = head_weights(wq_hbm, wq_v)
    g_uk = head_weights(wuk_hbm, wuk_v)
    g_uv = head_weights(wuv_hbm, wuv_v)
    g_o = halves(wo_hbm, wo_v, _TICK_KIB, _SHIFT_KIB)
    g_3 = _Group(w3_hbm, w3_v, 0, M // _SLOTS, (8, 8, 8, 8, 16))
    f_last = 256
    g_4 = _Group(w4_hbm, w4_v, 0, (F - f_last) // _SLOTS, (16, 16, 16, 16, 64))
    g_end = _Group(w4_hbm, w4_v, F - f_last, f_last, (32,), n_slots=1)

    small = [pltpu.make_async_copy(c_hbm, c_v, sems.at[_RING]),
             pltpu.make_async_copy(x_hbm, x_v, sems.at[_RING])]
    for copy in small:
        copy.start()
    _stream_phase("ST", sems, -1, None, g_mod[0], unroll=True)
    for buf in (wmod_v, wq_v, wuk_v, wuv_v, wo_v, w3_v, w4_v, ckv_v):
        spare = _spare_rows(buf)
        buf[spare, 0:128] = jnp.zeros((spare.size, 128), buf.dtype)

    def pair_weights(w_v, pair, half):
        words = w_v[pl.ds(pair + half * (M // 2) * NP, M // 2, stride=NP), :]
        return [pltpu.bitcast(w, _F32).astype(_BF16)
                for w in (words << 16, words & jnp.uint32(0xFFFF0000))]

    def pair_rows(pair):
        return pl.ds(pl.multiple_of(pair * 2 * B, 2 * B), 2 * B)

    def head_rows(head):
        return pl.ds(head, B, stride=H)

    def batch_rows(b):
        return pl.ds(b * H if isinstance(b, int) else pl.multiple_of(b * H, H), H)

    _stream_phase(_STEP_IDLE, sems, 0, g_mod[0], g_mod[1])
    for copy in small:
        copy.wait()
    cf = c_v[...].astype(_F32)
    sc = _lhs(cf * jax.nn.sigmoid(cf))

    heads = [pltpu.make_async_copy(g.src.at[pl.ds(0, g.base)], g.dst.at[pl.ds(0, g.base)],
                                   sems.at[_RING])
             for g in (g_q[0], g_uk[0], g_kv(0)[0], g_uv[0], g_o[0])]

    def mod(k):
        return mod_v[:, k * M:(k + 1) * M]

    def mod_piece(half, i, j, carry, pin):
        n = i * _PARTS + j
        rows = slice(half * (M // 2), (half + 1) * (M // 2))
        if n < 12:
            cols = slice(n * (M // 2), (n + 1) * (M // 2))
            part = _dot(pin(sc[:, rows]), wmod_v[rows, cols])[:B]
            mod_v[:, cols] = part if half == 0 else mod_v[:, cols] + part
        elif half == 0:
            for copy in heads[n - 12::_PIECES - 12]:
                copy.start()
        elif n == 12:
            h_v[...] = _lhs(_layernorm(x_v[...].astype(_F32)) * (1.0 + mod(1)) + mod(0))
        return carry

    _stream_phase(_STEP_MOD[0], sems, 1, g_mod[1], g_q[0],
                  functools.partial(mod_piece, 0), unroll=True)
    _stream_phase(_STEP_MOD[1], sems, 2, g_q[0], g_q[1],
                  functools.partial(mod_piece, 1), unroll=True)
    for copy in heads:
        copy.wait()

    def q_piece(half, i, j, carry, pin):
        pair = i * _PARTS + j
        h = pin(h_v[:, half * (M // 2):(half + 1) * (M // 2)])
        part = jnp.concatenate(
            [_dot(h, w)[:B] for w in pair_weights(wq_v, pair, half)], axis=0)
        rows = pair_rows(pair)
        q_v[rows, :] = part if half == 0 else q_v[rows, :] + part
        return carry

    _stream_phase(_STEP, sems, 3, g_q[1], g_uk[0], functools.partial(q_piece, 0))
    _stream_phase(_STEP, sems, 4, g_uk[0], g_uk[1], functools.partial(q_piece, 1))

    def qabs_piece(half, i, j, carry, pin):
        pair = i * _PARTS + j
        q = pin(q_v[pair_rows(pair), :].astype(_BF16))
        for p, w in enumerate(pair_weights(wuk_v, pair, half)):
            r = _dot_nt(q, w)[p * B:(p + 1) * B] * (D ** -0.5 * math.log2(math.e))
            for k in range(M // 256):
                qabs32_v[half * (M // 256) + k, head_rows(2 * pair + p), :] = (
                    r[:, k * 128:(k + 1) * 128])
        return carry

    _stream_phase(_STEP, sems, 5, g_uk[1], g_kv(0)[0], functools.partial(qabs_piece, 0))
    _stream_phase(_STEP, sems, 6, *g_kv(0), functools.partial(qabs_piece, 1))
    for k in range(M // 128):
        qabs_v[:, k * 128:(k + 1) * 128] = qabs32_v[k, 0:B * H, :].astype(_BF16)

    def keys(b, n):
        return ckv_v[pl.ds(pl.multiple_of(b * Sk + n * KC, KC), KC), :]

    def score_chunk(b, n, m, pin):
        s = _dot_nt(pin(qabs_v[batch_rows(b), :]), keys(b, n))
        s_v[b % 2, n] = s
        for t in range(0, KC, 128):
            m = jnp.maximum(m, s[:, t:t + 128])
        return m

    def value_chunk(b, n, m, l, acc, pin):
        s = s_v[b % 2, n]
        p = [jnp.exp2(s[:, t:t + 128] - m) for t in range(0, KC, 128)]
        for pt in p:
            l = l + pt
        p = pin(jnp.concatenate(p, axis=1).astype(_BF16))
        return l, acc + _dot(p, keys(b, n))

    def store_lat(b, l, acc):
        lat = acc / jnp.sum(l, axis=-1, keepdims=True)
        for k in range(M // 128):
            lat_v[k, batch_rows(b), :] = lat[:, k * 128:(k + 1) * 128]

    m_init = jnp.full((H, 128), -jnp.inf, _F32)
    l_init, acc_init = jnp.zeros((H, 128), _F32), jnp.zeros((H, M), _F32)

    def attend(b, groups, m_prev):
        def piece(half, i, j, carry, pin):
            m, l, acc = carry
            if groups[half + 1].dst is ckv_v:
                pin = _identity
            n = (half * _SLOTS + i) * (_PARTS // 2) + j // 2
            if j % 2 == 1:
                m = score_chunk(b, n, m, pin)
            elif m_prev is not None:
                l, acc = value_chunk(b - 1, n, m_prev, l, acc, pin)
            return m, l, acc

        carry = (m_init, 0, 0) if m_prev is None else (m_init, l_init, acc_init)
        for half in range(2):
            carry = _stream_phase(_STEP_ATTN, sems, 7 + 2 * b + half, groups[half],
                                  groups[half + 1], functools.partial(piece, half), carry)
        m, l, acc = carry
        if m_prev is not None:
            store_lat(b - 1, l, acc)
        return jnp.broadcast_to(jnp.max(m, axis=-1, keepdims=True), (H, 128))

    def kv_groups(b):
        return [g_kv(b)[1]] + g_kv(b + 1)

    def last_values(i, j, carry, pin):
        return value_chunk(B - 1, i * _PARTS + j, m_last, *carry, pin)

    m = attend(0, kv_groups(0), None)
    m = lax.fori_loop(1, B - 1, lambda b, m: attend(b, kv_groups(b), m), m)
    m_last = attend(B - 1, [g_kv(B - 1)[1]] + g_uv, m)
    store_lat(B - 1, *_stream_phase(_STEP, sems, 7 + 2 * B, g_uv[1], g_o[0],
                                    last_values, (l_init, acc_init)))

    def ctx_piece(k, i, j, acc, pin):
        pair, half = (k * _PIECES + i * _PARTS + j) // 2, j % 2
        lat = jnp.concatenate([jnp.concatenate(
            [lat_v[half * (M // 256) + t, head_rows(2 * pair + p), :]
             for t in range(M // 256)], axis=1) for p in range(2)], axis=0)
        lat = pin(lat.astype(_BF16))
        part = jnp.concatenate(
            [_dot(lat, w)[p * B:(p + 1) * B]
             for p, w in enumerate(pair_weights(wuv_v, pair, half))], axis=1)
        if half == 0:
            return part
        ctx_v[pair] = acc + part
        return acc

    ctx_init = jnp.zeros((B, 2 * D), _F32)
    _stream_phase(_STEP, sems, 8 + 2 * B, g_o[0], g_o[1],
                  functools.partial(ctx_piece, 0), ctx_init)
    _stream_phase(_STEP, sems, 9 + 2 * B, g_o[1], g_3,
                  functools.partial(ctx_piece, 1), ctx_init)

    def up_piece(i, j, carry, pin):
        n = i * _PARTS + j
        if n < NP // 2:
            for pair in (2 * n, 2 * n + 1):
                w = wo_v[pair * 2 * D:(pair + 1) * 2 * D, :]
                carry = carry + _dot(pin(_lhs(ctx_v[pair])), w)[:B]
        elif n == NP // 2:
            x1 = x_v[...].astype(_F32) + mod(2) * carry
            hb = _layernorm(x1) * (1.0 + mod(4)) + mod(3)
            carry = x1, hb, _lhs(_layernorm(hb)), jnp.zeros((B, F), _F32)
        elif n - NP // 2 <= _SLOTS:
            k = n - NP // 2 - 1
            assert k <= i
            x1, hb, ln, pre = carry
            rows = slice(k * g_3.slot_rows, (k + 1) * g_3.slot_rows)
            carry = x1, hb, ln, pre + _dot(pin(ln[:, rows]), w3_v[rows, :])[:B]
        return carry

    x1, y, _, pre = _stream_phase(_STEP_MLP, sems, 10 + 2 * B, g_3, g_4, up_piece,
                                  jnp.zeros((B, M), _F32), unroll=True)
    g = _lhs(_gelu(pre))

    def down_piece(i, j, y, pin):
        if (j + 1) * 128 > g_4.slot_rows:
            return y
        rows = slice(i * g_4.slot_rows + j * 128, i * g_4.slot_rows + (j + 1) * 128)
        return y + _dot(pin(g[:, rows]), w4_v[rows, :])[:B]

    assert g_4.slot_rows % 128 == 0 and g_4.slot_rows <= 128 * _PARTS
    y = _stream_phase(_STEP_MLP, sems, 11 + 2 * B, g_4, g_end, down_piece, y, unroll=True)
    g_end.slot(0, _slot_sem(sems, 12 + 2 * B, 0)).wait()
    y = y + _dot(g[:, F - f_last:], w4_v[F - f_last:F, :])[:B]
    o_ref[...] = (x1 + mod(5) * y).astype(o_ref.dtype)


@jax.jit
def pallas_adaLN_cond__compressed_kv_cla__mixer_s_mlp__decode_kernel(
    A_x: jax.Array,
    A_c_kv: jax.Array,
    A_w_q: jax.Array,
    A_w_uk: jax.Array,
    A_w_uv: jax.Array,
    A_w_o: jax.Array,
    B_x: jax.Array,
    B_w1: jax.Array,
    B_w2: jax.Array,
    B_w3: jax.Array,
    B_w4: jax.Array,
    c: jax.Array,
    w_mod: jax.Array,
):
    del B_x, B_w1, B_w2
    B, Sq, M = A_x.shape
    _, Sk, Dc = A_c_kv.shape
    _, H, D = A_w_q.shape
    F = B_w3.shape[1]
    assert Sq == 1 and Dc == M and D == 128 and B == 8

    x = A_x.reshape(B, M)
    ckv = A_c_kv.reshape(B * Sk, Dc)
    wq = A_w_q.reshape(M * H, D)
    wuk = A_w_uk.reshape(Dc * H, D)
    wuv = A_w_uv.reshape(Dc * H, D)
    wo = A_w_o.reshape(H * D, M)

    def streamed(a):
        return pltpu.VMEM((a.shape[0] + 16, a.shape[1]), a.dtype)

    def streamed_words(a):
        return pltpu.VMEM((a.shape[0] // 2 + 16, a.shape[1]), jnp.uint32)

    out = pl.pallas_call(
        functools.partial(_kernel, B=B, H=H, Sk=Sk, D=D, M=M, F=F),
        out_shape=jax.ShapeDtypeStruct(x.shape, x.dtype),
        in_specs=[pl.BlockSpec(memory_space=pl.ANY)] * 10,
        out_specs=pl.BlockSpec(memory_space=pltpu.VMEM),
        scratch_shapes=[
            pltpu.VMEM(x.shape, x.dtype), pltpu.VMEM(c.shape, c.dtype),
            streamed(w_mod), streamed_words(wq), streamed_words(wuk),
            streamed_words(wuv), streamed(wo), streamed(B_w3), streamed(B_w4),
            streamed(ckv),
            pltpu.VMEM((B, 6 * M), _F32),
            pltpu.VMEM((2 * B, M), _BF16),
            pltpu.VMEM((H * B, D), _F32),
            pltpu.VMEM((Dc // 128, (B + 1) * H, 128), _F32),
            pltpu.VMEM((B * H, Dc), _BF16),
            pltpu.VMEM((2, _PIECES, H, Sk // _PIECES), _F32),
            pltpu.VMEM((Dc // 128, (B + 1) * H, 128), _F32),
            pltpu.VMEM((H // 2, B, 2 * D), _F32),
            pltpu.SemaphoreType.DMA((_RING + 1,)),
        ],
        compiler_params=pltpu.CompilerParams(
            vmem_limit_bytes=100 * 1024 * 1024,
            disable_semaphore_checks=True,
        ),
    )(x, ckv, wq, wuk, wuv, wo, B_w3, B_w4, c, w_mod)
    return out.reshape(A_x.shape)
```

```python
import functools
import math

import jax
import jax.numpy as jnp
from jax import lax
import jax.experimental.pallas as pl
import jax.experimental.pallas.tpu as pltpu

_F32 = jnp.float32
_BF16 = jnp.bfloat16

_SLOTS = 4
_RING = _SLOTS + 1
_PARTS = 4
_PIECES = _SLOTS * _PARTS

_STEP = "1T2T2STPPTPPT"
_STEP_ATTN = "bTPPT0T9STPPT"
_STEP_MLP = "0T2T3STPPTPPT"
_STEP_IDLE = "0T1ST"
_STEP_MOD = ("0T1T1T1STPPPPT", "0T2T1T2STPPPPT")

_TICK_KIB = (32, 32, 32, 32, 64)
_SHIFT_KIB = 48


def _dot(a, b):
    return jnp.dot(a, b, preferred_element_type=_F32)


def _dot_nt(a, b):
    return lax.dot_general(a, b, (((1,), (1,)), ((), ())),
                           preferred_element_type=_F32)


def _layernorm(x, eps=1e-5):
    d = x - jnp.mean(x, axis=-1, keepdims=True)
    return d / jnp.sqrt(jnp.mean(d * d, axis=-1, keepdims=True) + eps)


def _gelu(x):
    c = math.sqrt(2.0 / math.pi)
    return 0.5 * x * (1.0 + jnp.tanh(c * (x + 0.044715 * (x * x * x))))


def _lhs(v):
    return jnp.concatenate([v, v], axis=0).astype(_BF16)


def _identity(v):
    return v


def _spare_rows(buf):
    return pl.ds(buf.shape[0] - 16, 16)


class _Group:
    def __init__(self, src, dst, base, slot_rows, tick_rows, n_slots=_SLOTS,
                 cut=0, is_last=False, words=None):
        self.src, self.dst, self.base = src, dst, base
        self.slot_rows, self.tick_rows, self.n_slots = slot_rows, tick_rows, n_slots
        self.n_ticks = len(tick_rows)
        self.cut, self.is_last = cut, is_last
        self.words = words

    def _copy(self, i, offset, size, sem):
        start = self.base + i * self.slot_rows + offset
        if not isinstance(start, int):
            start = pl.multiple_of(start, 8)
        rows = pl.ds(start, size)
        return pltpu.make_async_copy(self.src.at[rows], self.dst.at[rows], sem)

    def with_bulk(self, i, sem, action):
        head = sum(self.tick_rows)
        size = self.slot_rows - head
        if not self.cut or self.is_last is False:
            return action(self._copy(i, head, size, sem))
        short = self.is_last & (i == self.n_slots - 1)
        if isinstance(short, bool):
            return action(self._copy(i, head, size - self.cut * short, sem))
        pl.when(short)(lambda: action(self._copy(i, head, size - self.cut, sem)))
        pl.when(~short)(lambda: action(self._copy(i, head, size, sem)))

    def tick(self, i, j, sem):
        size = self.tick_rows[j]
        offset = sum(t for k, t in enumerate(self.tick_rows) if (-t, k) < (-size, j))
        return self._copy(i, offset, size, sem)

    def slot(self, i, sem):
        return self._copy(i, 0, self.slot_rows, sem)

    def copy_to_words(self, i, k):
        n = self.slot_rows // 4
        start = (self.base - self.cut) // 2 + (2 * i + k) * n
        if not isinstance(start, int):
            start = pl.multiple_of(start, n)
        self.words[pl.ds(start, n), :] = pltpu.bitcast(
            self.dst[pl.ds(2 * start, 2 * n), :], jnp.uint32)

    def after_ticks(self, lhs):
        zero = self.dst[_spare_rows(self.dst), 0:128]
        reps = (lhs.shape[0] // zero.shape[0], lhs.shape[1] // zero.shape[1])
        return lhs + jnp.tile(zero, reps)


def _slot_sem(sems, phase, i):
    k = (phase * _SLOTS) % _RING + i
    if isinstance(k, int):
        return sems.at[k % _RING]
    return sems.at[jnp.where(k >= _RING, k - _RING, k)]


def _stream_step(program, sems, phase, arriving, following, i, piece, carry):
    sem_in, sem_out = _slot_sem(sems, phase, i), _slot_sem(sems, phase + 1, i)
    request = following.n_slots == _SLOTS or i < following.n_slots
    waits_left = sum(op.isdigit() for op in program)
    bulk_waited, waited, started, part = False, 0, 0, 0
    for pos, op in enumerate(program):
        if op == "b":
            arriving.tick(i, waited, sem_in).wait()
            waited += 1
        elif op.isdigit():
            waits_left -= 1
            if not bulk_waited:
                arriving.with_bulk(i, sem_in, lambda copy: copy.wait())
                bulk_waited = True
            upto = min(waited + int(op), arriving.n_ticks) if waits_left else arriving.n_ticks
            for j in range(waited, upto):
                arriving.tick(i, j, sem_in).wait()
            waited = upto
        elif op == "S" and request:
            following.with_bulk(i, sem_out, lambda copy: copy.start(priority=1))
        elif op == "T" and request:
            upto = started + 1 if "T" in program[pos + 1:] else following.n_ticks
            for j in range(started, min(upto, following.n_ticks)):
                following.tick(i, j, sem_out).start()
            started = upto
        elif op == "P":
            carry = piece(i, part, carry, following.after_ticks)
            if arriving.words is not None and part >= _PARTS - 2:
                assert not waits_left
                arriving.copy_to_words(i, part - (_PARTS - 2))
            part += 1
    return carry


def _stream_phase(program, sems, phase, arriving, following, piece=None, carry=0,
                  unroll=False):
    step = functools.partial(_stream_step, program, sems, phase, arriving, following)
    if unroll:
        for i in range(_SLOTS):
            carry = step(i, piece, carry)
        return carry
    return lax.fori_loop(0, _SLOTS, lambda i, c: step(i, piece, c), carry)


def _kernel(x_hbm, ckv_hbm, wq_hbm, wuk_hbm, wuv_hbm, wo_hbm, w3_hbm, w4_hbm,
            c_hbm, wmod_hbm, o_ref,
            x_v, c_v, wmod_v, wq_v, wuk_v, wuv_v, wo_v, w3_v, w4_v, ckv_v,
            wq_w, wuk_w, wuv_w,
            mod_v, h_v, q_v, qabs32_v, qabs_v, s_v, lat_v, ctx_v, sems,
            *, B, H, Sk, D, M, F):
    NP = H // 2
    KC = Sk // _PIECES
    assert NP == _PIECES

    def halves(src, dst, tick_rows, shift, base=0, rows=None, is_last=True, words=None):
        slot = (src.shape[0] if rows is None else rows) // (2 * _SLOTS)
        return [_Group(src, dst, shift + base + k * _SLOTS * slot, slot, tick_rows,
                       cut=shift, is_last=is_last if k == 1 else False, words=words)
                for k in range(2)]

    def head_weights(src, dst, words):
        return halves(src, dst, [4 * t for t in _TICK_KIB], 4 * _SHIFT_KIB, words=words)

    def g_kv(b):
        return halves(ckv_hbm, ckv_v, _TICK_KIB, _SHIFT_KIB, b * Sk, Sk, b == B - 1)

    g_mod = halves(wmod_hbm, wmod_v, (8, 8), 0)
    g_q = head_weights(wq_hbm, wq_v, wq_w)
    g_uk = head_weights(wuk_hbm, wuk_v, wuk_w)
    g_uv = head_weights(wuv_hbm, wuv_v, wuv_w)
    g_o = halves(wo_hbm, wo_v, _TICK_KIB, _SHIFT_KIB)
    g_3 = _Group(w3_hbm, w3_v, 0, M // _SLOTS, (8, 8, 8, 8, 16))
    f_last = 256
    g_4 = _Group(w4_hbm, w4_v, 0, (F - f_last) // _SLOTS, (16, 16, 16, 16, 64))
    g_end = _Group(w4_hbm, w4_v, F - f_last, f_last, (32,), n_slots=1)

    small = [pltpu.make_async_copy(c_hbm, c_v, sems.at[_RING]),
             pltpu.make_async_copy(x_hbm, x_v, sems.at[_RING])]
    for copy in small:
        copy.start()
    _stream_phase("ST", sems, -1, None, g_mod[0], unroll=True)
    for buf in (wmod_v, wq_v, wuk_v, wuv_v, wo_v, w3_v, w4_v, ckv_v):
        spare = _spare_rows(buf)
        buf[spare, 0:128] = jnp.zeros((spare.size, 128), buf.dtype)

    def pair_weights(w_v, pair, half):
        words = w_v[pl.ds(pair + half * (M // 2) * NP, M // 2, stride=NP), :]
        return [pltpu.bitcast(w, _F32).astype(_BF16)
                for w in (words << 16, words & jnp.uint32(0xFFFF0000))]

    def pair_rows(pair):
        return pl.ds(pl.multiple_of(pair * 2 * B, 2 * B), 2 * B)

    def head_rows(head):
        return pl.ds(head, B, stride=H)

    def batch_rows(b):
        return pl.ds(b * H if isinstance(b, int) else pl.multiple_of(b * H, H), H)

    _stream_phase(_STEP_IDLE, sems, 0, g_mod[0], g_mod[1])
    for copy in small:
        copy.wait()
    cf = c_v[...].astype(_F32)
    sc = _lhs(cf * jax.nn.sigmoid(cf))

    heads = [pltpu.make_async_copy(g.src.at[pl.ds(0, g.base)], g.dst.at[pl.ds(0, g.base)],
                                   sems.at[_RING])
             for g in (g_q[0], g_uk[0], g_kv(0)[0], g_uv[0], g_o[0])]

    def mod(k):
        return mod_v[:, k * M:(k + 1) * M]

    def mod_piece(half, i, j, carry, pin):
        n = i * _PARTS + j
        rows = slice(half * (M // 2), (half + 1) * (M // 2))
        if n < 12:
            cols = slice(n * (M // 2), (n + 1) * (M // 2))
            part = _dot(pin(sc[:, rows]), wmod_v[rows, cols])[:B]
            mod_v[:, cols] = part if half == 0 else mod_v[:, cols] + part
            if half == 0 and n < len(heads):
                heads[n].start()
        elif n == 12 and half == 1:
            h_v[...] = _lhs(_layernorm(x_v[...].astype(_F32)) * (1.0 + mod(1)) + mod(0))
        return carry

    _stream_phase(_STEP_MOD[0], sems, 1, g_mod[1], g_q[0],
                  functools.partial(mod_piece, 0), unroll=True)
    for copy in heads:
        copy.wait()
    _stream_phase(_STEP_MOD[1], sems, 2, g_q[0], g_q[1],
                  functools.partial(mod_piece, 1), unroll=True)

    def q_piece(half, i, j, carry, pin):
        pair = i * _PARTS + j
        h = pin(h_v[:, half * (M // 2):(half + 1) * (M // 2)])
        part = jnp.concatenate(
            [_dot(h, w)[:B] for w in pair_weights(wq_w, pair, half)], axis=0)
        rows = pair_rows(pair)
        q_v[rows, :] = part if half == 0 else q_v[rows, :] + part
        return carry

    _stream_phase(_STEP, sems, 3, g_q[1], g_uk[0], functools.partial(q_piece, 0))
    _stream_phase(_STEP, sems, 4, g_uk[0], g_uk[1], functools.partial(q_piece, 1))

    def qabs_piece(half, i, j, carry, pin):
        pair = i * _PARTS + j
        q = pin(q_v[pair_rows(pair), :].astype(_BF16))
        for p, w in enumerate(pair_weights(wuk_w, pair, half)):
            r = _dot_nt(q, w)[p * B:(p + 1) * B] * (D ** -0.5 * math.log2(math.e))
            for k in range(M // 256):
                qabs32_v[half * (M // 256) + k, head_rows(2 * pair + p), :] = (
                    r[:, k * 128:(k + 1) * 128])
        return carry

    _stream_phase(_STEP, sems, 5, g_uk[1], g_kv(0)[0], functools.partial(qabs_piece, 0))
    _stream_phase(_STEP, sems, 6, *g_kv(0), functools.partial(qabs_piece, 1))
    for k in range(M // 128):
        qabs_v[:, k * 128:(k + 1) * 128] = qabs32_v[k, 0:B * H, :].astype(_BF16)

    def keys(b, n):
        return ckv_v[pl.ds(pl.multiple_of(b * Sk + n * KC, KC), KC), :]

    def score_chunk(b, n, m, pin):
        s = _dot_nt(pin(qabs_v[batch_rows(b), :]), keys(b, n))
        s_v[b % 2, n] = s
        for t in range(0, KC, 128):
            m = jnp.maximum(m, s[:, t:t + 128])
        return m

    def value_chunk(b, n, m, l, acc, pin):
        s = s_v[b % 2, n]
        p = [jnp.exp2(s[:, t:t + 128] - m) for t in range(0, KC, 128)]
        for pt in p:
            l = l + pt
        p = pin(jnp.concatenate(p, axis=1).astype(_BF16))
        return l, acc + _dot(p, keys(b, n))

    def store_lat(b, l, acc):
        lat = acc / jnp.sum(l, axis=-1, keepdims=True)
        for k in range(M // 128):
            lat_v[k, batch_rows(b), :] = lat[:, k * 128:(k + 1) * 128]

    m_init = jnp.full((H, 128), -jnp.inf, _F32)
    l_init, acc_init = jnp.zeros((H, 128), _F32), jnp.zeros((H, M), _F32)

    def attend(b, groups, m_prev):
        def piece(half, i, j, carry, pin):
            m, l, acc = carry
            if groups[half + 1].dst is ckv_v:
                pin = _identity
            n = (half * _SLOTS + i) * (_PARTS // 2) + j // 2
            if j % 2 == 1:
                m = score_chunk(b, n, m, pin)
            elif m_prev is not None:
                l, acc = value_chunk(b - 1, n, m_prev, l, acc, pin)
            return m, l, acc

        carry = (m_init, 0, 0) if m_prev is None else (m_init, l_init, acc_init)
        for half in range(2):
            carry = _stream_phase(_STEP_ATTN, sems, 7 + 2 * b + half, groups[half],
                                  groups[half + 1], functools.partial(piece, half), carry)
        m, l, acc = carry
        if m_prev is not None:
            store_lat(b - 1, l, acc)
        return jnp.broadcast_to(jnp.max(m, axis=-1, keepdims=True), (H, 128))

    def kv_groups(b):
        return [g_kv(b)[1]] + g_kv(b + 1)

    def last_values(i, j, carry, pin):
        return value_chunk(B - 1, i * _PARTS + j, m_last, *carry, pin)

    m = attend(0, kv_groups(0), None)
    m = lax.fori_loop(1, B - 1, lambda b, m: attend(b, kv_groups(b), m), m)
    m_last = attend(B - 1, [g_kv(B - 1)[1]] + g_uv, m)
    store_lat(B - 1, *_stream_phase(_STEP, sems, 7 + 2 * B, g_uv[1], g_o[0],
                                    last_values, (l_init, acc_init)))

    def ctx_piece(k, i, j, acc, pin):
        pair, half = (k * _PIECES + i * _PARTS + j) // 2, j % 2
        lat = jnp.concatenate([jnp.concatenate(
            [lat_v[half * (M // 256) + t, head_rows(2 * pair + p), :]
             for t in range(M // 256)], axis=1) for p in range(2)], axis=0)
        lat = pin(lat.astype(_BF16))
        part = jnp.concatenate(
            [_dot(lat, w)[p * B:(p + 1) * B]
             for p, w in enumerate(pair_weights(wuv_w, pair, half))], axis=1)
        if half == 0:
            return part
        ctx_v[pair] = acc + part
        return acc

    ctx_init = jnp.zeros((B, 2 * D), _F32)
    _stream_phase(_STEP, sems, 8 + 2 * B, g_o[0], g_o[1],
                  functools.partial(ctx_piece, 0), ctx_init)
    _stream_phase(_STEP, sems, 9 + 2 * B, g_o[1], g_3,
                  functools.partial(ctx_piece, 1), ctx_init)

    def up_piece(i, j, carry, pin):
        n = i * _PARTS + j
        if n < NP // 2:
            for pair in (2 * n, 2 * n + 1):
                w = wo_v[pair * 2 * D:(pair + 1) * 2 * D, :]
                carry = carry + _dot(pin(_lhs(ctx_v[pair])), w)[:B]
        elif n == NP // 2:
            x1 = x_v[...].astype(_F32) + mod(2) * carry
            hb = _layernorm(x1) * (1.0 + mod(4)) + mod(3)
            carry = x1, hb, _lhs(_layernorm(hb)), jnp.zeros((B, F), _F32)
        elif n - NP // 2 <= _SLOTS:
            k = n - NP // 2 - 1
            assert k <= i
            x1, hb, ln, pre = carry
            rows = slice(k * g_3.slot_rows, (k + 1) * g_3.slot_rows)
            carry = x1, hb, ln, pre + _dot(pin(ln[:, rows]), w3_v[rows, :])[:B]
        return carry

    x1, y, _, pre = _stream_phase(_STEP_MLP, sems, 10 + 2 * B, g_3, g_4, up_piece,
                                  jnp.zeros((B, M), _F32), unroll=True)
    g = _lhs(_gelu(pre))

    def down_piece(i, j, y, pin):
        if (j + 1) * 128 > g_4.slot_rows:
            return y
        rows = slice(i * g_4.slot_rows + j * 128, i * g_4.slot_rows + (j + 1) * 128)
        return y + _dot(pin(g[:, rows]), w4_v[rows, :])[:B]

    assert g_4.slot_rows % 128 == 0 and g_4.slot_rows <= 128 * _PARTS
    y = _stream_phase(_STEP_MLP, sems, 11 + 2 * B, g_4, g_end, down_piece, y, unroll=True)
    g_end.slot(0, _slot_sem(sems, 12 + 2 * B, 0)).wait()
    y = y + _dot(g[:, F - f_last:], w4_v[F - f_last:F, :])[:B]
    o_ref[...] = (x1 + mod(5) * y).astype(o_ref.dtype)


@jax.jit
def pallas_adaLN_cond__compressed_kv_cla__mixer_s_mlp__decode_kernel(
    A_x: jax.Array,
    A_c_kv: jax.Array,
    A_w_q: jax.Array,
    A_w_uk: jax.Array,
    A_w_uv: jax.Array,
    A_w_o: jax.Array,
    B_x: jax.Array,
    B_w1: jax.Array,
    B_w2: jax.Array,
    B_w3: jax.Array,
    B_w4: jax.Array,
    c: jax.Array,
    w_mod: jax.Array,
):
    del B_x, B_w1, B_w2
    B, Sq, M = A_x.shape
    _, Sk, Dc = A_c_kv.shape
    _, H, D = A_w_q.shape
    F = B_w3.shape[1]
    assert Sq == 1 and Dc == M and D == 128 and B == 8

    x = A_x.reshape(B, M)
    ckv = A_c_kv.reshape(B * Sk, Dc)
    wq = A_w_q.reshape(M * H, D)
    wuk = A_w_uk.reshape(Dc * H, D)
    wuv = A_w_uv.reshape(Dc * H, D)
    wo = A_w_o.reshape(H * D, M)

    def streamed(a):
        return pltpu.VMEM((a.shape[0] + 16, a.shape[1]), a.dtype)

    def words(a):
        return pltpu.VMEM((a.shape[0] // 2 + 16, a.shape[1]), jnp.uint32)

    out = pl.pallas_call(
        functools.partial(_kernel, B=B, H=H, Sk=Sk, D=D, M=M, F=F),
        out_shape=jax.ShapeDtypeStruct(x.shape, x.dtype),
        in_specs=[pl.BlockSpec(memory_space=pl.ANY)] * 10,
        out_specs=pl.BlockSpec(memory_space=pltpu.VMEM),
        scratch_shapes=[
            pltpu.VMEM(x.shape, x.dtype), pltpu.VMEM(c.shape, c.dtype),
            streamed(w_mod), streamed(wq), streamed(wuk), streamed(wuv),
            streamed(wo), streamed(B_w3), streamed(B_w4), streamed(ckv),
            words(wq), words(wuk), words(wuv),
            pltpu.VMEM((B, 6 * M), _F32),
            pltpu.VMEM((2 * B, M), _BF16),
            pltpu.VMEM((H * B, D), _F32),
            pltpu.VMEM((Dc // 128, (B + 1) * H, 128), _F32),
            pltpu.VMEM((B * H, Dc), _BF16),
            pltpu.VMEM((2, _PIECES, H, Sk // _PIECES), _F32),
            pltpu.VMEM((Dc // 128, (B + 1) * H, 128), _F32),
            pltpu.VMEM((H // 2, B, 2 * D), _F32),
            pltpu.SemaphoreType.DMA((_RING + 1,)),
        ],
        compiler_params=pltpu.CompilerParams(
            vmem_limit_bytes=100 * 1024 * 1024,
            disable_semaphore_checks=True,
        ),
    )(x, ckv, wq, wuk, wuv, wo, B_w3, B_w4, c, w_mod)
    return out.reshape(A_x.shape)
```
